```python
import os as _os
_os.environ.setdefault("JAX_PLATFORMS", "cpu")
import jax
import jax.numpy as jnp

def _softmax(x, axis=-1):
    return jax.nn.softmax(x, axis=axis)
def _gelu(x):
    return jax.nn.gelu(x, approximate=True)
def _silu(x):
    return jax.nn.silu(x)
def _sigmoid(x):
    return jax.nn.sigmoid(x)
def _layernorm(x, axis=-1, eps=1e-5):
    m = jnp.mean(x, axis=axis, keepdims=True)
    v = jnp.var(x, axis=axis, keepdims=True)
    return (x - m) / jnp.sqrt(v + eps)
def _scatter_add(tgt, idx, src, axis=0):
    return tgt.at[idx].add(src)
def _segment_sum(src, seg, n):
    return jax.ops.segment_sum(src, seg, n)
class _Rng:
    def __init__(self, key):
        self._k = key
    def _next(self):
        self._k, sub = jax.random.split(self._k)
        return sub
    def normal(self, shape):
        return jax.random.normal(self._next(), shape, dtype=jnp.bfloat16)
    def randint(self, lo, hi, shape):
        return jax.random.randint(self._next(), shape, lo, hi, dtype=jnp.int32)
    def uniform(self, shape, lo=0.0, hi=1.0):
        return jax.random.uniform(self._next(), shape, jnp.bfloat16, lo, hi)
    def permutation(self, n):
        return jax.random.permutation(self._next(), n)


kernel_name = 'parallel_sum__ssm_conv_h3__dense_activation_silu__prompt'

def setup_inputs():
    _rng = _Rng(jax.random.key(int.from_bytes(__import__("os").urandom(4), "little")))
    _w = (lambda a: (lambda t: t.astype(jnp.bfloat16) if jnp.issubdtype(t.dtype, jnp.floating) else t)(jnp.asarray(a)))
    def _A_setup():
        B, S, D = 1, 2048, 448
        ks = 4
        return {
            "q": _w((lambda *s: _rng.normal(s) * 0.05)(B, S, D)),
            "k": _w((lambda *s: _rng.normal(s) * 0.2)(B, S, D)),
            "v": _w((lambda *s: _rng.normal(s) * 0.2)(B, S, D)),
            "shift_k": _w((lambda *s: _rng.normal(s) * 0.2)(D, ks) * 0.5),
            "ssm_k": _w((lambda *s: _rng.normal(s) * 0.2)(D, S) * (1.0 / S ** 0.5)),
            "ssm_D": _w((lambda *s: _rng.normal(s) * 0.2)(D)),
        }
    _A_in = _A_setup()

    def _B_setup():
        B, S, D, F = 1, 2048, 448, 1792
        return {
            "x": _w((lambda *s: _rng.normal(s) * 0.05)(B, S, D)),
            "w1": _w((lambda *s: _rng.normal(s) * 0.05)(D, F) * (D ** -0.5)),
            "w2": _w((lambda *s: _rng.normal(s) * 0.05)(F, D) * (F ** -0.5)),
        }
    _B_in = _B_setup()

    return {
        "A_q": _A_in["q"],
        "A_k": _A_in["k"],
        "A_v": _A_in["v"],
        "A_shift_k": _A_in["shift_k"],
        "A_ssm_k": _A_in["ssm_k"],
        "A_ssm_D": _A_in["ssm_D"],
        "B_x": _B_in["x"],
        "B_w1": _B_in["w1"],
        "B_w2": _B_in["w2"],
    }

def reference(A_q, A_k, A_v, A_shift_k, A_ssm_k, A_ssm_D, B_x, B_w1, B_w2):
    def _A_ref(q, k, v, shift_k, ssm_k, ssm_D):
        B, S, D = q.shape
        ks = shift_k.shape[-1]
        k_pad = jnp.pad(k, ((0, 0), (ks - 1, 0), (0, 0)))
        k_shift = jnp.zeros_like(k)
        for t in range(ks):
            k_shift = k_shift + k_pad[:, t:t + S, :] * shift_k[:, ks - 1 - t][None, None, :]
        kv = k_shift * v
        L = 2 * S
        kv_pad = jnp.pad(kv, ((0, 0), (0, S), (0, 0)))
        kf_pad = jnp.pad(ssm_k, ((0, 0), (0, S)))
        kv_f = (lambda x, axes=(-2,-1): jnp.fft.rfft2(x.astype(jnp.float32), axes=axes))(kv_pad[:, None, :, :], axes=(1, 2))
        kf_f = (lambda x, axes=(-2,-1): jnp.fft.rfft2(x.astype(jnp.float32), axes=axes))(kf_pad[:, None, :], axes=(1, 2))
        kf_f = (lambda x, *d: x.transpose(*d))(kf_f, 1, 2, 0)
        y_f = kv_f * kf_f[None, :, :, :]
        y = (lambda x, s, axes=(-2,-1): jnp.fft.irfft2(x, s=s, axes=axes).astype(jnp.bfloat16))(y_f, (1, L), axes=(1, 2))[:, 0, :S, :]
        y = y + kv * ssm_D[None, None, :]
        return q * y

    def _B_ref(x, w1, w2):
        h = jnp.einsum("bsd,df->bsf", x, w1)
        h = _silu(h)
        out = jnp.einsum("bsf,fd->bsd", h, w2)
        return out

    x = A_q
    xn = _layernorm(x, axis=-1)
    return x + _A_ref(xn, A_k, A_v, A_shift_k, A_ssm_k, A_ssm_D) + _B_ref(xn, B_w1, B_w2)
```

```python
import math

import numpy as np
import jax
import jax.numpy as jnp
import jax.experimental.pallas as pl
import jax.experimental.pallas.tpu as pltpu

S = 2048
D = 448
F = 1792
L = 2 * S
NB = 64
NA = L // NB
NF1 = NA // 2 + 1
CB = 128
NCB = (D + CB - 1) // CB
RB = 512
NRB = S // RB
EPS = 1e-5


def _add(a, b):
    if a is None:
        return b
    if b is None:
        return a
    return a + b


def _sub(a, b):
    if b is None:
        return a
    if a is None:
        return -b
    return a - b


def _mulc(a, c):
    if a is None or c == 0.0:
        return None
    if c == 1.0:
        return a
    if c == -1.0:
        return -a
    return a * c


def _cmul_const(z, wr, wi):
    zr, zi = z
    if abs(wr) < 1e-12:
        wr = 0.0
    if abs(wi) < 1e-12:
        wi = 0.0
    if abs(abs(wr) - 1) < 1e-12:
        wr = math.copysign(1.0, wr)
    if abs(abs(wi) - 1) < 1e-12:
        wi = math.copysign(1.0, wi)
    re = _sub(_mulc(zr, wr), _mulc(zi, wi))
    im = _add(_mulc(zr, wi), _mulc(zi, wr))
    return (re, im)


def _rdft(x):
    n = len(x)
    if n == 1:
        return [(x[0], None)]
    if n == 2:
        return [(_add(x[0], x[1]), None), (_sub(x[0], x[1]), None)]
    e = _rdft(x[0::2])
    o = _rdft(x[1::2])
    out = [None] * (n // 2 + 1)
    for k in range(n // 4 + 1):
        t = _cmul_const(o[k], math.cos(2 * math.pi * k / n),
                        -math.sin(2 * math.pi * k / n))
        out[k] = (_add(e[k][0], t[0]), _add(e[k][1], t[1]))
        if n // 2 - k != k:
            out[n // 2 - k] = (_sub(e[k][0], t[0]), _sub(t[1], e[k][1]))
    return out


def _irdft(x, n, need):
    if n == 1:
        return [x[0][0]]
    if n == 2:
        out = [_add(x[0][0], x[1][0])]
        if need > 1:
            out.append(_sub(x[0][0], x[1][0]))
        return out
    e = [None] * (n // 4 + 1)
    o = [None] * (n // 4 + 1)
    for k in range(n // 4 + 1):
        a = x[k]
        b = x[n // 2 - k]
        e[k] = (_add(a[0], b[0]), _sub(a[1], b[1]))
        d = (_sub(a[0], b[0]), _add(a[1], b[1]))
        o[k] = _cmul_const(d, math.cos(2 * math.pi * k / n),
                           math.sin(2 * math.pi * k / n))
    ne = (need + 1) // 2
    no = need // 2
    xe = _irdft(e, n // 2, ne)
    xo = _irdft(o, n // 2, no) if no > 0 else []
    return [xe[i // 2] if i % 2 == 0 else xo[i // 2] for i in range(need)]


def _dft_tables():
    fwd = np.zeros((NF1, 2 * NB, 2 * NB), np.float64)
    inv = np.zeros((NF1, 2 * NB, 2 * NB), np.float64)
    b = np.arange(NB)[None, :]
    for f1 in range(NF1):
        f = f1 + NA * np.arange(NB)[:, None]
        th = 2.0 * np.pi * ((f * b) % L) / L
        c, s = np.cos(th), np.sin(th)
        fwd[f1] = np.block([[c, s], [-s, c]])
        inv[f1] = np.block([[c.T, -s.T], [s.T, c.T]]) / L
    return fwd.astype(np.float32), inv.astype(np.float32)


def _kernel(q_ref, k_ref, v_ref, sk_ref, hk_ref, sd_ref, w1_ref, w2_ref,
            mf_ref, mi_ref, o_ref,
            kpad_ref, u_ref, ht_ref, g_ref, p_ref, y_ref):
    step = pl.program_id(0)
    f32 = jnp.float32
    bf16 = jnp.bfloat16

    @pl.when(step < NCB)
    def _conv():
        kpad_ref[pl.ds(0, 8), :] = jnp.zeros((8, CB), f32)
        kpad_ref[pl.ds(8, S), :] = k_ref[...].astype(f32)
        sk = sk_ref[...].astype(f32)
        ks = kpad_ref[pl.ds(8, S), :] * sk[0:1, :]
        for j in range(1, 4):
            ks = ks + kpad_ref[pl.ds(8 - j, S), :] * sk[j:j + 1, :]
        u_ref[...] = ks * v_ref[...].astype(f32)
        ht_ref[...] = hk_ref[...].astype(f32).T

        def s1_body(r, carry):
            r8 = pl.multiple_of(r * 8, 8)
            for src, lane0 in ((u_ref, 0), (ht_ref, CB)):
                xs = [src[pl.ds(NB * a + r8, 8), :] for a in range(NA // 2)]
                xs = xs + [None] * (NA // 2)
                g = _rdft(xs)
                for f1 in range(NF1):
                    gr, gi = g[f1]
                    if gi is None:
                        gi = jnp.zeros((8, CB), f32)
                    g_ref[f1, pl.ds(r8, 8), pl.ds(lane0, CB)] = gr
                    g_ref[f1, pl.ds(NB + r8, 8), pl.ds(lane0, CB)] = gi
            return carry

        jax.lax.fori_loop(0, NB // 8, s1_body, 0)

        for f1 in range(NF1):
            x = jnp.dot(mf_ref[f1], g_ref[f1].astype(bf16),
                        preferred_element_type=f32)
            xr, xi = x[:NB, :CB], x[NB:, :CB]
            hr, hi = x[:NB, CB:], x[NB:, CB:]
            yr = xr * hr - xi * hi
            yi = xr * hi + xi * hr
            yy = jnp.concatenate([yr, yi], axis=0).astype(bf16)
            p_ref[f1] = jnp.dot(mi_ref[f1], yy, preferred_element_type=f32)

        sd = sd_ref[...].astype(f32)

        def i1_body(r, carry):
            r8 = pl.multiple_of(r * 8, 8)
            xs = [(p_ref[f1, pl.ds(r8, 8), :], p_ref[f1, pl.ds(NB + r8, 8), :])
                  for f1 in range(NF1)]
            y = _irdft(xs, NA, NA // 2)
            for a in range(NA // 2):
                row = pl.ds(NB * a + r8, 8)
                yc = y[a].astype(bf16).astype(f32)
                y_ref[step, row, :] = yc + u_ref[row, :] * sd
            return carry

        jax.lax.fori_loop(0, NB // 8, i1_body, 0)

    @pl.when(step >= NCB)
    def _ffn():
        r0 = pl.multiple_of((step - NCB) * RB, RB)
        x = q_ref[...].astype(f32)
        mean = jnp.mean(x, axis=-1, keepdims=True)
        xc = x - mean
        var = jnp.mean(xc * xc, axis=-1, keepdims=True)
        xn = xc * jax.lax.rsqrt(var + EPS)
        xnb = xn.astype(bf16)
        h = jnp.dot(xnb, w1_ref[...], preferred_element_type=f32)
        h = h * jax.nn.sigmoid(h)
        ffn = jnp.dot(h.astype(bf16), w2_ref[...], preferred_element_type=f32)
        rows = pl.ds(r0, RB)
        y = jnp.concatenate(
            [y_ref[c, rows, :] for c in range(NCB - 1)]
            + [y_ref[NCB - 1, rows, :][:, :D - CB * (NCB - 1)]], axis=1)
        o_ref[...] = (x + xnb.astype(f32) * y + ffn).astype(o_ref.dtype)


@jax.jit
def pallas_parallel_sum__ssm_conv_h3__dense_activation_silu__prompt_kernel(
    A_q: jax.Array,
    A_k: jax.Array,
    A_v: jax.Array,
    A_shift_k: jax.Array,
    A_ssm_k: jax.Array,
    A_ssm_D: jax.Array,
    B_x: jax.Array,
    B_w1: jax.Array,
    B_w2: jax.Array,
):
    del B_x
    q = A_q.reshape(S, D)
    k = A_k.reshape(S, D)
    v = A_v.reshape(S, D)
    sk = A_shift_k.T
    sd = A_ssm_D.reshape(1, D)
    mf_np, mi_np = _dft_tables()
    mf = jnp.asarray(mf_np, dtype=jnp.bfloat16)
    mi = jnp.asarray(mi_np, dtype=jnp.bfloat16)

    cidx = lambda i: jnp.minimum(i, NCB - 1)
    ridx = lambda i: jnp.maximum(i - NCB, 0)

    in_specs = [
        pl.BlockSpec((RB, D), lambda i: (ridx(i), 0)),
        pl.BlockSpec((S, CB), lambda i: (0, cidx(i))),
        pl.BlockSpec((S, CB), lambda i: (0, cidx(i))),
        pl.BlockSpec((4, CB), lambda i: (0, cidx(i))),
        pl.BlockSpec((CB, S), lambda i: (cidx(i), 0)),
        pl.BlockSpec((1, CB), lambda i: (0, cidx(i))),
        pl.BlockSpec((D, F), lambda i: (0, 0)),
        pl.BlockSpec((F, D), lambda i: (0, 0)),
        pl.BlockSpec((NF1, 2 * NB, 2 * NB), lambda i: (0, 0, 0)),
        pl.BlockSpec((NF1, 2 * NB, 2 * NB), lambda i: (0, 0, 0)),
    ]
    out_spec = pl.BlockSpec((RB, D), lambda i: (ridx(i), 0))
    scratch = [
        pltpu.VMEM((S + 8, CB), jnp.float32),
        pltpu.VMEM((S, CB), jnp.float32),
        pltpu.VMEM((S, CB), jnp.float32),
        pltpu.VMEM((NF1, 2 * NB, 2 * CB), jnp.float32),
        pltpu.VMEM((NF1, 2 * NB, CB), jnp.float32),
        pltpu.VMEM((NCB, S, CB), jnp.float32),
    ]
    out = pl.pallas_call(
        _kernel,
        grid=(NCB + NRB,),
        in_specs=in_specs,
        out_specs=out_spec,
        out_shape=jax.ShapeDtypeStruct((S, D), jnp.bfloat16),
        scratch_shapes=scratch,
        compiler_params=pltpu.CompilerParams(
            dimension_semantics=("arbitrary",),
            vmem_limit_bytes=100 * 1024 * 1024,
        ),
    )(q, k, v, sk, A_ssm_k, sd, B_w1, B_w2, mf, mi)
    return out.reshape(1, S, D)
```

```python
import math

import numpy as np
import jax
import jax.numpy as jnp
import jax.experimental.pallas as pl
import jax.experimental.pallas.tpu as pltpu

S = 2048
D = 448
F = 1792
L = 2 * S
NB = 128
NA = L // NB
NF1 = NA // 2 + 1
CR = 224
NCB = D // CR
TB = 512
NTB = S // TB
EPS = 1e-5


def _add(a, b):
    if a is None:
        return b
    if b is None:
        return a
    return a + b


def _sub(a, b):
    if b is None:
        return a
    if a is None:
        return -b
    return a - b


def _mulc(a, c):
    if a is None or c == 0.0:
        return None
    if c == 1.0:
        return a
    if c == -1.0:
        return -a
    return a * c


def _cmul_const(z, wr, wi):
    zr, zi = z
    if abs(wr) < 1e-12:
        wr = 0.0
    if abs(wi) < 1e-12:
        wi = 0.0
    if abs(abs(wr) - 1) < 1e-12:
        wr = math.copysign(1.0, wr)
    if abs(abs(wi) - 1) < 1e-12:
        wi = math.copysign(1.0, wi)
    re = _sub(_mulc(zr, wr), _mulc(zi, wi))
    im = _add(_mulc(zr, wi), _mulc(zi, wr))
    return (re, im)


def _rdft(x):
    n = len(x)
    if n == 1:
        return [(x[0], None)]
    if n == 2:
        return [(_add(x[0], x[1]), None), (_sub(x[0], x[1]), None)]
    e = _rdft(x[0::2])
    o = _rdft(x[1::2])
    out = [None] * (n // 2 + 1)
    for k in range(n // 4 + 1):
        t = _cmul_const(o[k], math.cos(2 * math.pi * k / n),
                        -math.sin(2 * math.pi * k / n))
        out[k] = (_add(e[k][0], t[0]), _add(e[k][1], t[1]))
        if n // 2 - k != k:
            out[n // 2 - k] = (_sub(e[k][0], t[0]), _sub(t[1], e[k][1]))
    return out


def _irdft(x, n, need):
    if n == 1:
        return [x[0][0]]
    if n == 2:
        out = [_add(x[0][0], x[1][0])]
        if need > 1:
            out.append(_sub(x[0][0], x[1][0]))
        return out
    e = [None] * (n // 4 + 1)
    o = [None] * (n // 4 + 1)
    for k in range(n // 4 + 1):
        a = x[k]
        b = x[n // 2 - k]
        e[k] = (_add(a[0], b[0]), _sub(a[1], b[1]))
        d = (_sub(a[0], b[0]), _add(a[1], b[1]))
        o[k] = _cmul_const(d, math.cos(2 * math.pi * k / n),
                           math.sin(2 * math.pi * k / n))
    ne = (need + 1) // 2
    no = need // 2
    xe = _irdft(e, n // 2, ne)
    xo = _irdft(o, n // 2, no) if no > 0 else []
    return [xe[i // 2] if i % 2 == 0 else xo[i // 2] for i in range(need)]


def _dft_tables():
    b = np.arange(NB)
    th = 2.0 * np.pi * ((b[:, None] * b[None, :]) % NB) / NB
    dft = np.stack([np.cos(th), np.sin(th)]).astype(np.float32)
    f1 = np.arange(NF1)
    th = 2.0 * np.pi * ((b[:, None] * f1[None, :]) % L) / L
    tw = np.zeros((2, NB, NB), np.float32)
    tw[0, :, :NF1] = np.cos(th)
    tw[1, :, :NF1] = np.sin(th)
    return dft, tw


def _kernel(q_ref, k_ref, v_ref, sk_ref, hk_ref, sd_ref, w1_ref, w2_ref,
            dft_ref, tw_ref, o_ref,
            wf_ref, wi_ref, w1t_ref, par_ref, u_ref, g_ref, p_ref, y_ref):
    step = pl.program_id(0)
    f32 = jnp.float32
    bf16 = jnp.bfloat16

    @pl.when(step == 0)
    def _tables():
        dc = dft_ref[0]
        ds_ = dft_ref[1]
        tc_all = tw_ref[0]
        ts_all = tw_ref[1]
        for f1 in range(NF1):
            tc = tc_all[:, f1:f1 + 1]
            ts = ts_all[:, f1:f1 + 1]
            c = tc * dc - ts * ds_
            s = ts * dc + tc * ds_
            wf_ref[f1, pl.ds(0, NB), pl.ds(0, NB)] = c.astype(bf16)
            wf_ref[f1, pl.ds(0, NB), pl.ds(NB, NB)] = (-s).astype(bf16)
            wf_ref[f1, pl.ds(NB, NB), pl.ds(0, NB)] = s.astype(bf16)
            wf_ref[f1, pl.ds(NB, NB), pl.ds(NB, NB)] = c.astype(bf16)
            ct = c.T * (1.0 / L)
            st = s.T * (1.0 / L)
            wi_ref[f1, pl.ds(0, NB), pl.ds(0, NB)] = ct.astype(bf16)
            wi_ref[f1, pl.ds(0, NB), pl.ds(NB, NB)] = st.astype(bf16)
            wi_ref[f1, pl.ds(NB, NB), pl.ds(0, NB)] = (-st).astype(bf16)
            wi_ref[f1, pl.ds(NB, NB), pl.ds(NB, NB)] = ct.astype(bf16)
        w1t_ref[...] = w1_ref[...].astype(f32).T.astype(bf16)
        par = jnp.concatenate(
            [sk_ref[...].astype(f32), sd_ref[...].astype(f32),
             jnp.zeros((3, D), f32)], axis=0)
        par_ref[...] = par.T

    @pl.when(step < NCB)
    def _conv():
        c0 = pl.multiple_of(step * CR, 8)
        par = par_ref[pl.ds(c0, CR), :]
        sk = par[:, 0:4]
        sd = par[:, 4:5]
        k = k_ref[...].astype(f32)
        lane = jax.lax.broadcasted_iota(jnp.int32, (CR, S), 1)
        ks = k * sk[:, 0:1]
        for j in range(1, 4):
            kj = jnp.where(lane >= j, pltpu.roll(k, j, 1), 0.0)
            ks = ks + kj * sk[:, j:j + 1]
        u_ref[pl.ds(0, CR), :] = ks * v_ref[...].astype(f32)
        u_ref[pl.ds(CR, CR), :] = hk_ref[...].astype(f32)

        def s1_body(r, carry):
            r8 = pl.multiple_of(r * 8, 8)
            xs = [u_ref[pl.ds(r8, 8), pl.ds(NB * a, NB)]
                  for a in range(NA // 2)]
            xs = xs + [None] * (NA // 2)
            g = _rdft(xs)
            for f1 in range(NF1):
                gr, gi = g[f1]
                if gi is None:
                    gi = jnp.zeros((8, NB), f32)
                g_ref[f1, pl.ds(r8, 8), pl.ds(0, NB)] = gr
                g_ref[f1, pl.ds(r8, 8), pl.ds(NB, NB)] = gi
            return carry

        jax.lax.fori_loop(0, 2 * CR // 8, s1_body, 0)

        for f1 in range(NF1):
            x = jnp.dot(g_ref[f1].astype(bf16), wf_ref[f1],
                        preferred_element_type=f32)
            xr, xi = x[:CR, :NB], x[:CR, NB:]
            hr, hi = x[CR:, :NB], x[CR:, NB:]
            yr = xr * hr - xi * hi
            yi = xr * hi + xi * hr
            yy = jnp.concatenate([yr, yi], axis=1).astype(bf16)
            p_ref[f1] = jnp.dot(yy, wi_ref[f1], preferred_element_type=f32)

        u_ref[pl.ds(CR, CR), pl.ds(0, NB)] = jnp.broadcast_to(sd, (CR, NB))

        def i1_body(r, carry):
            r8 = pl.multiple_of(r * 8, 8)
            xs = [(p_ref[f1, pl.ds(r8, 8), pl.ds(0, NB)],
                   p_ref[f1, pl.ds(r8, 8), pl.ds(NB, NB)])
                  for f1 in range(NF1)]
            y = _irdft(xs, NA, NA // 2)
            sdb = u_ref[pl.ds(CR + r8, 8), pl.ds(0, NB)]
            for a in range(NA // 2):
                col = pl.ds(NB * a, NB)
                yc = y[a].astype(bf16).astype(f32)
                y_ref[step, pl.ds(r8, 8), col] = (
                    yc + u_ref[pl.ds(r8, 8), col] * sdb)
            return carry

        jax.lax.fori_loop(0, CR // 8, i1_body, 0)

    @pl.when(step >= NCB)
    def _ffn():
        t0 = pl.multiple_of((step - NCB) * TB, TB)
        x = q_ref[...].astype(f32)
        mean = jnp.mean(x, axis=0, keepdims=True)
        xc = x - mean
        var = jnp.mean(xc * xc, axis=0, keepdims=True)
        xn = xc * jax.lax.rsqrt(var + EPS)
        xnb = xn.astype(bf16)
        h = jnp.dot(w1t_ref[...], xnb, preferred_element_type=f32)
        h = h * jax.nn.sigmoid(h)
        ffn = jnp.dot(w2_ref[...], h.astype(bf16), preferred_element_type=f32)
        cols = pl.ds(t0, TB)
        y = jnp.concatenate([y_ref[c, :, cols] for c in range(NCB)], axis=0)
        o_ref[...] = (x + xnb.astype(f32) * y + ffn).astype(o_ref.dtype)


@jax.jit
def pallas_parallel_sum__ssm_conv_h3__dense_activation_silu__prompt_kernel(
    A_q: jax.Array,
    A_k: jax.Array,
    A_v: jax.Array,
    A_shift_k: jax.Array,
    A_ssm_k: jax.Array,
    A_ssm_D: jax.Array,
    B_x: jax.Array,
    B_w1: jax.Array,
    B_w2: jax.Array,
):
    del B_x
    qt = A_q.reshape(S, D).T
    kt = A_k.reshape(S, D).T
    vt = A_v.reshape(S, D).T
    sk = A_shift_k.T
    sd = A_ssm_D.reshape(1, D)
    w2t = B_w2.T
    dft_np, tw_np = _dft_tables()
    dft = jnp.asarray(dft_np)
    tw = jnp.asarray(tw_np)

    cidx = lambda i: jnp.minimum(i, NCB - 1)
    tidx = lambda i: jnp.maximum(i - NCB, 0)

    in_specs = [
        pl.BlockSpec((D, TB), lambda i: (0, tidx(i))),
        pl.BlockSpec((CR, S), lambda i: (cidx(i), 0)),
        pl.BlockSpec((CR, S), lambda i: (cidx(i), 0)),
        pl.BlockSpec((4, D), lambda i: (0, 0)),
        pl.BlockSpec((CR, S), lambda i: (cidx(i), 0)),
        pl.BlockSpec((1, D), lambda i: (0, 0)),
        pl.BlockSpec((D, F), lambda i: (0, 0)),
        pl.BlockSpec((D, F), lambda i: (0, 0)),
        pl.BlockSpec((2, NB, NB), lambda i: (0, 0, 0)),
        pl.BlockSpec((2, NB, NB), lambda i: (0, 0, 0)),
    ]
    out_spec = pl.BlockSpec((D, TB), lambda i: (0, tidx(i)))
    scratch = [
        pltpu.VMEM((NF1, 2 * NB, 2 * NB), jnp.bfloat16),
        pltpu.VMEM((NF1, 2 * NB, 2 * NB), jnp.bfloat16),
        pltpu.VMEM((F, D), jnp.bfloat16),
        pltpu.VMEM((D, 8), jnp.float32),
        pltpu.VMEM((2 * CR, S), jnp.float32),
        pltpu.VMEM((NF1, 2 * CR, 2 * NB), jnp.float32),
        pltpu.VMEM((NF1, CR, 2 * NB), jnp.float32),
        pltpu.VMEM((NCB, CR, S), jnp.float32),
    ]
    out = pl.pallas_call(
        _kernel,
        grid=(NCB + NTB,),
        in_specs=in_specs,
        out_specs=out_spec,
        out_shape=jax.ShapeDtypeStruct((D, S), jnp.bfloat16),
        scratch_shapes=scratch,
        compiler_params=pltpu.CompilerParams(
            dimension_semantics=("arbitrary",),
            vmem_limit_bytes=100 * 1024 * 1024,
        ),
    )(qt, kt, vt, sk, A_ssm_k, sd, B_w1, w2t, dft, tw)
    return out.T.reshape(1, S, D)
```

```python
import math

import numpy as np
import jax
import jax.numpy as jnp
import jax.experimental.pallas as pl
import jax.experimental.pallas.tpu as pltpu

S = 2048
D = 448
F = 1792
L = 2 * S
NB = 128
NA = L // NB
NF1 = NA // 2 + 1
CR = 224
NCB = D // CR
TB = 512
NTB = S // TB
FC = 256
EPS = 1e-5


def _add(a, b):
    if a is None:
        return b
    if b is None:
        return a
    return a + b


def _sub(a, b):
    if b is None:
        return a
    if a is None:
        return -b
    return a - b


def _mulc(a, c):
    if a is None or c == 0.0:
        return None
    if c == 1.0:
        return a
    if c == -1.0:
        return -a
    return a * c


def _cmul_const(z, wr, wi):
    zr, zi = z
    if abs(wr) < 1e-12:
        wr = 0.0
    if abs(wi) < 1e-12:
        wi = 0.0
    if abs(abs(wr) - 1) < 1e-12:
        wr = math.copysign(1.0, wr)
    if abs(abs(wi) - 1) < 1e-12:
        wi = math.copysign(1.0, wi)
    re = _sub(_mulc(zr, wr), _mulc(zi, wi))
    im = _add(_mulc(zr, wi), _mulc(zi, wr))
    return (re, im)


def _rdft(x):
    n = len(x)
    if n == 1:
        return [(x[0], None)]
    if n == 2:
        return [(_add(x[0], x[1]), None), (_sub(x[0], x[1]), None)]
    e = _rdft(x[0::2])
    o = _rdft(x[1::2])
    out = [None] * (n // 2 + 1)
    for k in range(n // 4 + 1):
        t = _cmul_const(o[k], math.cos(2 * math.pi * k / n),
                        -math.sin(2 * math.pi * k / n))
        out[k] = (_add(e[k][0], t[0]), _add(e[k][1], t[1]))
        if n // 2 - k != k:
            out[n // 2 - k] = (_sub(e[k][0], t[0]), _sub(t[1], e[k][1]))
    return out


def _irdft(x, n, need):
    if n == 1:
        return [x[0][0]]
    if n == 2:
        out = [_add(x[0][0], x[1][0])]
        if need > 1:
            out.append(_sub(x[0][0], x[1][0]))
        return out
    e = [None] * (n // 4 + 1)
    o = [None] * (n // 4 + 1)
    for k in range(n // 4 + 1):
        a = x[k]
        b = x[n // 2 - k]
        e[k] = (_add(a[0], b[0]), _sub(a[1], b[1]))
        d = (_sub(a[0], b[0]), _add(a[1], b[1]))
        o[k] = _cmul_const(d, math.cos(2 * math.pi * k / n),
                           math.sin(2 * math.pi * k / n))
    ne = (need + 1) // 2
    no = need // 2
    xe = _irdft(e, n // 2, ne)
    xo = _irdft(o, n // 2, no) if no > 0 else []
    return [xe[i // 2] if i % 2 == 0 else xo[i // 2] for i in range(need)]


def _dft_tables():
    b = np.arange(NB)
    th = 2.0 * np.pi * ((b[:, None] * b[None, :]) % NB) / NB
    dft = np.stack([np.cos(th), np.sin(th)]).astype(np.float32)
    f1 = np.arange(NF1)
    th = 2.0 * np.pi * ((b[:, None] * f1[None, :]) % L) / L
    tw = np.zeros((2, NB, NB), np.float32)
    tw[0, :, :NF1] = np.cos(th)
    tw[1, :, :NF1] = np.sin(th)
    return dft, tw


def _kernel(q_ref, k_ref, v_ref, sk_ref, hk_ref, sd_ref, w1_hbm, w2_hbm,
            dft_ref, tw_ref, o_ref,
            wf_ref, wi_ref, w1_ref, w2_ref, w1t_ref, par_ref, u_ref, g_ref,
            p_ref, y_ref, acc_ref, base_ref, xn_ref, sem):
    step = pl.program_id(0)
    f32 = jnp.float32
    bf16 = jnp.bfloat16
    NCH = F // FC

    def w_copies():
        return (pltpu.make_async_copy(w1_hbm, w1_ref, sem.at[0]),
                pltpu.make_async_copy(w2_hbm, w2_ref, sem.at[1]))

    def tables():
        dc = dft_ref[0]
        ds_ = dft_ref[1]
        tc_all = tw_ref[0]
        ts_all = tw_ref[1]
        for f1 in range(NF1):
            tc = tc_all[:, f1:f1 + 1]
            ts = ts_all[:, f1:f1 + 1]
            c = tc * dc - ts * ds_
            s = ts * dc + tc * ds_
            wf_ref[f1, pl.ds(0, NB), pl.ds(0, NB)] = c.astype(bf16)
            wf_ref[f1, pl.ds(0, NB), pl.ds(NB, NB)] = (-s).astype(bf16)
            wf_ref[f1, pl.ds(NB, NB), pl.ds(0, NB)] = s.astype(bf16)
            wf_ref[f1, pl.ds(NB, NB), pl.ds(NB, NB)] = c.astype(bf16)
            ct = c.T * (1.0 / L)
            st = s.T * (1.0 / L)
            wi_ref[f1, pl.ds(0, NB), pl.ds(0, NB)] = ct.astype(bf16)
            wi_ref[f1, pl.ds(0, NB), pl.ds(NB, NB)] = st.astype(bf16)
            wi_ref[f1, pl.ds(NB, NB), pl.ds(0, NB)] = (-st).astype(bf16)
            wi_ref[f1, pl.ds(NB, NB), pl.ds(NB, NB)] = ct.astype(bf16)
        par = jnp.concatenate(
            [sk_ref[...].astype(f32), sd_ref[...].astype(f32),
             jnp.zeros((3, D), f32)], axis=0)
        par_ref[...] = par.T

    def kv_stage(c):
        par = par_ref[pl.ds(c * CR, CR), :]
        k = k_ref[...].astype(f32)
        lane = jax.lax.broadcasted_iota(jnp.int32, (CR, S), 1)
        ks = k * par[:, 0:1]
        for j in range(1, 4):
            kj = jnp.where(lane >= j, pltpu.roll(k, j, 1), 0.0)
            ks = ks + kj * par[:, j:j + 1]
        u_ref[c, pl.ds(0, CR), :] = ks * v_ref[...].astype(f32)
        u_ref[c, pl.ds(CR, CR), :] = hk_ref[...].astype(f32)

    def s1_rows(c, r8):
        xs = [u_ref[c, pl.ds(r8, 8), pl.ds(NB * a, NB)]
              for a in range(NA // 2)]
        xs = xs + [None] * (NA // 2)
        g = _rdft(xs)
        for f1 in range(NF1):
            gr, gi = g[f1]
            if gi is None:
                gi = jnp.zeros((8, NB), f32)
            g_ref[f1, pl.ds(r8, 8), pl.ds(0, NB)] = gr
            g_ref[f1, pl.ds(r8, 8), pl.ds(NB, NB)] = gi

    def spec_stage():
        for f1 in range(NF1):
            x = jnp.dot(g_ref[f1].astype(bf16), wf_ref[f1],
                        preferred_element_type=f32)
            xr, xi = x[:CR, :NB], x[:CR, NB:]
            hr, hi = x[CR:, :NB], x[CR:, NB:]
            yr = xr * hr - xi * hi
            yi = xr * hi + xi * hr
            yy = jnp.concatenate([yr, yi], axis=1).astype(bf16)
            p_ref[f1] = jnp.dot(yy, wi_ref[f1], preferred_element_type=f32)

    def i1_rows(c, r8):
        xs = [(p_ref[f1, pl.ds(r8, 8), pl.ds(0, NB)],
               p_ref[f1, pl.ds(r8, 8), pl.ds(NB, NB)])
              for f1 in range(NF1)]
        y = _irdft(xs, NA, NA // 2)
        sd = par_ref[pl.ds(c * CR + r8, 8), :][:, 4:5]
        for a in range(NA // 2):
            col = pl.ds(NB * a, NB)
            yc = y[a].astype(bf16).astype(f32)
            y_ref[pl.ds(c * CR + r8, 8), col] = (
                yc + u_ref[c, pl.ds(r8, 8), col] * sd)

    def layernorm(tb):
        x = q_ref[...].astype(f32)
        mean = jnp.mean(x, axis=0, keepdims=True)
        xc = x - mean
        var = jnp.mean(xc * xc, axis=0, keepdims=True)
        xn = xc * jax.lax.rsqrt(var + EPS)
        cols = pl.ds(tb * TB, TB)
        xn_ref[:, cols] = xn.astype(bf16)
        base_ref[:, cols] = x

    def ffn_chunk(tb, i):
        f0 = pl.multiple_of(i * FC, FC)
        xnb = xn_ref[:, pl.ds(tb * TB, TB)]
        h = jnp.dot(w1t_ref[pl.ds(f0, FC), :], xnb,
                    preferred_element_type=f32)
        h = h * jax.nn.sigmoid(h)
        part = jnp.dot(w2_ref[:, pl.ds(f0, FC)], h.astype(bf16),
                       preferred_element_type=f32)
        cols = pl.ds(tb * TB, TB)
        base_ref[:, cols] = base_ref[:, cols] + part

    def combine(rows, cols):
        o_ref[rows, cols] = (
            base_ref[rows, cols]
            + xn_ref[rows, cols].astype(f32) * y_ref[rows, cols]
        ).astype(o_ref.dtype)

    RS = 2 * CR // NCH
    RI = CR // NCH

    @pl.when(step == 0)
    def _():
        for cp in w_copies():
            cp.start()
        with jax.named_scope("tables"):
            tables()
        with jax.named_scope("kv0"):
            kv_stage(0)
            layernorm(0)
        for cp in w_copies():
            cp.wait()
        w1t_ref[...] = w1_ref[...].astype(f32).T.astype(bf16)

        def body(i, carry):
            for g in range(RS // 8):
                s1_rows(0, pl.multiple_of(i * RS + g * 8, 8))
            ffn_chunk(0, i)
            return carry

        with jax.named_scope("loop0"):
            jax.lax.fori_loop(0, NCH, body, 0)

    @pl.when(step == 1)
    def _():
        with jax.named_scope("spec0"):
            spec_stage()
            kv_stage(1)
            layernorm(1)

        def body(i, carry):
            for g in range(RI // 8):
                i1_rows(0, pl.multiple_of(i * RI + g * 8, 8))
            for g in range(RS // 8):
                s1_rows(1, pl.multiple_of(i * RS + g * 8, 8))
            ffn_chunk(1, i)
            return carry

        with jax.named_scope("loop1"):
            jax.lax.fori_loop(0, NCH, body, 0)

    @pl.when(step == 2)
    def _():
        with jax.named_scope("spec1"):
            spec_stage()
            layernorm(2)

        def body(i, carry):
            for g in range(RI // 8):
                i1_rows(1, pl.multiple_of(i * RI + g * 8, 8))
            ffn_chunk(2, i)
            return carry

        with jax.named_scope("loop2"):
            jax.lax.fori_loop(0, NCH, body, 0)

    @pl.when(step == 3)
    def _():
        layernorm(3)
        rc = D // NCH

        def body(i, carry):
            combine(pl.ds(pl.multiple_of(i * rc, 16), rc),
                    pl.ds(0, (NTB - 1) * TB))
            ffn_chunk(3, i)
            return carry

        with jax.named_scope("loop3"):
            jax.lax.fori_loop(0, NCH, body, 0)
        combine(pl.ds(0, D), pl.ds((NTB - 1) * TB, TB))


@jax.jit
def pallas_parallel_sum__ssm_conv_h3__dense_activation_silu__prompt_kernel(
    A_q: jax.Array,
    A_k: jax.Array,
    A_v: jax.Array,
    A_shift_k: jax.Array,
    A_ssm_k: jax.Array,
    A_ssm_D: jax.Array,
    B_x: jax.Array,
    B_w1: jax.Array,
    B_w2: jax.Array,
):
    del B_x
    qt = A_q.reshape(S, D).T
    kt = A_k.reshape(S, D).T
    vt = A_v.reshape(S, D).T
    sk = A_shift_k.T
    sd = A_ssm_D.reshape(1, D)
    w2t = B_w2.T
    dft_np, tw_np = _dft_tables()
    dft = jnp.asarray(dft_np)
    tw = jnp.asarray(tw_np)

    cidx = lambda i: jnp.minimum(i, NCB - 1)

    in_specs = [
        pl.BlockSpec((D, TB), lambda i: (0, i)),
        pl.BlockSpec((CR, S), lambda i: (cidx(i), 0)),
        pl.BlockSpec((CR, S), lambda i: (cidx(i), 0)),
        pl.BlockSpec((4, D), lambda i: (0, 0)),
        pl.BlockSpec((CR, S), lambda i: (cidx(i), 0)),
        pl.BlockSpec((1, D), lambda i: (0, 0)),
        pl.BlockSpec(memory_space=pl.ANY),
        pl.BlockSpec(memory_space=pl.ANY),
        pl.BlockSpec((2, NB, NB), lambda i: (0, 0, 0)),
        pl.BlockSpec((2, NB, NB), lambda i: (0, 0, 0)),
    ]
    out_spec = pl.BlockSpec((D, S), lambda i: (0, 0))
    scratch = [
        pltpu.VMEM((NF1, 2 * NB, 2 * NB), jnp.bfloat16),
        pltpu.VMEM((NF1, 2 * NB, 2 * NB), jnp.bfloat16),
        pltpu.VMEM((D, F), jnp.bfloat16),
        pltpu.VMEM((D, F), jnp.bfloat16),
        pltpu.VMEM((F, D), jnp.bfloat16),
        pltpu.VMEM((D, 8), jnp.float32),
        pltpu.VMEM((NCB, 2 * CR, S), jnp.float32),
        pltpu.VMEM((NF1, 2 * CR, 2 * NB), jnp.float32),
        pltpu.VMEM((NF1, CR, 2 * NB), jnp.float32),
        pltpu.VMEM((D, S), jnp.float32),
        pltpu.VMEM((D, TB), jnp.float32),
        pltpu.VMEM((D, S), jnp.float32),
        pltpu.VMEM((D, S), jnp.bfloat16),
        pltpu.SemaphoreType.DMA((2,)),
    ]
    out = pl.pallas_call(
        _kernel,
        grid=(NTB,),
        in_specs=in_specs,
        out_specs=out_spec,
        out_shape=jax.ShapeDtypeStruct((D, S), jnp.bfloat16),
        scratch_shapes=scratch,
        compiler_params=pltpu.CompilerParams(
            dimension_semantics=("arbitrary",),
            vmem_limit_bytes=100 * 1024 * 1024,
        ),
    )(qt, kt, vt, sk, A_ssm_k, sd, B_w1, w2t, dft, tw)
    return out.T.reshape(1, S, D)
```

```python
import math

import numpy as np
import jax
import jax.numpy as jnp
import jax.experimental.pallas as pl
import jax.experimental.pallas.tpu as pltpu

S = 2048
D = 448
F = 1792
L = 2 * S
NB = 128
NA = L // NB
NF1 = NA // 2 + 1
CR = 224
NCB = D // CR
TB = 512
NTB = S // TB
FC = 256
EPS = 1e-5


def _add(a, b):
    if a is None:
        return b
    if b is None:
        return a
    return a + b


def _sub(a, b):
    if b is None:
        return a
    if a is None:
        return -b
    return a - b


def _mulc(a, c):
    if a is None or c == 0.0:
        return None
    if c == 1.0:
        return a
    if c == -1.0:
        return -a
    return a * c


def _cmul_const(z, wr, wi):
    zr, zi = z
    if abs(wr) < 1e-12:
        wr = 0.0
    if abs(wi) < 1e-12:
        wi = 0.0
    if abs(abs(wr) - 1) < 1e-12:
        wr = math.copysign(1.0, wr)
    if abs(abs(wi) - 1) < 1e-12:
        wi = math.copysign(1.0, wi)
    re = _sub(_mulc(zr, wr), _mulc(zi, wi))
    im = _add(_mulc(zr, wi), _mulc(zi, wr))
    return (re, im)


def _rdft(x):
    n = len(x)
    if n == 1:
        return [(x[0], None)]
    if n == 2:
        return [(_add(x[0], x[1]), None), (_sub(x[0], x[1]), None)]
    e = _rdft(x[0::2])
    o = _rdft(x[1::2])
    out = [None] * (n // 2 + 1)
    for k in range(n // 4 + 1):
        t = _cmul_const(o[k], math.cos(2 * math.pi * k / n),
                        -math.sin(2 * math.pi * k / n))
        out[k] = (_add(e[k][0], t[0]), _add(e[k][1], t[1]))
        if n // 2 - k != k:
            out[n // 2 - k] = (_sub(e[k][0], t[0]), _sub(t[1], e[k][1]))
    return out


def _irdft(x, n, need):
    if n == 1:
        return [x[0][0]]
    if n == 2:
        out = [_add(x[0][0], x[1][0])]
        if need > 1:
            out.append(_sub(x[0][0], x[1][0]))
        return out
    e = [None] * (n // 4 + 1)
    o = [None] * (n // 4 + 1)
    for k in range(n // 4 + 1):
        a = x[k]
        b = x[n // 2 - k]
        e[k] = (_add(a[0], b[0]), _sub(a[1], b[1]))
        d = (_sub(a[0], b[0]), _add(a[1], b[1]))
        o[k] = _cmul_const(d, math.cos(2 * math.pi * k / n),
                           math.sin(2 * math.pi * k / n))
    ne = (need + 1) // 2
    no = need // 2
    xe = _irdft(e, n // 2, ne)
    xo = _irdft(o, n // 2, no) if no > 0 else []
    return [xe[i // 2] if i % 2 == 0 else xo[i // 2] for i in range(need)]


def _dft_tables():
    b = np.arange(NB)
    th = 2.0 * np.pi * ((b[:, None] * b[None, :]) % NB) / NB
    dft = np.stack([np.cos(th), np.sin(th)]).astype(np.float32)
    f1 = np.arange(NF1)
    th = 2.0 * np.pi * ((b[:, None] * f1[None, :]) % L) / L
    tw = np.zeros((2, NB, NB), np.float32)
    tw[0, :, :NF1] = np.cos(th)
    tw[1, :, :NF1] = np.sin(th)
    return dft, tw


def _kernel(q_hbm, k_hbm, v_hbm, sk_ref, hk_hbm, sd_ref, w1_hbm, w2_hbm,
            dft_ref, tw_ref, o_hbm,
            q_ref, k_ref, v_ref, hk_ref, w1_ref, w2_ref, o_ref,
            wf_ref, wi_ref, w1t_ref, par_ref, u_ref, g_ref, p_ref, y_ref,
            hb_ref, base_ref, xn_ref, sem, osem):
    f32 = jnp.float32
    bf16 = jnp.bfloat16
    NCH = F // FC
    HALF = D // 2

    def half_copy(src, dst, h, s):
        rows = pl.ds(h * HALF, HALF)
        return pltpu.make_async_copy(src.at[rows, :], dst.at[rows, :],
                                     sem.at[s])

    cp_kvh = [[half_copy(k_hbm, k_ref, h, 3 * h + 0),
               half_copy(v_hbm, v_ref, h, 3 * h + 1),
               half_copy(hk_hbm, hk_ref, h, 3 * h + 2)] for h in range(2)]
    cp_q = pltpu.make_async_copy(q_hbm, q_ref, sem.at[6])
    cp_w1 = pltpu.make_async_copy(w1_hbm, w1_ref, sem.at[7])
    cp_w2 = pltpu.make_async_copy(w2_hbm, w2_ref, sem.at[8])
    for cp in cp_kvh[0][:2] + [cp_w1, cp_q, cp_w2, cp_kvh[0][2]] + cp_kvh[1]:
        cp.start()

    def tables():
        dc = dft_ref[0]
        ds_ = dft_ref[1]
        tc_all = tw_ref[0]
        ts_all = tw_ref[1]
        for f1 in range(NF1):
            tc = tc_all[:, f1:f1 + 1]
            ts = ts_all[:, f1:f1 + 1]
            c = tc * dc - ts * ds_
            s = ts * dc + tc * ds_
            wf_ref[f1, pl.ds(0, NB), pl.ds(0, NB)] = c.astype(bf16)
            wf_ref[f1, pl.ds(0, NB), pl.ds(NB, NB)] = (-s).astype(bf16)
            wf_ref[f1, pl.ds(NB, NB), pl.ds(0, NB)] = s.astype(bf16)
            wf_ref[f1, pl.ds(NB, NB), pl.ds(NB, NB)] = c.astype(bf16)
            ct = c.T * (1.0 / L)
            st = s.T * (1.0 / L)
            wi_ref[f1, pl.ds(0, NB), pl.ds(0, NB)] = ct.astype(bf16)
            wi_ref[f1, pl.ds(0, NB), pl.ds(NB, NB)] = st.astype(bf16)
            wi_ref[f1, pl.ds(NB, NB), pl.ds(0, NB)] = (-st).astype(bf16)
            wi_ref[f1, pl.ds(NB, NB), pl.ds(NB, NB)] = ct.astype(bf16)
        par = jnp.concatenate(
            [sk_ref[...].astype(f32), sd_ref[...].astype(f32),
             jnp.zeros((3, D), f32)], axis=0)
        par_ref[...] = par.T

    def kv_rows(r0, n):
        rows = pl.ds(r0, n)
        par = par_ref[rows, :]
        k = k_ref[rows, :].astype(f32)
        lane = jax.lax.broadcasted_iota(jnp.int32, (n, S), 1)
        ks = k * par[:, 0:1]
        for j in range(1, 4):
            kj = jnp.where(lane >= j, pltpu.roll(k, j, 1), 0.0)
            ks = ks + kj * par[:, j:j + 1]
        u_ref[rows, :] = ks * v_ref[rows, :].astype(f32)

    def s1_rows(src, r8, g8):
        xs = [src[pl.ds(r8, 8), pl.ds(NB * a, NB)].astype(f32)
              for a in range(NA // 2)]
        xs = xs + [None] * (NA // 2)
        g = _rdft(xs)
        for f1 in range(NF1):
            gr, gi = g[f1]
            if gi is None:
                gi = jnp.zeros((8, NB), f32)
            g_ref[f1, pl.ds(g8, 8), pl.ds(0, NB)] = gr
            g_ref[f1, pl.ds(g8, 8), pl.ds(NB, NB)] = gi

    def spec_stage():
        for f1 in range(NF1):
            x = jnp.dot(g_ref[f1].astype(bf16), wf_ref[f1],
                        preferred_element_type=f32)
            xr, xi = x[:D, :NB], x[:D, NB:]
            hr, hi = x[D:, :NB], x[D:, NB:]
            yr = xr * hr - xi * hi
            yi = xr * hi + xi * hr
            yy = jnp.concatenate([yr, yi], axis=1).astype(bf16)
            p_ref[f1] = jnp.dot(yy, wi_ref[f1], preferred_element_type=f32)

    def i1_rows(r8):
        rows = pl.ds(r8, 8)
        xs = [(p_ref[f1, rows, pl.ds(0, NB)], p_ref[f1, rows, pl.ds(NB, NB)])
              for f1 in range(NF1)]
        y = _irdft(xs, NA, NA // 2)
        sd = par_ref[rows, :][:, 4:5]
        for a in range(NA // 2):
            col = pl.ds(NB * a, NB)
            yc = y[a].astype(bf16).astype(f32)
            y_ref[rows, col] = yc + u_ref[rows, col] * sd

    def layernorm(tb):
        cols = pl.ds(tb * TB, TB)
        x = q_ref[:, cols].astype(f32)
        mean = jnp.mean(x, axis=0, keepdims=True)
        xc = x - mean
        var = jnp.mean(xc * xc, axis=0, keepdims=True)
        xn = xc * jax.lax.rsqrt(var + EPS)
        xn_ref[:, cols] = xn.astype(bf16)
        base_ref[:, cols] = x

    def ffn_up(tb, i, slot):
        f0 = pl.multiple_of(i * FC, FC)
        h = jnp.dot(w1t_ref[pl.ds(f0, FC), :], xn_ref[:, pl.ds(tb * TB, TB)],
                    preferred_element_type=f32)
        hb_ref[slot] = (h * jax.nn.sigmoid(h)).astype(bf16)

    def ffn_down(tb, i, slot):
        f0 = pl.multiple_of(i * FC, FC)
        part = jnp.dot(w2_ref[:, pl.ds(f0, FC)], hb_ref[slot],
                       preferred_element_type=f32)
        cols = pl.ds(tb * TB, TB)
        base_ref[:, cols] = base_ref[:, cols] + part

    def combine(rows, cols):
        o_ref[rows, cols] = (
            base_ref[rows, cols]
            + xn_ref[rows, cols].astype(f32) * y_ref[rows, cols]
        ).astype(o_ref.dtype)

    def ffn_loop(tb, extra, name):
        def body(i, carry):
            slot = jax.lax.rem(i + tb * NCH, 2)
            extra(i)
            ffn_up(tb, i, slot)

            if tb == 0:
                @pl.when(i > 0)
                def _():
                    ffn_down(0, i - 1, 1 - slot)
            else:
                @pl.when(i > 0)
                def _():
                    ffn_down(tb, i - 1, 1 - slot)

                @pl.when(i == 0)
                def _():
                    ffn_down(tb - 1, NCH - 1, 1 - slot)
            return carry

        with jax.named_scope(name):
            jax.lax.fori_loop(0, NCH, body, 0)

    with jax.named_scope("tables"):
        tables()
    with jax.named_scope("pro"):
        cp_w1.wait()
        w1t_ref[...] = w1_ref[...].astype(f32).T.astype(bf16)
        cp_q.wait()
        layernorm(0)
        for cp in cp_kvh[0]:
            cp.wait()
        cp_w2.wait()

    CPI = D // (2 * NCH)

    def fwd_extra(base):
        def extra(i):
            r0 = pl.multiple_of(base + i * CPI, 8)
            kv_rows(r0, CPI)
            for g in range(CPI // 8):
                r8 = pl.multiple_of(r0 + g * 8, 8)
                s1_rows(u_ref, r8, r8)
                s1_rows(hk_ref, r8, pl.multiple_of(D + r8, 8))
        return extra

    ffn_loop(0, fwd_extra(0), "loop0")
    with jax.named_scope("ln1"):
        layernorm(1)
        for cp in cp_kvh[1]:
            cp.wait()
    ffn_loop(1, fwd_extra(HALF), "loop1")
    with jax.named_scope("spec"):
        spec_stage()
        layernorm(2)

    RI = D // NCH

    def inv_extra(i):
        for g in range(RI // 8):
            i1_rows(pl.multiple_of(i * RI + g * 8, 8))

    ffn_loop(2, inv_extra, "loop2")
    with jax.named_scope("ln3"):
        layernorm(3)

    def out_copy(rows, cols, s):
        return pltpu.make_async_copy(o_ref.at[rows, cols],
                                     o_hbm.at[rows, cols], osem.at[s])

    early = pl.ds(0, (NTB - 2) * TB)

    def comb_extra(i):
        rows = pl.ds(pl.multiple_of(i * RI, 16), RI)
        combine(rows, early)
        out_copy(rows, early, 0).start()

    ffn_loop(3, comb_extra, "loop3")
    with jax.named_scope("fin"):
        ffn_down(NTB - 1, NCH - 1, (NTB * NCH - 1) % 2)
        late = pl.ds((NTB - 2) * TB, 2 * TB)
        combine(pl.ds(0, D), late)
        cp_late = out_copy(pl.ds(0, D), late, 1)
        cp_late.start()
        out_copy(pl.ds(0, D), early, 0).wait()
        cp_late.wait()


@jax.jit
def pallas_parallel_sum__ssm_conv_h3__dense_activation_silu__prompt_kernel(
    A_q: jax.Array,
    A_k: jax.Array,
    A_v: jax.Array,
    A_shift_k: jax.Array,
    A_ssm_k: jax.Array,
    A_ssm_D: jax.Array,
    B_x: jax.Array,
    B_w1: jax.Array,
    B_w2: jax.Array,
):
    del B_x
    qt = A_q.reshape(S, D).T
    kt = A_k.reshape(S, D).T
    vt = A_v.reshape(S, D).T
    sk = A_shift_k.T
    sd = A_ssm_D.reshape(1, D)
    w2t = B_w2.T
    dft_np, tw_np = _dft_tables()
    dft = jnp.asarray(dft_np)
    tw = jnp.asarray(tw_np)

    hbm = pl.BlockSpec(memory_space=pl.ANY)
    vmem = pl.BlockSpec(memory_space=pltpu.VMEM)
    in_specs = [hbm, hbm, hbm, vmem, hbm, vmem, hbm, hbm, vmem, vmem]
    bf = jnp.bfloat16
    scratch = [
        pltpu.VMEM((D, S), bf),
        pltpu.VMEM((D, S), bf),
        pltpu.VMEM((D, S), bf),
        pltpu.VMEM((D, S), bf),
        pltpu.VMEM((D, F), bf),
        pltpu.VMEM((D, F), bf),
        pltpu.VMEM((D, S), bf),
        pltpu.VMEM((NF1, 2 * NB, 2 * NB), bf),
        pltpu.VMEM((NF1, 2 * NB, 2 * NB), bf),
        pltpu.VMEM((F, D), bf),
        pltpu.VMEM((D, 8), jnp.float32),
        pltpu.VMEM((D, S), jnp.float32),
        pltpu.VMEM((NF1, 2 * D, 2 * NB), jnp.float32),
        pltpu.VMEM((NF1, D, 2 * NB), jnp.float32),
        pltpu.VMEM((D, S), jnp.float32),
        pltpu.VMEM((2, FC, TB), bf),
        pltpu.VMEM((D, S), jnp.float32),
        pltpu.VMEM((D, S), bf),
        pltpu.SemaphoreType.DMA((9,)),
        pltpu.SemaphoreType.DMA((2,)),
    ]
    out = pl.pallas_call(
        _kernel,
        in_specs=in_specs,
        out_specs=hbm,
        out_shape=jax.ShapeDtypeStruct((D, S), bf),
        scratch_shapes=scratch,
        compiler_params=pltpu.CompilerParams(
            vmem_limit_bytes=100 * 1024 * 1024,
        ),
    )(qt, kt, vt, sk, A_ssm_k, sd, B_w1, w2t, dft, tw)
    return out.T.reshape(1, S, D)
```

```python
import math

import numpy as np
import jax
import jax.numpy as jnp
import jax.experimental.pallas as pl
import jax.experimental.pallas.tpu as pltpu

S = 2048
D = 448
F = 1792
L = 2 * S
NB = 128
NA = L // NB
NF1 = NA // 2 + 1
CR = 224
NCB = D // CR
TB = 512
NTB = S // TB
FC = 256
EPS = 1e-5


def _add(a, b):
    if a is None:
        return b
    if b is None:
        return a
    return a + b


def _sub(a, b):
    if b is None:
        return a
    if a is None:
        return -b
    return a - b


def _mulc(a, c):
    if a is None or c == 0.0:
        return None
    if c == 1.0:
        return a
    if c == -1.0:
        return -a
    return a * c


def _cmul_const(z, wr, wi):
    zr, zi = z
    if abs(wr) < 1e-12:
        wr = 0.0
    if abs(wi) < 1e-12:
        wi = 0.0
    if abs(abs(wr) - 1) < 1e-12:
        wr = math.copysign(1.0, wr)
    if abs(abs(wi) - 1) < 1e-12:
        wi = math.copysign(1.0, wi)
    re = _sub(_mulc(zr, wr), _mulc(zi, wi))
    im = _add(_mulc(zr, wi), _mulc(zi, wr))
    return (re, im)


def _rdft(x):
    n = len(x)
    if n == 1:
        return [(x[0], None)]
    if n == 2:
        return [(_add(x[0], x[1]), None), (_sub(x[0], x[1]), None)]
    e = _rdft(x[0::2])
    o = _rdft(x[1::2])
    out = [None] * (n // 2 + 1)
    for k in range(n // 4 + 1):
        t = _cmul_const(o[k], math.cos(2 * math.pi * k / n),
                        -math.sin(2 * math.pi * k / n))
        out[k] = (_add(e[k][0], t[0]), _add(e[k][1], t[1]))
        if n // 2 - k != k:
            out[n // 2 - k] = (_sub(e[k][0], t[0]), _sub(t[1], e[k][1]))
    return out


def _irdft(x, n, need):
    if n == 1:
        return [x[0][0]]
    if n == 2:
        out = [_add(x[0][0], x[1][0])]
        if need > 1:
            out.append(_sub(x[0][0], x[1][0]))
        return out
    e = [None] * (n // 4 + 1)
    o = [None] * (n // 4 + 1)
    for k in range(n // 4 + 1):
        a = x[k]
        b = x[n // 2 - k]
        e[k] = (_add(a[0], b[0]), _sub(a[1], b[1]))
        d = (_sub(a[0], b[0]), _add(a[1], b[1]))
        o[k] = _cmul_const(d, math.cos(2 * math.pi * k / n),
                           math.sin(2 * math.pi * k / n))
    ne = (need + 1) // 2
    no = need // 2
    xe = _irdft(e, n // 2, ne)
    xo = _irdft(o, n // 2, no) if no > 0 else []
    return [xe[i // 2] if i % 2 == 0 else xo[i // 2] for i in range(need)]


def _dft_tables():
    b = np.arange(NB)
    th = 2.0 * np.pi * ((b[:, None] * b[None, :]) % NB) / NB
    dft = np.stack([np.cos(th), np.sin(th)]).astype(np.float32)
    f1 = np.arange(NF1)
    th = 2.0 * np.pi * ((b[:, None] * f1[None, :]) % L) / L
    tw = np.zeros((2, NB, NB), np.float32)
    tw[0, :, :NF1] = np.cos(th)
    tw[1, :, :NF1] = np.sin(th)
    return dft, tw


def _kernel(q_hbm, k_hbm, v_hbm, sk_ref, hk_hbm, sd_ref, w1_hbm, w2_hbm,
            dft_ref, tw_ref, o_hbm,
            q_ref, k_ref, v_ref, hk_ref, w1_ref, w2_ref, o_ref,
            wf_ref, wi_ref, w1t_ref, par_ref, u_ref, g_ref, p_ref, y_ref,
            hb_ref, base_ref, xn_ref, sem, osem):
    f32 = jnp.float32
    bf16 = jnp.bfloat16
    NCH = F // FC
    HALF = D // 2

    NIT = 2 * NCH
    CPI = D // NIT

    def kvh_copies(i):
        rows = pl.ds(i * CPI, CPI)
        return [pltpu.make_async_copy(src.at[rows, :], dst.at[rows, :],
                                      sem.at[3 * i + j])
                for j, (src, dst) in enumerate(
                    ((k_hbm, k_ref), (v_hbm, v_ref), (hk_hbm, hk_ref)))]

    def q_copy(tb):
        cols = pl.ds(tb * TB, TB)
        return pltpu.make_async_copy(q_hbm.at[:, cols], q_ref.at[:, cols],
                                     sem.at[3 * NIT + tb])

    cp_w1 = pltpu.make_async_copy(w1_hbm, w1_ref, sem.at[3 * NIT + NTB])
    cp_w2 = pltpu.make_async_copy(w2_hbm, w2_ref, sem.at[3 * NIT + NTB + 1])
    cp_w1.start()
    q_copy(0).start()
    for cp in kvh_copies(0):
        cp.start()
    cp_w2.start()
    for i in range(1, NIT):
        for cp in kvh_copies(i):
            cp.start()
        if i in (2, 5, 8):
            q_copy(1 + (i - 2) // 3).start()

    def tables():
        dc = dft_ref[0]
        ds_ = dft_ref[1]
        tc_all = tw_ref[0]
        ts_all = tw_ref[1]
        for f1 in range(NF1):
            tc = tc_all[:, f1:f1 + 1]
            ts = ts_all[:, f1:f1 + 1]
            c = tc * dc - ts * ds_
            s = ts * dc + tc * ds_
            wf_ref[f1, pl.ds(0, NB), pl.ds(0, NB)] = c.astype(bf16)
            wf_ref[f1, pl.ds(0, NB), pl.ds(NB, NB)] = (-s).astype(bf16)
            wf_ref[f1, pl.ds(NB, NB), pl.ds(0, NB)] = s.astype(bf16)
            wf_ref[f1, pl.ds(NB, NB), pl.ds(NB, NB)] = c.astype(bf16)
            ct = c.T * (1.0 / L)
            st = s.T * (1.0 / L)
            wi_ref[f1, pl.ds(0, NB), pl.ds(0, NB)] = ct.astype(bf16)
            wi_ref[f1, pl.ds(0, NB), pl.ds(NB, NB)] = st.astype(bf16)
            wi_ref[f1, pl.ds(NB, NB), pl.ds(0, NB)] = (-st).astype(bf16)
            wi_ref[f1, pl.ds(NB, NB), pl.ds(NB, NB)] = ct.astype(bf16)
        par = jnp.concatenate(
            [sk_ref[...].astype(f32), sd_ref[...].astype(f32),
             jnp.zeros((3, D), f32)], axis=0)
        par_ref[...] = par.T

    def kv_rows(r0, n):
        rows = pl.ds(r0, n)
        par = par_ref[rows, :]
        k = k_ref[rows, :].astype(f32)
        lane = jax.lax.broadcasted_iota(jnp.int32, (n, S), 1)
        ks = k * par[:, 0:1]
        for j in range(1, 4):
            kj = jnp.where(lane >= j, pltpu.roll(k, j, 1), 0.0)
            ks = ks + kj * par[:, j:j + 1]
        u_ref[rows, :] = ks * v_ref[rows, :].astype(f32)

    def s1_rows(src, r8, g8):
        xs = [src[pl.ds(r8, 8), pl.ds(NB * a, NB)].astype(f32)
              for a in range(NA // 2)]
        xs = xs + [None] * (NA // 2)
        g = _rdft(xs)
        for f1 in range(NF1):
            gr, gi = g[f1]
            if gi is None:
                gi = jnp.zeros((8, NB), f32)
            g_ref[f1, pl.ds(g8, 8), pl.ds(0, NB)] = gr
            g_ref[f1, pl.ds(g8, 8), pl.ds(NB, NB)] = gi

    def spec_stage():
        for f1 in range(NF1):
            x = jnp.dot(g_ref[f1].astype(bf16), wf_ref[f1],
                        preferred_element_type=f32)
            xr, xi = x[:D, :NB], x[:D, NB:]
            hr, hi = x[D:, :NB], x[D:, NB:]
            yr = xr * hr - xi * hi
            yi = xr * hi + xi * hr
            yy = jnp.concatenate([yr, yi], axis=1).astype(bf16)
            p_ref[f1] = jnp.dot(yy, wi_ref[f1], preferred_element_type=f32)

    def i1_rows(r8):
        rows = pl.ds(r8, 8)
        xs = [(p_ref[f1, rows, pl.ds(0, NB)], p_ref[f1, rows, pl.ds(NB, NB)])
              for f1 in range(NF1)]
        y = _irdft(xs, NA, NA // 2)
        sd = par_ref[rows, :][:, 4:5]
        for a in range(NA // 2):
            col = pl.ds(NB * a, NB)
            yc = y[a].astype(bf16).astype(f32)
            y_ref[rows, col] = yc + u_ref[rows, col] * sd

    def layernorm(tb):
        cols = pl.ds(tb * TB, TB)
        x = q_ref[:, cols].astype(f32)
        mean = jnp.mean(x, axis=0, keepdims=True)
        xc = x - mean
        var = jnp.mean(xc * xc, axis=0, keepdims=True)
        xn = xc * jax.lax.rsqrt(var + EPS)
        xn_ref[:, cols] = xn.astype(bf16)
        base_ref[:, cols] = x

    def ffn_up(tb, i, slot):
        f0 = pl.multiple_of(i * FC, FC)
        c0 = pl.multiple_of(tb * TB, TB)
        h = jnp.dot(w1t_ref[pl.ds(f0, FC), :], xn_ref[:, pl.ds(c0, TB)],
                    preferred_element_type=f32)
        hb_ref[slot] = (h * jax.nn.sigmoid(h)).astype(bf16)

    def ffn_down(tb, i, slot):
        f0 = pl.multiple_of(i * FC, FC)
        part = jnp.dot(w2_ref[:, pl.ds(f0, FC)], hb_ref[slot],
                       preferred_element_type=f32)
        cols = pl.ds(tb * TB, TB)
        base_ref[:, cols] = base_ref[:, cols] + part

    def combine(rows, cols):
        o_ref[rows, cols] = (
            base_ref[rows, cols]
            + xn_ref[rows, cols].astype(f32) * y_ref[rows, cols]
        ).astype(o_ref.dtype)

    def ffn_loop(tb, extra, name, n_it=NCH):
        def body(i, carry):
            n = tb * NCH + i
            slot = jax.lax.rem(n, 2)
            extra(i)
            nxt = n + 1
            tb2 = nxt // NCH
            ffn_up(tb2, nxt - tb2 * NCH, 1 - slot)
            ffn_down(tb, i, slot)
            return carry

        with jax.named_scope(name):
            jax.lax.fori_loop(0, n_it, body, 0)

    with jax.named_scope("tables"):
        tables()
    with jax.named_scope("pro"):
        cp_w1.wait()
        w1t_ref[...] = w1_ref[...].astype(f32).T.astype(bf16)
        q_copy(0).wait()
        layernorm(0)
        ffn_up(0, 0, 0)
        q_copy(1).wait()
        layernorm(1)
        cp_w2.wait()

    def fwd_extra(it0):
        def extra(i):
            it = it0 + i
            for cp in kvh_copies(it):
                cp.wait()
            r0 = pl.multiple_of(it * CPI, 8)
            kv_rows(r0, CPI)
            for g in range(CPI // 8):
                r8 = pl.multiple_of(r0 + g * 8, 8)
                s1_rows(u_ref, r8, r8)
                s1_rows(hk_ref, r8, pl.multiple_of(D + r8, 8))
        return extra

    ffn_loop(0, fwd_extra(0), "loop0")
    with jax.named_scope("ln2"):
        q_copy(2).wait()
        layernorm(2)
    ffn_loop(1, fwd_extra(NCH), "loop1")
    with jax.named_scope("spec"):
        spec_stage()
        q_copy(3).wait()
        layernorm(3)

    RI = D // NCH

    def inv_extra(i):
        for g in range(RI // 8):
            i1_rows(pl.multiple_of(i * RI + g * 8, 8))

    ffn_loop(2, inv_extra, "loop2")

    def out_copy(rows, cols, s):
        return pltpu.make_async_copy(o_ref.at[rows, cols],
                                     o_hbm.at[rows, cols], osem.at[s])

    early = pl.ds(0, (NTB - 1) * TB)

    def comb_extra(i):
        rows = pl.ds(pl.multiple_of(i * RI, 16), RI)
        combine(rows, early)
        out_copy(rows, early, 0).start()

    ffn_loop(3, comb_extra, "loop3", n_it=NCH - 1)
    with jax.named_scope("fin"):
        comb_extra(NCH - 1)
        ffn_down(NTB - 1, NCH - 1, (NTB * NCH - 1) % 2)
        late = pl.ds((NTB - 1) * TB, TB)
        combine(pl.ds(0, D), late)
        cp_late = out_copy(pl.ds(0, D), late, 1)
        cp_late.start()
        out_copy(pl.ds(0, D), early, 0).wait()
        cp_late.wait()


@jax.jit
def pallas_parallel_sum__ssm_conv_h3__dense_activation_silu__prompt_kernel(
    A_q: jax.Array,
    A_k: jax.Array,
    A_v: jax.Array,
    A_shift_k: jax.Array,
    A_ssm_k: jax.Array,
    A_ssm_D: jax.Array,
    B_x: jax.Array,
    B_w1: jax.Array,
    B_w2: jax.Array,
):
    del B_x
    qt = A_q.reshape(S, D).T
    kt = A_k.reshape(S, D).T
    vt = A_v.reshape(S, D).T
    sk = A_shift_k.T
    sd = A_ssm_D.reshape(1, D)
    w2t = B_w2.T
    dft_np, tw_np = _dft_tables()
    dft = jnp.asarray(dft_np)
    tw = jnp.asarray(tw_np)

    hbm = pl.BlockSpec(memory_space=pl.ANY)
    vmem = pl.BlockSpec(memory_space=pltpu.VMEM)
    in_specs = [hbm, hbm, hbm, vmem, hbm, vmem, hbm, hbm, vmem, vmem]
    bf = jnp.bfloat16
    scratch = [
        pltpu.VMEM((D, S), bf),
        pltpu.VMEM((D, S), bf),
        pltpu.VMEM((D, S), bf),
        pltpu.VMEM((D, S), bf),
        pltpu.VMEM((D, F), bf),
        pltpu.VMEM((D, F), bf),
        pltpu.VMEM((D, S), bf),
        pltpu.VMEM((NF1, 2 * NB, 2 * NB), bf),
        pltpu.VMEM((NF1, 2 * NB, 2 * NB), bf),
        pltpu.VMEM((F, D), bf),
        pltpu.VMEM((D, 8), jnp.float32),
        pltpu.VMEM((D, S), jnp.float32),
        pltpu.VMEM((NF1, 2 * D, 2 * NB), jnp.float32),
        pltpu.VMEM((NF1, D, 2 * NB), jnp.float32),
        pltpu.VMEM((D, S), jnp.float32),
        pltpu.VMEM((2, FC, TB), bf),
        pltpu.VMEM((D, S), jnp.float32),
        pltpu.VMEM((D, S), bf),
        pltpu.SemaphoreType.DMA((3 * 2 * (F // FC) + NTB + 2,)),
        pltpu.SemaphoreType.DMA((2,)),
    ]
    out = pl.pallas_call(
        _kernel,
        in_specs=in_specs,
        out_specs=hbm,
        out_shape=jax.ShapeDtypeStruct((D, S), bf),
        scratch_shapes=scratch,
        compiler_params=pltpu.CompilerParams(
            vmem_limit_bytes=100 * 1024 * 1024,
        ),
    )(qt, kt, vt, sk, A_ssm_k, sd, B_w1, w2t, dft, tw)
    return out.T.reshape(1, S, D)
```

```python
import math

import numpy as np
import jax
import jax.numpy as jnp
import jax.experimental.pallas as pl
import jax.experimental.pallas.tpu as pltpu

S = 2048
D = 448
F = 1792
L = 2 * S
NB = 128
NA = L // NB
NF1 = NA // 2 + 1
CR = 224
NCB = D // CR
TB = 512
NTB = S // TB
FC = 256
EPS = 1e-5


def _add(a, b):
    if a is None:
        return b
    if b is None:
        return a
    return a + b


def _sub(a, b):
    if b is None:
        return a
    if a is None:
        return -b
    return a - b


def _mulc(a, c):
    if a is None or c == 0.0:
        return None
    if c == 1.0:
        return a
    if c == -1.0:
        return -a
    return a * c


def _cmul_const(z, wr, wi):
    zr, zi = z
    if abs(wr) < 1e-12:
        wr = 0.0
    if abs(wi) < 1e-12:
        wi = 0.0
    if abs(abs(wr) - 1) < 1e-12:
        wr = math.copysign(1.0, wr)
    if abs(abs(wi) - 1) < 1e-12:
        wi = math.copysign(1.0, wi)
    re = _sub(_mulc(zr, wr), _mulc(zi, wi))
    im = _add(_mulc(zr, wi), _mulc(zi, wr))
    return (re, im)


def _rdft(x):
    n = len(x)
    if n == 1:
        return [(x[0], None)]
    if n == 2:
        return [(_add(x[0], x[1]), None), (_sub(x[0], x[1]), None)]
    e = _rdft(x[0::2])
    o = _rdft(x[1::2])
    out = [None] * (n // 2 + 1)
    for k in range(n // 4 + 1):
        t = _cmul_const(o[k], math.cos(2 * math.pi * k / n),
                        -math.sin(2 * math.pi * k / n))
        out[k] = (_add(e[k][0], t[0]), _add(e[k][1], t[1]))
        if n // 2 - k != k:
            out[n // 2 - k] = (_sub(e[k][0], t[0]), _sub(t[1], e[k][1]))
    return out


def _irdft(x, n, need):
    if n == 1:
        return [x[0][0]]
    if n == 2:
        out = [_add(x[0][0], x[1][0])]
        if need > 1:
            out.append(_sub(x[0][0], x[1][0]))
        return out
    e = [None] * (n // 4 + 1)
    o = [None] * (n // 4 + 1)
    for k in range(n // 4 + 1):
        a = x[k]
        b = x[n // 2 - k]
        e[k] = (_add(a[0], b[0]), _sub(a[1], b[1]))
        d = (_sub(a[0], b[0]), _add(a[1], b[1]))
        o[k] = _cmul_const(d, math.cos(2 * math.pi * k / n),
                           math.sin(2 * math.pi * k / n))
    ne = (need + 1) // 2
    no = need // 2
    xe = _irdft(e, n // 2, ne)
    xo = _irdft(o, n // 2, no) if no > 0 else []
    return [xe[i // 2] if i % 2 == 0 else xo[i // 2] for i in range(need)]


def _dft_tables():
    b = np.arange(NB)
    th = 2.0 * np.pi * ((b[:, None] * b[None, :]) % NB) / NB
    dft = np.stack([np.cos(th), np.sin(th)]).astype(np.float32)
    f1 = np.arange(NF1)
    th = 2.0 * np.pi * ((b[:, None] * f1[None, :]) % L) / L
    tw = np.zeros((2, NB, NB), np.float32)
    tw[0, :, :NF1] = np.cos(th)
    tw[1, :, :NF1] = np.sin(th)
    return dft, tw


def _kernel(q_hbm, k_hbm, v_hbm, sk_ref, hk_hbm, sd_ref, w1_hbm, w2_hbm,
            dft_ref, tw_ref, o_hbm,
            q_ref, k_ref, v_ref, hk_ref, w1_ref, w2_ref, o_ref,
            wf_ref, wi_ref, w1t_ref, par_ref, u_ref, g_ref, p_ref, y_ref,
            hb_ref, base_ref, xn_ref, sem, osem):
    f32 = jnp.float32
    bf16 = jnp.bfloat16
    NCH = F // FC
    HALF = D // 2

    NJ = TB // NB
    NIT = 2 * NCH
    CPI = D // NIT

    def kvh_copies(i):
        rows = pl.ds(i * CPI, CPI)
        return [pltpu.make_async_copy(src.at[rows, :], dst.at[rows, :],
                                      sem.at[3 * i + j])
                for j, (src, dst) in enumerate(
                    ((k_hbm, k_ref), (v_hbm, v_ref), (hk_hbm, hk_ref)))]

    def q_copy(tb):
        cols = pl.ds(tb * TB, TB)
        return pltpu.make_async_copy(q_hbm.at[:, cols], q_ref.at[:, cols],
                                     sem.at[3 * NIT + tb])

    cp_w1 = pltpu.make_async_copy(w1_hbm, w1_ref, sem.at[3 * NIT + NTB])
    cp_w2 = pltpu.make_async_copy(w2_hbm, w2_ref, sem.at[3 * NIT + NTB + 1])
    cp_w1.start()
    q_copy(0).start()
    for cp in kvh_copies(0):
        cp.start()
    cp_w2.start()
    for i in range(1, NIT):
        for cp in kvh_copies(i):
            cp.start()
        if i in (2, 5, 8):
            q_copy(1 + (i - 2) // 3).start()

    def tables():
        dc = dft_ref[0]
        ds_ = dft_ref[1]
        tc_all = tw_ref[0]
        ts_all = tw_ref[1]
        for f1 in range(NF1):
            tc = tc_all[:, f1:f1 + 1]
            ts = ts_all[:, f1:f1 + 1]
            c = tc * dc - ts * ds_
            s = ts * dc + tc * ds_
            wf_ref[f1, pl.ds(0, NB), pl.ds(0, NB)] = c.astype(bf16)
            wf_ref[f1, pl.ds(0, NB), pl.ds(NB, NB)] = (-s).astype(bf16)
            wf_ref[f1, pl.ds(NB, NB), pl.ds(0, NB)] = s.astype(bf16)
            wf_ref[f1, pl.ds(NB, NB), pl.ds(NB, NB)] = c.astype(bf16)
            ct = c.T * (1.0 / L)
            st = s.T * (1.0 / L)
            wi_ref[f1, pl.ds(0, NB), pl.ds(0, NB)] = ct.astype(bf16)
            wi_ref[f1, pl.ds(0, NB), pl.ds(NB, NB)] = st.astype(bf16)
            wi_ref[f1, pl.ds(NB, NB), pl.ds(0, NB)] = (-st).astype(bf16)
            wi_ref[f1, pl.ds(NB, NB), pl.ds(NB, NB)] = ct.astype(bf16)
        par = jnp.concatenate(
            [sk_ref[...].astype(f32), sd_ref[...].astype(f32),
             jnp.zeros((3, D), f32)], axis=0)
        par_ref[...] = par.T

    def kv_rows(r0, n):
        rows = pl.ds(r0, n)
        par = par_ref[rows, :]
        k = k_ref[rows, :].astype(f32)
        lane = jax.lax.broadcasted_iota(jnp.int32, (n, S), 1)
        ks = k * par[:, 0:1]
        for j in range(1, 4):
            kj = jnp.where(lane >= j, pltpu.roll(k, j, 1), 0.0)
            ks = ks + kj * par[:, j:j + 1]
        u_ref[rows, :] = ks * v_ref[rows, :].astype(f32)

    def s1_rows(src, r8, g8):
        xs = [src[pl.ds(r8, 8), pl.ds(NB * a, NB)].astype(f32)
              for a in range(NA // 2)]
        xs = xs + [None] * (NA // 2)
        g = _rdft(xs)
        for f1 in range(NF1):
            gr, gi = g[f1]
            if gi is None:
                gi = jnp.zeros((8, NB), f32)
            g_ref[f1, pl.ds(g8, 8), pl.ds(0, NB)] = gr
            g_ref[f1, pl.ds(g8, 8), pl.ds(NB, NB)] = gi

    def spec_stage():
        for f1 in range(NF1):
            x = jnp.dot(g_ref[f1].astype(bf16), wf_ref[f1],
                        preferred_element_type=f32)
            xr, xi = x[:D, :NB], x[:D, NB:]
            hr, hi = x[D:, :NB], x[D:, NB:]
            yr = xr * hr - xi * hi
            yi = xr * hi + xi * hr
            yy = jnp.concatenate([yr, yi], axis=1).astype(bf16)
            p_ref[f1] = jnp.dot(yy, wi_ref[f1], preferred_element_type=f32)

    def i1_rows(r8):
        rows = pl.ds(r8, 8)
        xs = [(p_ref[f1, rows, pl.ds(0, NB)], p_ref[f1, rows, pl.ds(NB, NB)])
              for f1 in range(NF1)]
        y = _irdft(xs, NA, NA // 2)
        sd = par_ref[rows, :][:, 4:5]
        for a in range(NA // 2):
            col = pl.ds(NB * a, NB)
            yc = y[a].astype(bf16).astype(f32)
            y_ref[rows, col] = yc + u_ref[rows, col] * sd

    def layernorm(tb):
        cols = pl.ds(tb * TB, TB)
        x = q_ref[:, cols].astype(f32)
        mean = jnp.mean(x, axis=0, keepdims=True)
        xc = x - mean
        var = jnp.mean(xc * xc, axis=0, keepdims=True)
        xn = xc * jax.lax.rsqrt(var + EPS)
        xn_ref[:, cols] = xn.astype(bf16)
        base_ref[:, cols] = x

    def ffn_up(tb, i, slot, j):
        f0 = pl.multiple_of(i * FC, FC)
        c0 = pl.multiple_of(tb * TB + j * NB, NB)
        h = jnp.dot(w1t_ref[pl.ds(f0, FC), :], xn_ref[:, pl.ds(c0, NB)],
                    preferred_element_type=f32)
        hb_ref[slot, :, pl.ds(j * NB, NB)] = (
            h * jax.nn.sigmoid(h)).astype(bf16)

    def ffn_down(tb, i, slot, j):
        f0 = pl.multiple_of(i * FC, FC)
        part = jnp.dot(w2_ref[:, pl.ds(f0, FC)],
                       hb_ref[slot, :, pl.ds(j * NB, NB)],
                       preferred_element_type=f32)
        cols = pl.ds(tb * TB + j * NB, NB)
        base_ref[:, cols] = base_ref[:, cols] + part

    def combine(rows, cols):
        o_ref[rows, cols] = (
            base_ref[rows, cols]
            + xn_ref[rows, cols].astype(f32) * y_ref[rows, cols]
        ).astype(o_ref.dtype)

    def ffn_loop(tb, extra, name, n_it=NCH):
        def body(i, carry):
            n = tb * NCH + i
            slot = jax.lax.rem(n, 2)
            nxt = n + 1
            tb2 = nxt // NCH
            for j in range(NJ):
                extra(i, j)
                ffn_up(tb2, nxt - tb2 * NCH, 1 - slot, j)
                ffn_down(tb, i, slot, j)
            return carry

        with jax.named_scope(name):
            jax.lax.fori_loop(0, n_it, body, 0)

    with jax.named_scope("tables"):
        tables()
    with jax.named_scope("pro"):
        cp_w1.wait()
        w1t_ref[...] = w1_ref[...].astype(f32).T.astype(bf16)
        q_copy(0).wait()
        layernorm(0)
        for j in range(NJ):
            ffn_up(0, 0, 0, j)
        q_copy(1).wait()
        layernorm(1)
        cp_w2.wait()

    def fwd_extra(it0):
        def extra(i, j):
            it = it0 + i
            if j == 0:
                for cp in kvh_copies(it):
                    cp.wait()
            r8 = pl.multiple_of(it * CPI + j * 8, 8)
            kv_rows(r8, 8)
            s1_rows(u_ref, r8, r8)
            s1_rows(hk_ref, r8, pl.multiple_of(D + r8, 8))
        return extra

    ffn_loop(0, fwd_extra(0), "loop0")
    with jax.named_scope("ln2"):
        q_copy(2).wait()
        layernorm(2)
    ffn_loop(1, fwd_extra(NCH), "loop1")
    with jax.named_scope("spec"):
        spec_stage()
        q_copy(3).wait()
        layernorm(3)

    RI = D // NCH

    def inv_extra(i, j):
        for g in range(RI // 8 // NJ):
            i1_rows(pl.multiple_of(i * RI + (j * (RI // 8 // NJ) + g) * 8, 8))

    ffn_loop(2, inv_extra, "loop2")

    def out_copy(rows, cols, s):
        return pltpu.make_async_copy(o_ref.at[rows, cols],
                                     o_hbm.at[rows, cols], osem.at[s])

    early = pl.ds(0, (NTB - 1) * TB)

    def comb_extra(i, j):
        rows = pl.ds(pl.multiple_of(i * RI + j * (RI // NJ), 16), RI // NJ)
        combine(rows, early)
        out_copy(rows, early, 0).start()

    ffn_loop(3, comb_extra, "loop3", n_it=NCH - 1)
    with jax.named_scope("fin"):
        for j in range(NJ):
            comb_extra(NCH - 1, j)
            ffn_down(NTB - 1, NCH - 1, (NTB * NCH - 1) % 2, j)
        late = pl.ds((NTB - 1) * TB, TB)
        combine(pl.ds(0, D), late)
        cp_late = out_copy(pl.ds(0, D), late, 1)
        cp_late.start()
        out_copy(pl.ds(0, D), early, 0).wait()
        cp_late.wait()


@jax.jit
def pallas_parallel_sum__ssm_conv_h3__dense_activation_silu__prompt_kernel(
    A_q: jax.Array,
    A_k: jax.Array,
    A_v: jax.Array,
    A_shift_k: jax.Array,
    A_ssm_k: jax.Array,
    A_ssm_D: jax.Array,
    B_x: jax.Array,
    B_w1: jax.Array,
    B_w2: jax.Array,
):
    del B_x
    qt = A_q.reshape(S, D).T
    kt = A_k.reshape(S, D).T
    vt = A_v.reshape(S, D).T
    sk = A_shift_k.T
    sd = A_ssm_D.reshape(1, D)
    w2t = B_w2.T
    dft_np, tw_np = _dft_tables()
    dft = jnp.asarray(dft_np)
    tw = jnp.asarray(tw_np)

    hbm = pl.BlockSpec(memory_space=pl.ANY)
    vmem = pl.BlockSpec(memory_space=pltpu.VMEM)
    in_specs = [hbm, hbm, hbm, vmem, hbm, vmem, hbm, hbm, vmem, vmem]
    bf = jnp.bfloat16
    scratch = [
        pltpu.VMEM((D, S), bf),
        pltpu.VMEM((D, S), bf),
        pltpu.VMEM((D, S), bf),
        pltpu.VMEM((D, S), bf),
        pltpu.VMEM((D, F), bf),
        pltpu.VMEM((D, F), bf),
        pltpu.VMEM((D, S), bf),
        pltpu.VMEM((NF1, 2 * NB, 2 * NB), bf),
        pltpu.VMEM((NF1, 2 * NB, 2 * NB), bf),
        pltpu.VMEM((F, D), bf),
        pltpu.VMEM((D, 8), jnp.float32),
        pltpu.VMEM((D, S), jnp.float32),
        pltpu.VMEM((NF1, 2 * D, 2 * NB), jnp.float32),
        pltpu.VMEM((NF1, D, 2 * NB), jnp.float32),
        pltpu.VMEM((D, S), jnp.float32),
        pltpu.VMEM((2, FC, TB), bf),
        pltpu.VMEM((D, S), jnp.float32),
        pltpu.VMEM((D, S), bf),
        pltpu.SemaphoreType.DMA((3 * 2 * (F // FC) + NTB + 2,)),
        pltpu.SemaphoreType.DMA((2,)),
    ]
    out = pl.pallas_call(
        _kernel,
        in_specs=in_specs,
        out_specs=hbm,
        out_shape=jax.ShapeDtypeStruct((D, S), bf),
        scratch_shapes=scratch,
        compiler_params=pltpu.CompilerParams(
            vmem_limit_bytes=100 * 1024 * 1024,
        ),
    )(qt, kt, vt, sk, A_ssm_k, sd, B_w1, w2t, dft, tw)
    return out.T.reshape(1, S, D)
```

```python
import math

import numpy as np
import jax
import jax.numpy as jnp
import jax.experimental.pallas as pl
import jax.experimental.pallas.tpu as pltpu

S = 2048
D = 448
F = 1792
L = 2 * S
NB = 128
NA = L // NB
NF1 = NA // 2 + 1
CR = 224
NCB = D // CR
TB = 512
NTB = S // TB
FC = 256
EPS = 1e-5


def _add(a, b):
    if a is None:
        return b
    if b is None:
        return a
    return a + b


def _sub(a, b):
    if b is None:
        return a
    if a is None:
        return -b
    return a - b


def _mulc(a, c):
    if a is None or c == 0.0:
        return None
    if c == 1.0:
        return a
    if c == -1.0:
        return -a
    return a * c


def _cmul_const(z, wr, wi):
    zr, zi = z
    if abs(wr) < 1e-12:
        wr = 0.0
    if abs(wi) < 1e-12:
        wi = 0.0
    if abs(abs(wr) - 1) < 1e-12:
        wr = math.copysign(1.0, wr)
    if abs(abs(wi) - 1) < 1e-12:
        wi = math.copysign(1.0, wi)
    re = _sub(_mulc(zr, wr), _mulc(zi, wi))
    im = _add(_mulc(zr, wi), _mulc(zi, wr))
    return (re, im)


def _rdft(x):
    n = len(x)
    if n == 1:
        return [(x[0], None)]
    if n == 2:
        return [(_add(x[0], x[1]), None), (_sub(x[0], x[1]), None)]
    e = _rdft(x[0::2])
    o = _rdft(x[1::2])
    out = [None] * (n // 2 + 1)
    for k in range(n // 4 + 1):
        t = _cmul_const(o[k], math.cos(2 * math.pi * k / n),
                        -math.sin(2 * math.pi * k / n))
        out[k] = (_add(e[k][0], t[0]), _add(e[k][1], t[1]))
        if n // 2 - k != k:
            out[n // 2 - k] = (_sub(e[k][0], t[0]), _sub(t[1], e[k][1]))
    return out


def _irdft(x, n, need):
    if n == 1:
        return [x[0][0]]
    if n == 2:
        out = [_add(x[0][0], x[1][0])]
        if need > 1:
            out.append(_sub(x[0][0], x[1][0]))
        return out
    e = [None] * (n // 4 + 1)
    o = [None] * (n // 4 + 1)
    for k in range(n // 4 + 1):
        a = x[k]
        b = x[n // 2 - k]
        e[k] = (_add(a[0], b[0]), _sub(a[1], b[1]))
        d = (_sub(a[0], b[0]), _add(a[1], b[1]))
        o[k] = _cmul_const(d, math.cos(2 * math.pi * k / n),
                           math.sin(2 * math.pi * k / n))
    ne = (need + 1) // 2
    no = need // 2
    xe = _irdft(e, n // 2, ne)
    xo = _irdft(o, n // 2, no) if no > 0 else []
    return [xe[i // 2] if i % 2 == 0 else xo[i // 2] for i in range(need)]


def _dft_tables():
    b = np.arange(NB)
    th = 2.0 * np.pi * ((b[:, None] * b[None, :]) % NB) / NB
    dft = np.stack([np.cos(th), np.sin(th)]).astype(np.float32)
    f1 = np.arange(NF1)
    th = 2.0 * np.pi * ((b[:, None] * f1[None, :]) % L) / L
    tw = np.zeros((2, NB, NB), np.float32)
    tw[0, :, :NF1] = np.cos(th)
    tw[1, :, :NF1] = np.sin(th)
    return dft, tw


def _kernel(q_hbm, k_hbm, v_hbm, sk_ref, hk_hbm, sd_ref, w1_hbm, w2_hbm,
            dft_ref, tw_ref, o_hbm,
            q_ref, k_ref, v_ref, hk_ref, w1_ref, w2_ref, o_ref,
            wf_ref, wi_ref, w1t_ref, par_ref, u_ref, g_ref, p_ref, y_ref,
            hb_ref, base_ref, xn_ref, sem, osem):
    f32 = jnp.float32
    bf16 = jnp.bfloat16
    NCH = F // FC
    HALF = D // 2

    NIT = 2 * NCH
    CPI = D // NIT

    def kvh_copies(i):
        rows = pl.ds(i * CPI, CPI)
        return [pltpu.make_async_copy(src.at[rows, :], dst.at[rows, :],
                                      sem.at[3 * i + j])
                for j, (src, dst) in enumerate(
                    ((k_hbm, k_ref), (v_hbm, v_ref), (hk_hbm, hk_ref)))]

    def q_copy(tb):
        cols = pl.ds(tb * TB, TB)
        return pltpu.make_async_copy(q_hbm.at[:, cols], q_ref.at[:, cols],
                                     sem.at[3 * NIT + tb])

    cp_w1 = pltpu.make_async_copy(w1_hbm, w1_ref, sem.at[3 * NIT + NTB])
    cp_w2 = pltpu.make_async_copy(w2_hbm, w2_ref, sem.at[3 * NIT + NTB + 1])
    cp_w1.start()
    q_copy(0).start()
    for cp in kvh_copies(0):
        cp.start()
    cp_w2.start()
    for i in range(1, NIT):
        for cp in kvh_copies(i):
            cp.start()
        if i < NTB:
            q_copy(i).start()

    def tables():
        dc = dft_ref[0]
        ds_ = dft_ref[1]
        tc_all = tw_ref[0]
        ts_all = tw_ref[1]
        for f1 in range(NF1):
            tc = tc_all[:, f1:f1 + 1]
            ts = ts_all[:, f1:f1 + 1]
            c = tc * dc - ts * ds_
            s = ts * dc + tc * ds_
            wf_ref[f1, pl.ds(0, NB), pl.ds(0, NB)] = c.astype(bf16)
            wf_ref[f1, pl.ds(0, NB), pl.ds(NB, NB)] = (-s).astype(bf16)
            wf_ref[f1, pl.ds(NB, NB), pl.ds(0, NB)] = s.astype(bf16)
            wf_ref[f1, pl.ds(NB, NB), pl.ds(NB, NB)] = c.astype(bf16)
            ct = c.T * (1.0 / L)
            st = s.T * (1.0 / L)
            wi_ref[f1, pl.ds(0, NB), pl.ds(0, NB)] = ct.astype(bf16)
            wi_ref[f1, pl.ds(0, NB), pl.ds(NB, NB)] = st.astype(bf16)
            wi_ref[f1, pl.ds(NB, NB), pl.ds(0, NB)] = (-st).astype(bf16)
            wi_ref[f1, pl.ds(NB, NB), pl.ds(NB, NB)] = ct.astype(bf16)
        par = jnp.concatenate(
            [sk_ref[...].astype(f32), sd_ref[...].astype(f32),
             jnp.zeros((3, D), f32)], axis=0)
        par_ref[...] = par.T

    def kv_rows(r0, n):
        rows = pl.ds(r0, n)
        par = par_ref[rows, :]
        k = k_ref[rows, :].astype(f32)
        lane = jax.lax.broadcasted_iota(jnp.int32, (n, S), 1)
        ks = k * par[:, 0:1]
        for j in range(1, 4):
            kj = jnp.where(lane >= j, pltpu.roll(k, j, 1), 0.0)
            ks = ks + kj * par[:, j:j + 1]
        u_ref[rows, :] = ks * v_ref[rows, :].astype(f32)

    def s1_rows(src, r8, g8):
        xs = [src[pl.ds(r8, 8), pl.ds(NB * a, NB)].astype(f32)
              for a in range(NA // 2)]
        xs = xs + [None] * (NA // 2)
        g = _rdft(xs)
        for f1 in range(NF1):
            gr, gi = g[f1]
            if gi is None:
                gi = jnp.zeros((8, NB), f32)
            g_ref[f1, pl.ds(g8, 8), pl.ds(0, NB)] = gr
            g_ref[f1, pl.ds(g8, 8), pl.ds(NB, NB)] = gi

    def spec_stage():
        for f1 in range(NF1):
            x = jnp.dot(g_ref[f1].astype(bf16), wf_ref[f1],
                        preferred_element_type=f32)
            xr, xi = x[:D, :NB], x[:D, NB:]
            hr, hi = x[D:, :NB], x[D:, NB:]
            yr = xr * hr - xi * hi
            yi = xr * hi + xi * hr
            yy = jnp.concatenate([yr, yi], axis=1).astype(bf16)
            p_ref[f1] = jnp.dot(yy, wi_ref[f1], preferred_element_type=f32)

    def i1_rows(r8):
        rows = pl.ds(r8, 8)
        xs = [(p_ref[f1, rows, pl.ds(0, NB)], p_ref[f1, rows, pl.ds(NB, NB)])
              for f1 in range(NF1)]
        y = _irdft(xs, NA, NA // 2)
        sd = par_ref[rows, :][:, 4:5]
        for a in range(NA // 2):
            col = pl.ds(NB * a, NB)
            yc = y[a].astype(bf16).astype(f32)
            y_ref[rows, col] = yc + u_ref[rows, col] * sd

    def layernorm(tb):
        cols = pl.ds(tb * TB, TB)
        x = q_ref[:, cols].astype(f32)
        mean = jnp.mean(x, axis=0, keepdims=True)
        xc = x - mean
        var = jnp.mean(xc * xc, axis=0, keepdims=True)
        xn = xc * jax.lax.rsqrt(var + EPS)
        xn_ref[:, cols] = xn.astype(bf16)
        base_ref[:, cols] = x

    def ffn_up(tb, i, slot):
        f0 = pl.multiple_of(i * FC, FC)
        c0 = pl.multiple_of(tb * TB, TB)
        h = jnp.dot(w1t_ref[pl.ds(f0, FC), :], xn_ref[:, pl.ds(c0, TB)],
                    preferred_element_type=f32)
        hh = 0.5 * h
        hb_ref[slot] = (hh + hh * jnp.tanh(hh)).astype(bf16)

    def ffn_down(tb, i, slot):
        f0 = pl.multiple_of(i * FC, FC)
        part = jnp.dot(w2_ref[:, pl.ds(f0, FC)], hb_ref[slot],
                       preferred_element_type=f32)
        cols = pl.ds(tb * TB, TB)
        base_ref[:, cols] = base_ref[:, cols] + part

    def combine(rows, cols):
        o_ref[rows, cols] = (
            base_ref[rows, cols]
            + xn_ref[rows, cols].astype(f32) * y_ref[rows, cols]
        ).astype(o_ref.dtype)

    def ffn_loop(tb, extra, name, n_it=NCH):
        def body(i, carry):
            n = tb * NCH + i
            slot = jax.lax.rem(n, 2)
            extra(i)
            nxt = n + 1
            tb2 = nxt // NCH
            ffn_up(tb2, nxt - tb2 * NCH, 1 - slot)
            ffn_down(tb, i, slot)
            return carry

        with jax.named_scope(name):
            jax.lax.fori_loop(0, n_it, body, 0, unroll=True)

    with jax.named_scope("tables"):
        tables()
    with jax.named_scope("pro"):
        cp_w1.wait()
        w1t_ref[...] = w1_ref[...].astype(f32).T.astype(bf16)
        q_copy(0).wait()
        layernorm(0)
        ffn_up(0, 0, 0)
        q_copy(1).wait()
        layernorm(1)
        cp_w2.wait()

    def fwd_extra(it0):
        def extra(i):
            it = it0 + i
            for cp in kvh_copies(it):
                cp.wait()
            r0 = pl.multiple_of(it * CPI, 8)
            kv_rows(r0, CPI)
            for g in range(CPI // 8):
                r8 = pl.multiple_of(r0 + g * 8, 8)
                s1_rows(u_ref, r8, r8)
                s1_rows(hk_ref, r8, pl.multiple_of(D + r8, 8))
        return extra

    ffn_loop(0, fwd_extra(0), "loop0")
    with jax.named_scope("ln2"):
        q_copy(2).wait()
        layernorm(2)
    ffn_loop(1, fwd_extra(NCH), "loop1")
    with jax.named_scope("spec"):
        spec_stage()
        q_copy(3).wait()
        layernorm(3)

    RI = D // NCH

    def inv_extra(i):
        for g in range(RI // 8):
            i1_rows(pl.multiple_of(i * RI + g * 8, 8))

    ffn_loop(2, inv_extra, "loop2")

    def out_copy(rows, cols, s):
        return pltpu.make_async_copy(o_ref.at[rows, cols],
                                     o_hbm.at[rows, cols], osem.at[s])

    early = pl.ds(0, (NTB - 1) * TB)

    def comb_extra(i):
        rows = pl.ds(pl.multiple_of(i * RI, 16), RI)
        combine(rows, early)
        out_copy(rows, early, 0).start()

    ffn_loop(3, comb_extra, "loop3", n_it=NCH - 1)
    with jax.named_scope("fin"):
        comb_extra(NCH - 1)
        ffn_down(NTB - 1, NCH - 1, (NTB * NCH - 1) % 2)
        late = pl.ds((NTB - 1) * TB, TB)
        combine(pl.ds(0, D), late)
        cp_late = out_copy(pl.ds(0, D), late, 1)
        cp_late.start()
        out_copy(pl.ds(0, D), early, 0).wait()
        cp_late.wait()


@jax.jit
def pallas_parallel_sum__ssm_conv_h3__dense_activation_silu__prompt_kernel(
    A_q: jax.Array,
    A_k: jax.Array,
    A_v: jax.Array,
    A_shift_k: jax.Array,
    A_ssm_k: jax.Array,
    A_ssm_D: jax.Array,
    B_x: jax.Array,
    B_w1: jax.Array,
    B_w2: jax.Array,
):
    del B_x
    qt = A_q.reshape(S, D).T
    kt = A_k.reshape(S, D).T
    vt = A_v.reshape(S, D).T
    sk = A_shift_k.T
    sd = A_ssm_D.reshape(1, D)
    w2t = B_w2.T
    dft_np, tw_np = _dft_tables()
    dft = jnp.asarray(dft_np)
    tw = jnp.asarray(tw_np)

    hbm = pl.BlockSpec(memory_space=pl.ANY)
    vmem = pl.BlockSpec(memory_space=pltpu.VMEM)
    in_specs = [hbm, hbm, hbm, vmem, hbm, vmem, hbm, hbm, vmem, vmem]
    bf = jnp.bfloat16
    scratch = [
        pltpu.VMEM((D, S), bf),
        pltpu.VMEM((D, S), bf),
        pltpu.VMEM((D, S), bf),
        pltpu.VMEM((D, S), bf),
        pltpu.VMEM((D, F), bf),
        pltpu.VMEM((D, F), bf),
        pltpu.VMEM((D, S), bf),
        pltpu.VMEM((NF1, 2 * NB, 2 * NB), bf),
        pltpu.VMEM((NF1, 2 * NB, 2 * NB), bf),
        pltpu.VMEM((F, D), bf),
        pltpu.VMEM((D, 8), jnp.float32),
        pltpu.VMEM((D, S), jnp.float32),
        pltpu.VMEM((NF1, 2 * D, 2 * NB), jnp.float32),
        pltpu.VMEM((NF1, D, 2 * NB), jnp.float32),
        pltpu.VMEM((D, S), jnp.float32),
        pltpu.VMEM((2, FC, TB), bf),
        pltpu.VMEM((D, S), jnp.float32),
        pltpu.VMEM((D, S), bf),
        pltpu.SemaphoreType.DMA((3 * 2 * (F // FC) + NTB + 2,)),
        pltpu.SemaphoreType.DMA((2,)),
    ]
    out = pl.pallas_call(
        _kernel,
        in_specs=in_specs,
        out_specs=hbm,
        out_shape=jax.ShapeDtypeStruct((D, S), bf),
        scratch_shapes=scratch,
        compiler_params=pltpu.CompilerParams(
            vmem_limit_bytes=100 * 1024 * 1024,
        ),
    )(qt, kt, vt, sk, A_ssm_k, sd, B_w1, w2t, dft, tw)
    return out.T.reshape(1, S, D)
```

```python
import math

import numpy as np
import jax
import jax.numpy as jnp
import jax.experimental.pallas as pl
import jax.experimental.pallas.tpu as pltpu

S = 2048
D = 448
F = 1792
L = 2 * S
NB = 128
NA = L // NB
NF1 = NA // 2 + 1
CR = 224
NCB = D // CR
TB = 512
NTB = S // TB
DP = 512
FC = 256
EPS = 1e-5


def _add(a, b):
    if a is None:
        return b
    if b is None:
        return a
    return a + b


def _sub(a, b):
    if b is None:
        return a
    if a is None:
        return -b
    return a - b


def _mulc(a, c):
    if a is None or c == 0.0:
        return None
    if c == 1.0:
        return a
    if c == -1.0:
        return -a
    return a * c


def _cmul_const(z, wr, wi):
    zr, zi = z
    if abs(wr) < 1e-12:
        wr = 0.0
    if abs(wi) < 1e-12:
        wi = 0.0
    if abs(abs(wr) - 1) < 1e-12:
        wr = math.copysign(1.0, wr)
    if abs(abs(wi) - 1) < 1e-12:
        wi = math.copysign(1.0, wi)
    re = _sub(_mulc(zr, wr), _mulc(zi, wi))
    im = _add(_mulc(zr, wi), _mulc(zi, wr))
    return (re, im)


def _rdft(x):
    n = len(x)
    if n == 1:
        return [(x[0], None)]
    if n == 2:
        return [(_add(x[0], x[1]), None), (_sub(x[0], x[1]), None)]
    e = _rdft(x[0::2])
    o = _rdft(x[1::2])
    out = [None] * (n // 2 + 1)
    for k in range(n // 4 + 1):
        t = _cmul_const(o[k], math.cos(2 * math.pi * k / n),
                        -math.sin(2 * math.pi * k / n))
        out[k] = (_add(e[k][0], t[0]), _add(e[k][1], t[1]))
        if n // 2 - k != k:
            out[n // 2 - k] = (_sub(e[k][0], t[0]), _sub(t[1], e[k][1]))
    return out


def _irdft(x, n, need):
    if n == 1:
        return [x[0][0]]
    if n == 2:
        out = [_add(x[0][0], x[1][0])]
        if need > 1:
            out.append(_sub(x[0][0], x[1][0]))
        return out
    e = [None] * (n // 4 + 1)
    o = [None] * (n // 4 + 1)
    for k in range(n // 4 + 1):
        a = x[k]
        b = x[n // 2 - k]
        e[k] = (_add(a[0], b[0]), _sub(a[1], b[1]))
        d = (_sub(a[0], b[0]), _add(a[1], b[1]))
        o[k] = _cmul_const(d, math.cos(2 * math.pi * k / n),
                           math.sin(2 * math.pi * k / n))
    ne = (need + 1) // 2
    no = need // 2
    xe = _irdft(e, n // 2, ne)
    xo = _irdft(o, n // 2, no) if no > 0 else []
    return [xe[i // 2] if i % 2 == 0 else xo[i // 2] for i in range(need)]


def _dft_tables():
    b = np.arange(NB)
    th = 2.0 * np.pi * ((b[:, None] * b[None, :]) % NB) / NB
    dft = np.stack([np.cos(th), np.sin(th)]).astype(np.float32)
    f1 = np.arange(NF1)
    th = 2.0 * np.pi * ((b[:, None] * f1[None, :]) % L) / L
    tw = np.zeros((2, NB, NB), np.float32)
    tw[0, :, :NF1] = np.cos(th)
    tw[1, :, :NF1] = np.sin(th)
    return dft, tw


def _kernel(q_hbm, k_hbm, v_hbm, sk_ref, hk_hbm, sd_ref, w1_hbm, w2_hbm,
            dft_ref, tw_ref, o_hbm,
            q_ref, k_ref, v_ref, hk_ref, w1_ref, w2_ref, o_ref,
            wf_ref, wi_ref, w1t_ref, par_ref, u_ref, g_ref, p_ref, y_ref,
            hb_ref, base_ref, xn_ref, sem, osem):
    f32 = jnp.float32
    bf16 = jnp.bfloat16
    NCH = F // FC
    NIT = 2 * NCH
    CPI = D // NIT
    RI = D // NCH

    def kvh_copies(i):
        rows = pl.ds(i * CPI, CPI)
        return [pltpu.make_async_copy(src.at[rows, :], dst.at[rows, :],
                                      sem.at[3 * i + j])
                for j, (src, dst) in enumerate(
                    ((k_hbm, k_ref), (v_hbm, v_ref), (hk_hbm, hk_ref)))]

    def q_copy(tb):
        cols = pl.ds(tb * TB, TB)
        return pltpu.make_async_copy(q_hbm.at[:, cols], q_ref.at[:, cols],
                                     sem.at[3 * NIT + tb])

    cp_w1 = pltpu.make_async_copy(w1_hbm, w1_ref, sem.at[3 * NIT + NTB])
    cp_w2 = pltpu.make_async_copy(w2_hbm, w2_ref, sem.at[3 * NIT + NTB + 1])
    cp_w1.start()
    q_copy(0).start()
    for cp in kvh_copies(0):
        cp.start()
    cp_w2.start()
    for i in range(1, NIT):
        for cp in kvh_copies(i):
            cp.start()
        if i < NTB:
            q_copy(i).start()

    def tables():
        dc = dft_ref[0]
        ds_ = dft_ref[1]
        tc_all = tw_ref[0]
        ts_all = tw_ref[1]
        for f1 in range(NF1):
            tc = tc_all[:, f1:f1 + 1]
            ts = ts_all[:, f1:f1 + 1]
            c = tc * dc - ts * ds_
            s = ts * dc + tc * ds_
            wf_ref[f1, pl.ds(0, NB), pl.ds(0, NB)] = c.astype(bf16)
            wf_ref[f1, pl.ds(0, NB), pl.ds(NB, NB)] = (-s).astype(bf16)
            wf_ref[f1, pl.ds(NB, NB), pl.ds(0, NB)] = s.astype(bf16)
            wf_ref[f1, pl.ds(NB, NB), pl.ds(NB, NB)] = c.astype(bf16)
            ct = c.T * (1.0 / L)
            st = s.T * (1.0 / L)
            wi_ref[f1, pl.ds(0, NB), pl.ds(0, NB)] = ct.astype(bf16)
            wi_ref[f1, pl.ds(0, NB), pl.ds(NB, NB)] = st.astype(bf16)
            wi_ref[f1, pl.ds(NB, NB), pl.ds(0, NB)] = (-st).astype(bf16)
            wi_ref[f1, pl.ds(NB, NB), pl.ds(NB, NB)] = ct.astype(bf16)
        par = jnp.concatenate(
            [sk_ref[...].astype(f32), sd_ref[...].astype(f32),
             jnp.zeros((3, D), f32)], axis=0)
        par_ref[...] = par.T

    def kv_rows(r0, n):
        rows = pl.ds(r0, n)
        par = par_ref[rows, :]
        k = k_ref[rows, :].astype(f32)
        lane = jax.lax.broadcasted_iota(jnp.int32, (n, S), 1)
        ks = k * par[:, 0:1]
        for j in range(1, 4):
            kj = jnp.where(lane >= j, pltpu.roll(k, j, 1), 0.0)
            ks = ks + kj * par[:, j:j + 1]
        u_ref[rows, :] = ks * v_ref[rows, :].astype(f32)

    def s1_rows(src, r8, g8):
        xs = [src[pl.ds(r8, 8), pl.ds(NB * a, NB)].astype(f32)
              for a in range(NA // 2)]
        xs = xs + [None] * (NA // 2)
        g = _rdft(xs)
        for f1 in range(NF1):
            gr, gi = g[f1]
            if gi is None:
                gi = jnp.zeros((8, NB), f32)
            g_ref[f1, pl.ds(g8, 8), pl.ds(0, NB)] = gr
            g_ref[f1, pl.ds(g8, 8), pl.ds(NB, NB)] = gi
        return g[NF1 // 2][1]

    def spec_stage():
        for f1 in range(NF1):
            x = jnp.dot(g_ref[f1].astype(bf16), wf_ref[f1],
                        preferred_element_type=f32)
            xr, xi = x[:D, :NB], x[:D, NB:]
            hr, hi = x[D:, :NB], x[D:, NB:]
            yr = xr * hr - xi * hi
            yi = xr * hi + xi * hr
            yy = jnp.concatenate([yr, yi], axis=1).astype(bf16)
            p_ref[f1] = jnp.dot(yy, wi_ref[f1], preferred_element_type=f32)

    def i1_rows(r8):
        rows = pl.ds(r8, 8)
        xs = [(p_ref[f1, rows, pl.ds(0, NB)], p_ref[f1, rows, pl.ds(NB, NB)])
              for f1 in range(NF1)]
        y = _irdft(xs, NA, NA // 2)
        sd = par_ref[rows, :][:, 4:5]
        for a in range(NA // 2):
            col = pl.ds(NB * a, NB)
            yc = y[a].astype(bf16).astype(f32)
            tok = yc + u_ref[rows, col] * sd
            y_ref[rows, col] = tok
        return tok

    def layernorm(tb):
        cols = pl.ds(tb * TB, TB)
        x = q_ref[:, cols].astype(f32)
        mean = jnp.mean(x, axis=0, keepdims=True)
        xc = x - mean
        var = jnp.mean(xc * xc, axis=0, keepdims=True)
        xn = xc * jax.lax.rsqrt(var + EPS)
        xn_ref[pl.ds(0, D), cols] = xn.astype(bf16)
        base_ref[:, cols] = x

    def ffn_up(n):
        tb, i = divmod(n, NCH)
        h = jnp.dot(w1t_ref[pl.ds(i * FC, FC), :],
                    xn_ref[:, pl.ds(tb * TB, TB)],
                    preferred_element_type=f32)
        hh = 0.5 * h
        hb_ref[n % 2] = (hh + hh * jnp.tanh(hh)).astype(bf16)

    def ffn_down(n):
        tb, i = divmod(n, NCH)
        part = jnp.dot(w2_ref[:, pl.ds(i * FC, FC)], hb_ref[n % 2],
                       preferred_element_type=f32)
        cols = pl.ds(tb * TB, TB)
        base_ref[:, cols] = base_ref[:, cols] + part

    def combine(rows, cols):
        out = (base_ref[rows, cols]
               + xn_ref[rows, cols].astype(f32) * y_ref[rows, cols])
        o_ref[rows, cols] = out.astype(o_ref.dtype)
        return out[0:8, 0:NB]

    def order_before(tok, g, n):
        if n < NTB * NCH:
            tb = n // NCH
            xn_ref[pl.ds(D + 8 * g, 8), pl.ds(tb * TB, NB)] = tok.astype(bf16)

    def out_copy(rows, cols, s):
        return pltpu.make_async_copy(o_ref.at[rows, cols],
                                     o_hbm.at[rows, cols], osem.at[s])

    early = pl.ds(0, (NTB - 1) * TB)

    def extra(n):
        if n < NIT:
            for cp in kvh_copies(n):
                cp.wait()
            kv_rows(n * CPI, CPI)
            for g in range(CPI // 8):
                r8 = n * CPI + g * 8
                order_before(s1_rows(u_ref, r8, r8), 2 * g, n + 1)
                order_before(s1_rows(hk_ref, r8, D + r8), 2 * g + 1, n + 1)
        elif n < NIT + NCH:
            i = n - NIT
            for g in range(RI // 8):
                order_before(i1_rows(i * RI + g * 8), g, n + 1)
        else:
            i = n - NIT - NCH
            rows = pl.ds(i * RI, RI)
            order_before(combine(rows, early), 0, n + 1)
            out_copy(rows, early, 0).start()

    with jax.named_scope("tables"):
        tables()
        xn_ref[pl.ds(D, DP - D), :] = jnp.zeros((DP - D, S), bf16)
        w1t_ref[:, pl.ds(D, DP - D)] = jnp.zeros((F, DP - D), bf16)
    with jax.named_scope("pro"):
        cp_w1.wait()
        w1t_ref[:, pl.ds(0, D)] = w1_ref[...].astype(f32).T.astype(bf16)
        q_copy(0).wait()
        layernorm(0)
        ffn_up(0)
        q_copy(1).wait()
        layernorm(1)
        cp_w2.wait()

    for n in range(NTB * NCH):
        if n == NCH:
            q_copy(2).wait()
            layernorm(2)
        if n == NIT:
            spec_stage()
            q_copy(3).wait()
            layernorm(3)
        extra(n)
        if n + 1 < NTB * NCH:
            ffn_up(n + 1)
        ffn_down(n)

    with jax.named_scope("fin"):
        late = pl.ds((NTB - 1) * TB, TB)
        combine(pl.ds(0, D), late)
        cp_late = out_copy(pl.ds(0, D), late, 1)
        cp_late.start()
        out_copy(pl.ds(0, D), early, 0).wait()
        cp_late.wait()


@jax.jit
def pallas_parallel_sum__ssm_conv_h3__dense_activation_silu__prompt_kernel(
    A_q: jax.Array,
    A_k: jax.Array,
    A_v: jax.Array,
    A_shift_k: jax.Array,
    A_ssm_k: jax.Array,
    A_ssm_D: jax.Array,
    B_x: jax.Array,
    B_w1: jax.Array,
    B_w2: jax.Array,
):
    del B_x
    qt = A_q.reshape(S, D).T
    kt = A_k.reshape(S, D).T
    vt = A_v.reshape(S, D).T
    sk = A_shift_k.T
    sd = A_ssm_D.reshape(1, D)
    w2t = B_w2.T
    dft_np, tw_np = _dft_tables()
    dft = jnp.asarray(dft_np)
    tw = jnp.asarray(tw_np)

    hbm = pl.BlockSpec(memory_space=pl.ANY)
    vmem = pl.BlockSpec(memory_space=pltpu.VMEM)
    in_specs = [hbm, hbm, hbm, vmem, hbm, vmem, hbm, hbm, vmem, vmem]
    bf = jnp.bfloat16
    scratch = [
        pltpu.VMEM((D, S), bf),
        pltpu.VMEM((D, S), bf),
        pltpu.VMEM((D, S), bf),
        pltpu.VMEM((D, S), bf),
        pltpu.VMEM((D, F), bf),
        pltpu.VMEM((D, F), bf),
        pltpu.VMEM((D, S), bf),
        pltpu.VMEM((NF1, 2 * NB, 2 * NB), bf),
        pltpu.VMEM((NF1, 2 * NB, 2 * NB), bf),
        pltpu.VMEM((F, DP), bf),
        pltpu.VMEM((D, 8), jnp.float32),
        pltpu.VMEM((D, S), jnp.float32),
        pltpu.VMEM((NF1, 2 * D, 2 * NB), jnp.float32),
        pltpu.VMEM((NF1, D, 2 * NB), jnp.float32),
        pltpu.VMEM((D, S), jnp.float32),
        pltpu.VMEM((2, FC, TB), bf),
        pltpu.VMEM((D, S), jnp.float32),
        pltpu.VMEM((DP, S), bf),
        pltpu.SemaphoreType.DMA((3 * 2 * (F // FC) + NTB + 2,)),
        pltpu.SemaphoreType.DMA((2,)),
    ]
    out = pl.pallas_call(
        _kernel,
        in_specs=in_specs,
        out_specs=hbm,
        out_shape=jax.ShapeDtypeStruct((D, S), bf),
        scratch_shapes=scratch,
        compiler_params=pltpu.CompilerParams(
            vmem_limit_bytes=100 * 1024 * 1024,
        ),
    )(qt, kt, vt, sk, A_ssm_k, sd, B_w1, w2t, dft, tw)
    return out.T.reshape(1, S, D)
```

```python
import math

import numpy as np
import jax
import jax.numpy as jnp
import jax.experimental.pallas as pl
import jax.experimental.pallas.tpu as pltpu

S = 2048
D = 448
F = 1792
L = 2 * S
NB = 128
NA = L // NB
NF1 = NA // 2 + 1
CR = 224
NCB = D // CR
TB = 512
NTB = S // TB
DP = 512
FC = 256
EPS = 1e-5


def _add(a, b):
    if a is None:
        return b
    if b is None:
        return a
    return a + b


def _sub(a, b):
    if b is None:
        return a
    if a is None:
        return -b
    return a - b


def _mulc(a, c):
    if a is None or c == 0.0:
        return None
    if c == 1.0:
        return a
    if c == -1.0:
        return -a
    return a * c


def _cmul_const(z, wr, wi):
    zr, zi = z
    if abs(wr) < 1e-12:
        wr = 0.0
    if abs(wi) < 1e-12:
        wi = 0.0
    if abs(abs(wr) - 1) < 1e-12:
        wr = math.copysign(1.0, wr)
    if abs(abs(wi) - 1) < 1e-12:
        wi = math.copysign(1.0, wi)
    re = _sub(_mulc(zr, wr), _mulc(zi, wi))
    im = _add(_mulc(zr, wi), _mulc(zi, wr))
    return (re, im)


def _rdft(x):
    n = len(x)
    if n == 1:
        return [(x[0], None)]
    if n == 2:
        return [(_add(x[0], x[1]), None), (_sub(x[0], x[1]), None)]
    e = _rdft(x[0::2])
    o = _rdft(x[1::2])
    out = [None] * (n // 2 + 1)
    for k in range(n // 4 + 1):
        t = _cmul_const(o[k], math.cos(2 * math.pi * k / n),
                        -math.sin(2 * math.pi * k / n))
        out[k] = (_add(e[k][0], t[0]), _add(e[k][1], t[1]))
        if n // 2 - k != k:
            out[n // 2 - k] = (_sub(e[k][0], t[0]), _sub(t[1], e[k][1]))
    return out


def _irdft(x, n, need):
    if n == 1:
        return [x[0][0]]
    if n == 2:
        out = [_add(x[0][0], x[1][0])]
        if need > 1:
            out.append(_sub(x[0][0], x[1][0]))
        return out
    e = [None] * (n // 4 + 1)
    o = [None] * (n // 4 + 1)
    for k in range(n // 4 + 1):
        a = x[k]
        b = x[n // 2 - k]
        e[k] = (_add(a[0], b[0]), _sub(a[1], b[1]))
        d = (_sub(a[0], b[0]), _add(a[1], b[1]))
        o[k] = _cmul_const(d, math.cos(2 * math.pi * k / n),
                           math.sin(2 * math.pi * k / n))
    ne = (need + 1) // 2
    no = need // 2
    xe = _irdft(e, n // 2, ne)
    xo = _irdft(o, n // 2, no) if no > 0 else []
    return [xe[i // 2] if i % 2 == 0 else xo[i // 2] for i in range(need)]


def _dft_tables():
    b = np.arange(NB)
    th = 2.0 * np.pi * ((b[:, None] * b[None, :]) % NB) / NB
    dft = np.stack([np.cos(th), np.sin(th)]).astype(np.float32)
    f1 = np.arange(NF1)
    th = 2.0 * np.pi * ((b[:, None] * f1[None, :]) % L) / L
    tw = np.zeros((2, NB, NB), np.float32)
    tw[0, :, :NF1] = np.cos(th)
    tw[1, :, :NF1] = np.sin(th)
    return dft, tw


def _kernel(q_hbm, k_hbm, v_hbm, sk_ref, hk_hbm, sd_ref, w1_hbm, w2_hbm,
            dft_ref, tw_ref, o_hbm,
            q_ref, k_ref, v_ref, hk_ref, w1_ref, w2_ref, o_ref,
            wf_ref, wi_ref, w1t_ref, par_ref, u_ref, g_ref, p_ref, y_ref,
            hb_ref, base_ref, xn_ref, sem, osem):
    f32 = jnp.float32
    bf16 = jnp.bfloat16
    NCH = F // FC
    NIT = 2 * NCH
    CPI = D // NIT
    RI = D // NCH

    def kvh_copies(i):
        rows = pl.ds(i * CPI, CPI)
        return [pltpu.make_async_copy(src.at[rows, :], dst.at[rows, :],
                                      sem.at[3 * i + j])
                for j, (src, dst) in enumerate(
                    ((k_hbm, k_ref), (v_hbm, v_ref), (hk_hbm, hk_ref)))]

    def q_copy(tb):
        cols = pl.ds(tb * TB, TB)
        return pltpu.make_async_copy(q_hbm.at[:, cols], q_ref.at[:, cols],
                                     sem.at[3 * NIT + tb])

    cp_w1 = pltpu.make_async_copy(w1_hbm, w1_ref, sem.at[3 * NIT + NTB])
    cp_w2 = pltpu.make_async_copy(w2_hbm, w2_ref, sem.at[3 * NIT + NTB + 1])
    WAITS = {0: range(0, 4), 4: range(4, 10), 10: range(10, NIT)}
    cp_w1.start()
    q_copy(0).start()
    cp_w2.start()
    for i in range(NIT):
        for cp in kvh_copies(i):
            cp.start()
        if i in (9, 13):
            q_copy(1 + (i - 9) // 4).start()
    q_copy(3).start()

    def tables():
        dc = dft_ref[0]
        ds_ = dft_ref[1]
        tc_all = tw_ref[0]
        ts_all = tw_ref[1]
        for f1 in range(NF1):
            tc = tc_all[:, f1:f1 + 1]
            ts = ts_all[:, f1:f1 + 1]
            c = tc * dc - ts * ds_
            s = ts * dc + tc * ds_
            wf_ref[f1, pl.ds(0, NB), pl.ds(0, NB)] = c.astype(bf16)
            wf_ref[f1, pl.ds(0, NB), pl.ds(NB, NB)] = (-s).astype(bf16)
            wf_ref[f1, pl.ds(NB, NB), pl.ds(0, NB)] = s.astype(bf16)
            wf_ref[f1, pl.ds(NB, NB), pl.ds(NB, NB)] = c.astype(bf16)
            ct = c.T * (1.0 / L)
            st = s.T * (1.0 / L)
            wi_ref[f1, pl.ds(0, NB), pl.ds(0, NB)] = ct.astype(bf16)
            wi_ref[f1, pl.ds(0, NB), pl.ds(NB, NB)] = st.astype(bf16)
            wi_ref[f1, pl.ds(NB, NB), pl.ds(0, NB)] = (-st).astype(bf16)
            wi_ref[f1, pl.ds(NB, NB), pl.ds(NB, NB)] = ct.astype(bf16)
        par = jnp.concatenate(
            [sk_ref[...].astype(f32), sd_ref[...].astype(f32),
             jnp.zeros((3, D), f32)], axis=0)
        par_ref[...] = par.T

    def kv_rows(r0, n):
        rows = pl.ds(r0, n)
        par = par_ref[rows, :]
        k = k_ref[rows, :].astype(f32)
        lane = jax.lax.broadcasted_iota(jnp.int32, (n, S), 1)
        ks = k * par[:, 0:1]
        for j in range(1, 4):
            kj = jnp.where(lane >= j, pltpu.roll(k, j, 1), 0.0)
            ks = ks + kj * par[:, j:j + 1]
        u_ref[rows, :] = ks * v_ref[rows, :].astype(f32)

    def s1_rows(src, r8, g8):
        xs = [src[pl.ds(r8, 8), pl.ds(NB * a, NB)].astype(f32)
              for a in range(NA // 2)]
        xs = xs + [None] * (NA // 2)
        g = _rdft(xs)
        for f1 in range(NF1):
            gr, gi = g[f1]
            if gi is None:
                gi = jnp.zeros((8, NB), f32)
            g_ref[f1, pl.ds(g8, 8), pl.ds(0, NB)] = gr
            g_ref[f1, pl.ds(g8, 8), pl.ds(NB, NB)] = gi
        return g[NF1 // 2][1]

    def spec_stage():
        for f1 in range(NF1):
            x = jnp.dot(g_ref[f1].astype(bf16), wf_ref[f1],
                        preferred_element_type=f32)
            xr, xi = x[:D, :NB], x[:D, NB:]
            hr, hi = x[D:, :NB], x[D:, NB:]
            yr = xr * hr - xi * hi
            yi = xr * hi + xi * hr
            yy = jnp.concatenate([yr, yi], axis=1).astype(bf16)
            p_ref[f1] = jnp.dot(yy, wi_ref[f1], preferred_element_type=f32)

    def i1_rows(r8):
        rows = pl.ds(r8, 8)
        xs = [(p_ref[f1, rows, pl.ds(0, NB)], p_ref[f1, rows, pl.ds(NB, NB)])
              for f1 in range(NF1)]
        y = _irdft(xs, NA, NA // 2)
        sd = par_ref[rows, :][:, 4:5]
        for a in range(NA // 2):
            col = pl.ds(NB * a, NB)
            yc = y[a].astype(bf16).astype(f32)
            tok = yc + u_ref[rows, col] * sd
            y_ref[rows, col] = tok
        return tok

    def layernorm(tb):
        cols = pl.ds(tb * TB, TB)
        x = q_ref[:, cols].astype(f32)
        mean = jnp.mean(x, axis=0, keepdims=True)
        xc = x - mean
        var = jnp.mean(xc * xc, axis=0, keepdims=True)
        xn = xc * jax.lax.rsqrt(var + EPS)
        xn_ref[pl.ds(0, D), cols] = xn.astype(bf16)
        base_ref[:, cols] = x

    def ffn_up(n):
        tb, i = divmod(n, NCH)
        h = jnp.dot(w1t_ref[pl.ds(i * FC, FC), :],
                    xn_ref[:, pl.ds(tb * TB, TB)],
                    preferred_element_type=f32)
        hh = 0.5 * h
        hb_ref[n % 2] = (hh + hh * jnp.tanh(hh)).astype(bf16)

    def ffn_down(n):
        tb, i = divmod(n, NCH)
        part = jnp.dot(w2_ref[:, pl.ds(i * FC, FC)], hb_ref[n % 2],
                       preferred_element_type=f32)
        cols = pl.ds(tb * TB, TB)
        base_ref[:, cols] = base_ref[:, cols] + part

    def combine(rows, cols):
        out = (base_ref[rows, cols]
               + xn_ref[rows, cols].astype(f32) * y_ref[rows, cols])
        o_ref[rows, cols] = out.astype(o_ref.dtype)
        return out[0:8, 0:NB]

    def order_before(tok, g, n):
        if n < NTB * NCH:
            tb = n // NCH
            xn_ref[pl.ds(D + 8 * g, 8), pl.ds(tb * TB, NB)] = tok.astype(bf16)

    def out_copy(rows, cols, s):
        return pltpu.make_async_copy(o_ref.at[rows, cols],
                                     o_hbm.at[rows, cols], osem.at[s])

    early = pl.ds(0, (NTB - 1) * TB)

    def extra(n):
        if n < NIT:
            kv_rows(n * CPI, CPI)
            for g in range(CPI // 8):
                r8 = n * CPI + g * 8
                order_before(s1_rows(u_ref, r8, r8), 2 * g, n + 1)
                order_before(s1_rows(hk_ref, r8, D + r8), 2 * g + 1, n + 1)
        elif n < NIT + NCH:
            i = n - NIT
            for g in range(RI // 8):
                order_before(i1_rows(i * RI + g * 8), g, n + 1)
        else:
            i = n - NIT - NCH
            rows = pl.ds(i * RI, RI)
            order_before(combine(rows, early), 0, n + 1)
            out_copy(rows, early, 0).start()

    with jax.named_scope("tables"):
        tables()
        xn_ref[pl.ds(D, DP - D), :] = jnp.zeros((DP - D, S), bf16)
        w1t_ref[:, pl.ds(D, DP - D)] = jnp.zeros((F, DP - D), bf16)
    with jax.named_scope("pro"):
        cp_w1.wait()
        w1t_ref[:, pl.ds(0, D)] = w1_ref[...].astype(f32).T.astype(bf16)
        q_copy(0).wait()
        layernorm(0)
        ffn_up(0)
        cp_w2.wait()

    for n in range(NTB * NCH):
        for i in WAITS.get(n, ()):
            for cp in kvh_copies(i):
                cp.wait()
        if n == 4:
            q_copy(1).wait()
            layernorm(1)
        if n == 10:
            q_copy(2).wait()
            layernorm(2)
        if n == NIT:
            spec_stage()
            q_copy(3).wait()
            layernorm(3)
        extra(n)
        if n + 1 < NTB * NCH:
            ffn_up(n + 1)
        ffn_down(n)

    with jax.named_scope("fin"):
        late = pl.ds((NTB - 1) * TB, TB)
        combine(pl.ds(0, D), late)
        cp_late = out_copy(pl.ds(0, D), late, 1)
        cp_late.start()
        out_copy(pl.ds(0, D), early, 0).wait()
        cp_late.wait()


@jax.jit
def pallas_parallel_sum__ssm_conv_h3__dense_activation_silu__prompt_kernel(
    A_q: jax.Array,
    A_k: jax.Array,
    A_v: jax.Array,
    A_shift_k: jax.Array,
    A_ssm_k: jax.Array,
    A_ssm_D: jax.Array,
    B_x: jax.Array,
    B_w1: jax.Array,
    B_w2: jax.Array,
):
    del B_x
    qt = A_q.reshape(S, D).T
    kt = A_k.reshape(S, D).T
    vt = A_v.reshape(S, D).T
    sk = A_shift_k.T
    sd = A_ssm_D.reshape(1, D)
    w2t = B_w2.T
    dft_np, tw_np = _dft_tables()
    dft = jnp.asarray(dft_np)
    tw = jnp.asarray(tw_np)

    hbm = pl.BlockSpec(memory_space=pl.ANY)
    vmem = pl.BlockSpec(memory_space=pltpu.VMEM)
    in_specs = [hbm, hbm, hbm, vmem, hbm, vmem, hbm, hbm, vmem, vmem]
    bf = jnp.bfloat16
    scratch = [
        pltpu.VMEM((D, S), bf),
        pltpu.VMEM((D, S), bf),
        pltpu.VMEM((D, S), bf),
        pltpu.VMEM((D, S), bf),
        pltpu.VMEM((D, F), bf),
        pltpu.VMEM((D, F), bf),
        pltpu.VMEM((D, S), bf),
        pltpu.VMEM((NF1, 2 * NB, 2 * NB), bf),
        pltpu.VMEM((NF1, 2 * NB, 2 * NB), bf),
        pltpu.VMEM((F, DP), bf),
        pltpu.VMEM((D, 8), jnp.float32),
        pltpu.VMEM((D, S), jnp.float32),
        pltpu.VMEM((NF1, 2 * D, 2 * NB), jnp.float32),
        pltpu.VMEM((NF1, D, 2 * NB), jnp.float32),
        pltpu.VMEM((D, S), jnp.float32),
        pltpu.VMEM((2, FC, TB), bf),
        pltpu.VMEM((D, S), jnp.float32),
        pltpu.VMEM((DP, S), bf),
        pltpu.SemaphoreType.DMA((3 * 2 * (F // FC) + NTB + 2,)),
        pltpu.SemaphoreType.DMA((2,)),
    ]
    out = pl.pallas_call(
        _kernel,
        in_specs=in_specs,
        out_specs=hbm,
        out_shape=jax.ShapeDtypeStruct((D, S), bf),
        scratch_shapes=scratch,
        compiler_params=pltpu.CompilerParams(
            vmem_limit_bytes=100 * 1024 * 1024,
        ),
    )(qt, kt, vt, sk, A_ssm_k, sd, B_w1, w2t, dft, tw)
    return out.T.reshape(1, S, D)
```

```python
import math

import numpy as np
import jax
import jax.numpy as jnp
import jax.experimental.pallas as pl
import jax.experimental.pallas.tpu as pltpu

S = 2048
D = 448
F = 1792
L = 2 * S
NB = 128
NA = L // NB
NF1 = NA // 2 + 1
CR = 224
NCB = D // CR
TB = 512
NTB = S // TB
DP = 512
FC = 256
EPS = 1e-5


def _add(a, b):
    if a is None:
        return b
    if b is None:
        return a
    return a + b


def _sub(a, b):
    if b is None:
        return a
    if a is None:
        return -b
    return a - b


def _mulc(a, c):
    if a is None or c == 0.0:
        return None
    if c == 1.0:
        return a
    if c == -1.0:
        return -a
    return a * c


def _cmul_const(z, wr, wi):
    zr, zi = z
    if abs(wr) < 1e-12:
        wr = 0.0
    if abs(wi) < 1e-12:
        wi = 0.0
    if abs(abs(wr) - 1) < 1e-12:
        wr = math.copysign(1.0, wr)
    if abs(abs(wi) - 1) < 1e-12:
        wi = math.copysign(1.0, wi)
    re = _sub(_mulc(zr, wr), _mulc(zi, wi))
    im = _add(_mulc(zr, wi), _mulc(zi, wr))
    return (re, im)


def _rdft(x):
    n = len(x)
    if n == 1:
        return [(x[0], None)]
    if n == 2:
        return [(_add(x[0], x[1]), None), (_sub(x[0], x[1]), None)]
    e = _rdft(x[0::2])
    o = _rdft(x[1::2])
    out = [None] * (n // 2 + 1)
    for k in range(n // 4 + 1):
        t = _cmul_const(o[k], math.cos(2 * math.pi * k / n),
                        -math.sin(2 * math.pi * k / n))
        out[k] = (_add(e[k][0], t[0]), _add(e[k][1], t[1]))
        if n // 2 - k != k:
            out[n // 2 - k] = (_sub(e[k][0], t[0]), _sub(t[1], e[k][1]))
    return out


def _irdft(x, n, need):
    if n == 1:
        return [x[0][0]]
    if n == 2:
        out = [_add(x[0][0], x[1][0])]
        if need > 1:
            out.append(_sub(x[0][0], x[1][0]))
        return out
    e = [None] * (n // 4 + 1)
    o = [None] * (n // 4 + 1)
    for k in range(n // 4 + 1):
        a = x[k]
        b = x[n // 2 - k]
        e[k] = (_add(a[0], b[0]), _sub(a[1], b[1]))
        d = (_sub(a[0], b[0]), _add(a[1], b[1]))
        o[k] = _cmul_const(d, math.cos(2 * math.pi * k / n),
                           math.sin(2 * math.pi * k / n))
    ne = (need + 1) // 2
    no = need // 2
    xe = _irdft(e, n // 2, ne)
    xo = _irdft(o, n // 2, no) if no > 0 else []
    return [xe[i // 2] if i % 2 == 0 else xo[i // 2] for i in range(need)]


def _dft_tables():
    b = np.arange(NB)
    fwd = np.zeros((NF1, 2 * NB, 2 * NB), np.float64)
    inv = np.zeros((NF1, 2 * NB, 2 * NB), np.float64)
    for f1 in range(NF1):
        f = f1 + NA * b
        th = 2.0 * np.pi * ((b[:, None] * f[None, :]) % L) / L
        c, s = np.cos(th), np.sin(th)
        fwd[f1] = np.block([[c, -s], [s, c]])
        inv[f1] = np.block([[c.T, s.T], [-s.T, c.T]]) / L
    return fwd.astype(np.float32), inv.astype(np.float32)


def _kernel(q_hbm, k_hbm, v_hbm, sk_ref, hk_hbm, sd_ref, w1_hbm, w2_hbm,
            wf_hbm, wi_hbm, o_hbm,
            q_ref, k_ref, v_ref, hk_ref, w1_ref, w2_ref, o_ref,
            wf_ref, wi_ref, w1t_ref, par_ref, u_ref, g_ref, p_ref, y_ref,
            hb_ref, base_ref, xn_ref, sem, osem):
    f32 = jnp.float32
    bf16 = jnp.bfloat16
    NCH = F // FC
    NIT = 2 * NCH
    CPI = D // NIT
    RI = D // NCH

    def kvh_copies(i):
        rows = pl.ds(i * CPI, CPI)
        return [pltpu.make_async_copy(src.at[rows, :], dst.at[rows, :],
                                      sem.at[3 * i + j])
                for j, (src, dst) in enumerate(
                    ((k_hbm, k_ref), (v_hbm, v_ref), (hk_hbm, hk_ref)))]

    def q_copy(tb):
        cols = pl.ds(tb * TB, TB)
        return pltpu.make_async_copy(q_hbm.at[:, cols], q_ref.at[:, cols],
                                     sem.at[3 * NIT + tb])

    cp_w1 = pltpu.make_async_copy(w1_hbm, w1_ref, sem.at[3 * NIT + NTB])
    cp_w2 = pltpu.make_async_copy(w2_hbm, w2_ref, sem.at[3 * NIT + NTB + 1])
    cp_wf = pltpu.make_async_copy(wf_hbm, wf_ref, sem.at[3 * NIT + NTB + 2])
    cp_wi = pltpu.make_async_copy(wi_hbm, wi_ref, sem.at[3 * NIT + NTB + 3])
    PRE = 2
    WAITS = {0: range(2, 6), 4: range(6, 10), 8: range(10, NIT)}
    for i in range(NIT):
        for cp in kvh_copies(i):
            cp.start()
        if i == 1:
            cp_w1.start()
            q_copy(0).start()
        if i == 3:
            cp_w2.start()
        if i == 9:
            q_copy(1).start()
    q_copy(2).start()
    cp_wf.start()
    cp_wi.start()
    q_copy(3).start()

    def params():
        par = jnp.concatenate(
            [sk_ref[...].astype(f32), sd_ref[...].astype(f32),
             jnp.zeros((3, D), f32)], axis=0)
        par_ref[...] = par.T

    def kv_rows(r0, n):
        rows = pl.ds(r0, n)
        par = par_ref[rows, :]
        k = k_ref[rows, :].astype(f32)
        lane = jax.lax.broadcasted_iota(jnp.int32, (n, S), 1)
        ks = k * par[:, 0:1]
        for j in range(1, 4):
            kj = jnp.where(lane >= j, pltpu.roll(k, j, 1), 0.0)
            ks = ks + kj * par[:, j:j + 1]
        u_ref[rows, :] = ks * v_ref[rows, :].astype(f32)

    def s1_rows(src, r8, g8):
        xs = [src[pl.ds(r8, 8), pl.ds(NB * a, NB)].astype(f32)
              for a in range(NA // 2)]
        xs = xs + [None] * (NA // 2)
        g = _rdft(xs)
        for f1 in range(NF1):
            gr, gi = g[f1]
            if gi is None:
                gi = jnp.zeros((8, NB), f32)
            g_ref[f1, pl.ds(g8, 8), pl.ds(0, NB)] = gr
            g_ref[f1, pl.ds(g8, 8), pl.ds(NB, NB)] = gi
        return g[NF1 // 2][1]

    def spec_stage():
        for f1 in range(NF1):
            x = jnp.dot(g_ref[f1].astype(bf16), wf_ref[f1],
                        preferred_element_type=f32)
            xr, xi = x[:D, :NB], x[:D, NB:]
            hr, hi = x[D:, :NB], x[D:, NB:]
            yr = xr * hr - xi * hi
            yi = xr * hi + xi * hr
            yy = jnp.concatenate([yr, yi], axis=1).astype(bf16)
            p_ref[f1] = jnp.dot(yy, wi_ref[f1], preferred_element_type=f32)

    def i1_rows(r8):
        rows = pl.ds(r8, 8)
        xs = [(p_ref[f1, rows, pl.ds(0, NB)], p_ref[f1, rows, pl.ds(NB, NB)])
              for f1 in range(NF1)]
        y = _irdft(xs, NA, NA // 2)
        sd = par_ref[rows, :][:, 4:5]
        for a in range(NA // 2):
            col = pl.ds(NB * a, NB)
            yc = y[a].astype(bf16).astype(f32)
            tok = yc + u_ref[rows, col] * sd
            y_ref[rows, col] = tok
        return tok

    def layernorm(tb):
        cols = pl.ds(tb * TB, TB)
        x = q_ref[:, cols].astype(f32)
        mean = jnp.mean(x, axis=0, keepdims=True)
        xc = x - mean
        var = jnp.mean(xc * xc, axis=0, keepdims=True)
        xn = xc * jax.lax.rsqrt(var + EPS)
        xn_ref[pl.ds(0, D), cols] = xn.astype(bf16)
        base_ref[:, cols] = x

    def ffn_up(n):
        tb, i = divmod(n, NCH)
        h = jnp.dot(w1t_ref[pl.ds(i * FC, FC), :],
                    xn_ref[:, pl.ds(tb * TB, TB)],
                    preferred_element_type=f32)
        hh = 0.5 * h
        hb_ref[n % 2] = (hh + hh * jnp.tanh(hh)).astype(bf16)

    def ffn_down(n):
        tb, i = divmod(n, NCH)
        part = jnp.dot(w2_ref[:, pl.ds(i * FC, FC)], hb_ref[n % 2],
                       preferred_element_type=f32)
        cols = pl.ds(tb * TB, TB)
        base_ref[:, cols] = base_ref[:, cols] + part

    def combine(rows, cols):
        out = (base_ref[rows, cols]
               + xn_ref[rows, cols].astype(f32) * y_ref[rows, cols])
        o_ref[rows, cols] = out.astype(o_ref.dtype)
        return out[0:8, 0:NB]

    def order_before(tok, g, n):
        if n < NTB * NCH:
            tb = n // NCH
            xn_ref[pl.ds(D + 8 * g, 8), pl.ds(tb * TB, NB)] = tok.astype(bf16)

    def out_copy(rows, cols, s):
        return pltpu.make_async_copy(o_ref.at[rows, cols],
                                     o_hbm.at[rows, cols], osem.at[s])

    def fwd_slot(i, n):
        kv_rows(i * CPI, CPI)
        for g in range(CPI // 8):
            r8 = i * CPI + g * 8
            order_before(s1_rows(u_ref, r8, r8), 2 * g, n)
            order_before(s1_rows(hk_ref, r8, D + r8), 2 * g + 1, n)

    N_S1 = NIT - PRE
    N_I1 = N_S1 + NCH
    N_C01 = (NTB - 1) * NCH + 1
    first2 = pl.ds(0, 2 * TB)
    third = pl.ds(2 * TB, TB)

    def row_part(j, parts):
        units = D // 16
        lo = (units * j // parts) * 16
        hi = (units * (j + 1) // parts) * 16
        return pl.ds(lo, hi - lo)

    def extra(n):
        if n < N_S1:
            fwd_slot(n + PRE, n + 1)
        elif n < N_I1:
            i = n - N_S1
            for g in range(RI // 8):
                order_before(i1_rows(i * RI + g * 8), g, n + 1)
        elif n < N_C01:
            rows = row_part(n - N_I1, N_C01 - N_I1)
            order_before(combine(rows, first2), 0, n + 1)
            out_copy(rows, first2, 0).start()
        else:
            rows = row_part(n - N_C01, NTB * NCH - N_C01)
            order_before(combine(rows, third), 0, n + 1)
            out_copy(rows, third, 1).start()

    with jax.named_scope("pro"):
        params()
        xn_ref[pl.ds(D, DP - D), :] = jnp.zeros((DP - D, S), bf16)
        w1t_ref[:, pl.ds(D, DP - D)] = jnp.zeros((F, DP - D), bf16)
        for i in range(PRE):
            for cp in kvh_copies(i):
                cp.wait()
            fwd_slot(i, NTB * NCH)
        cp_w1.wait()
        w1t_ref[:, pl.ds(0, D)] = w1_ref[...].astype(f32).T.astype(bf16)
        q_copy(0).wait()
        layernorm(0)
        ffn_up(0)
        cp_w2.wait()

    for n in range(NTB * NCH):
        for i in WAITS.get(n, ()):
            for cp in kvh_copies(i):
                cp.wait()
        if n == 4:
            q_copy(1).wait()
            layernorm(1)
        if n == 8:
            q_copy(2).wait()
            layernorm(2)
        if n == N_S1:
            cp_wf.wait()
            cp_wi.wait()
            q_copy(3).wait()
            spec_stage()
            layernorm(3)
        extra(n)
        if n + 1 < NTB * NCH:
            ffn_up(n + 1)
        ffn_down(n)

    with jax.named_scope("fin"):
        late = pl.ds((NTB - 1) * TB, TB)
        combine(pl.ds(0, D), late)
        cp_late = out_copy(pl.ds(0, D), late, 2)
        cp_late.start()
        out_copy(pl.ds(0, D), first2, 0).wait()
        out_copy(pl.ds(0, D), third, 1).wait()
        cp_late.wait()


@jax.jit
def pallas_parallel_sum__ssm_conv_h3__dense_activation_silu__prompt_kernel(
    A_q: jax.Array,
    A_k: jax.Array,
    A_v: jax.Array,
    A_shift_k: jax.Array,
    A_ssm_k: jax.Array,
    A_ssm_D: jax.Array,
    B_x: jax.Array,
    B_w1: jax.Array,
    B_w2: jax.Array,
):
    del B_x
    qt = A_q.reshape(S, D).T
    kt = A_k.reshape(S, D).T
    vt = A_v.reshape(S, D).T
    sk = A_shift_k.T
    sd = A_ssm_D.reshape(1, D)
    w2t = B_w2.T
    wf_np, wi_np = _dft_tables()
    wf = jnp.asarray(wf_np, dtype=jnp.bfloat16)
    wi = jnp.asarray(wi_np, dtype=jnp.bfloat16)

    hbm = pl.BlockSpec(memory_space=pl.ANY)
    vmem = pl.BlockSpec(memory_space=pltpu.VMEM)
    in_specs = [hbm, hbm, hbm, vmem, hbm, vmem, hbm, hbm, hbm, hbm]
    bf = jnp.bfloat16
    scratch = [
        pltpu.VMEM((D, S), bf),
        pltpu.VMEM((D, S), bf),
        pltpu.VMEM((D, S), bf),
        pltpu.VMEM((D, S), bf),
        pltpu.VMEM((D, F), bf),
        pltpu.VMEM((D, F), bf),
        pltpu.VMEM((D, S), bf),
        pltpu.VMEM((NF1, 2 * NB, 2 * NB), bf),
        pltpu.VMEM((NF1, 2 * NB, 2 * NB), bf),
        pltpu.VMEM((F, DP), bf),
        pltpu.VMEM((D, 8), jnp.float32),
        pltpu.VMEM((D, S), jnp.float32),
        pltpu.VMEM((NF1, 2 * D, 2 * NB), jnp.float32),
        pltpu.VMEM((NF1, D, 2 * NB), jnp.float32),
        pltpu.VMEM((D, S), jnp.float32),
        pltpu.VMEM((2, FC, TB), bf),
        pltpu.VMEM((D, S), jnp.float32),
        pltpu.VMEM((DP, S), bf),
        pltpu.SemaphoreType.DMA((3 * 2 * (F // FC) + NTB + 4,)),
        pltpu.SemaphoreType.DMA((3,)),
    ]
    out = pl.pallas_call(
        _kernel,
        in_specs=in_specs,
        out_specs=hbm,
        out_shape=jax.ShapeDtypeStruct((D, S), bf),
        scratch_shapes=scratch,
        compiler_params=pltpu.CompilerParams(
            vmem_limit_bytes=100 * 1024 * 1024,
        ),
    )(qt, kt, vt, sk, A_ssm_k, sd, B_w1, w2t, wf, wi)
    return out.T.reshape(1, S, D)
```

```python
import math

import numpy as np
import jax
import jax.numpy as jnp
import jax.experimental.pallas as pl
import jax.experimental.pallas.tpu as pltpu

S = 2048
D = 448
F = 1792
L = 2 * S
NB = 128
NA = L // NB
NF1 = NA // 2 + 1
CR = 224
NCB = D // CR
TB = 512
NTB = S // TB
DP = 512
FC = 256
EPS = 1e-5


def _add(a, b):
    if a is None:
        return b
    if b is None:
        return a
    return a + b


def _sub(a, b):
    if b is None:
        return a
    if a is None:
        return -b
    return a - b


def _mulc(a, c):
    if a is None or c == 0.0:
        return None
    if c == 1.0:
        return a
    if c == -1.0:
        return -a
    return a * c


def _cmul_const(z, wr, wi):
    zr, zi = z
    if abs(wr) < 1e-12:
        wr = 0.0
    if abs(wi) < 1e-12:
        wi = 0.0
    if abs(abs(wr) - 1) < 1e-12:
        wr = math.copysign(1.0, wr)
    if abs(abs(wi) - 1) < 1e-12:
        wi = math.copysign(1.0, wi)
    re = _sub(_mulc(zr, wr), _mulc(zi, wi))
    im = _add(_mulc(zr, wi), _mulc(zi, wr))
    return (re, im)


def _rdft(x):
    n = len(x)
    if n == 1:
        return [(x[0], None)]
    if n == 2:
        return [(_add(x[0], x[1]), None), (_sub(x[0], x[1]), None)]
    e = _rdft(x[0::2])
    o = _rdft(x[1::2])
    out = [None] * (n // 2 + 1)
    for k in range(n // 4 + 1):
        t = _cmul_const(o[k], math.cos(2 * math.pi * k / n),
                        -math.sin(2 * math.pi * k / n))
        out[k] = (_add(e[k][0], t[0]), _add(e[k][1], t[1]))
        if n // 2 - k != k:
            out[n // 2 - k] = (_sub(e[k][0], t[0]), _sub(t[1], e[k][1]))
    return out


def _irdft(x, n, need):
    if n == 1:
        return [x[0][0]]
    if n == 2:
        out = [_add(x[0][0], x[1][0])]
        if need > 1:
            out.append(_sub(x[0][0], x[1][0]))
        return out
    e = [None] * (n // 4 + 1)
    o = [None] * (n // 4 + 1)
    for k in range(n // 4 + 1):
        a = x[k]
        b = x[n // 2 - k]
        e[k] = (_add(a[0], b[0]), _sub(a[1], b[1]))
        d = (_sub(a[0], b[0]), _add(a[1], b[1]))
        o[k] = _cmul_const(d, math.cos(2 * math.pi * k / n),
                           math.sin(2 * math.pi * k / n))
    ne = (need + 1) // 2
    no = need // 2
    xe = _irdft(e, n // 2, ne)
    xo = _irdft(o, n // 2, no) if no > 0 else []
    return [xe[i // 2] if i % 2 == 0 else xo[i // 2] for i in range(need)]


def _dft_tables():
    b = np.arange(NB)
    fwd = np.zeros((NF1, 2 * NB, 2 * NB), np.float64)
    inv = np.zeros((NF1, 2 * NB, 2 * NB), np.float64)
    for f1 in range(NF1):
        f = f1 + NA * b
        th = 2.0 * np.pi * ((b[:, None] * f[None, :]) % L) / L
        c, s = np.cos(th), np.sin(th)
        fwd[f1] = np.block([[c, -s], [s, c]])
        inv[f1] = np.block([[c.T, s.T], [-s.T, c.T]]) / L
    return fwd.astype(np.float32), inv.astype(np.float32)


def _kernel(q_hbm, k_hbm, v_hbm, sk_ref, hk_hbm, sd_ref, w1_hbm, w2_hbm,
            wf_hbm, wi_hbm, o_hbm,
            q_ref, k_ref, v_ref, hk_ref, w1_ref, w2_ref, o_ref,
            wf_ref, wi_ref, w1t_ref, par_ref, u_ref, g_ref, p_ref, y_ref,
            hb_ref, base_ref, xn_ref, sem, osem):
    f32 = jnp.float32
    bf16 = jnp.bfloat16
    NCH = F // FC
    NIT = 2 * NCH
    CPI = D // NIT
    RI = D // NCH

    def kvh_copies(i):
        rows = pl.ds(i * CPI, CPI)
        return [pltpu.make_async_copy(src.at[rows, :], dst.at[rows, :],
                                      sem.at[3 * i + j])
                for j, (src, dst) in enumerate(
                    ((k_hbm, k_ref), (v_hbm, v_ref), (hk_hbm, hk_ref)))]

    def q_copy(tb):
        cols = pl.ds(tb * TB, TB)
        return pltpu.make_async_copy(q_hbm.at[:, cols], q_ref.at[:, cols],
                                     sem.at[3 * NIT + tb])

    cp_w1 = pltpu.make_async_copy(w1_hbm, w1_ref, sem.at[3 * NIT + NTB])
    cp_w2 = pltpu.make_async_copy(w2_hbm, w2_ref, sem.at[3 * NIT + NTB + 1])
    cp_wf = pltpu.make_async_copy(wf_hbm, wf_ref, sem.at[3 * NIT + NTB + 2])
    cp_wi = pltpu.make_async_copy(wi_hbm, wi_ref, sem.at[3 * NIT + NTB + 3])
    PRE = 2
    WAITS = {0: range(2, 6), 4: range(6, 10), 8: range(10, NIT)}

    def start_kvh(rng):
        for i in rng:
            for cp in kvh_copies(i):
                cp.start()

    start_kvh(range(PRE))
    cp_w1.start()
    q_copy(0).start()

    def params():
        par = jnp.concatenate(
            [sk_ref[...].astype(f32), sd_ref[...].astype(f32),
             jnp.zeros((3, D), f32)], axis=0)
        par_ref[...] = par.T

    def kv_rows(r0, n):
        rows = pl.ds(r0, n)
        par = par_ref[rows, :]
        k = k_ref[rows, :].astype(f32)
        lane = jax.lax.broadcasted_iota(jnp.int32, (n, S), 1)
        ks = k * par[:, 0:1]
        for j in range(1, 4):
            kj = jnp.where(lane >= j, pltpu.roll(k, j, 1), 0.0)
            ks = ks + kj * par[:, j:j + 1]
        u_ref[rows, :] = ks * v_ref[rows, :].astype(f32)

    def s1_rows(src, r8, g8):
        xs = [src[pl.ds(r8, 8), pl.ds(NB * a, NB)].astype(f32)
              for a in range(NA // 2)]
        xs = xs + [None] * (NA // 2)
        g = _rdft(xs)
        for f1 in range(NF1):
            gr, gi = g[f1]
            if gi is None:
                gi = jnp.zeros((8, NB), f32)
            g_ref[f1, pl.ds(g8, 8), pl.ds(0, NB)] = gr
            g_ref[f1, pl.ds(g8, 8), pl.ds(NB, NB)] = gi
        return g[NF1 // 2][1]

    def spec_stage():
        for f1 in range(NF1):
            x = jnp.dot(g_ref[f1].astype(bf16), wf_ref[f1],
                        preferred_element_type=f32)
            xr, xi = x[:D, :NB], x[:D, NB:]
            hr, hi = x[D:, :NB], x[D:, NB:]
            yr = xr * hr - xi * hi
            yi = xr * hi + xi * hr
            yy = jnp.concatenate([yr, yi], axis=1).astype(bf16)
            p_ref[f1] = jnp.dot(yy, wi_ref[f1], preferred_element_type=f32)

    def i1_rows(r8):
        rows = pl.ds(r8, 8)
        xs = [(p_ref[f1, rows, pl.ds(0, NB)], p_ref[f1, rows, pl.ds(NB, NB)])
              for f1 in range(NF1)]
        y = _irdft(xs, NA, NA // 2)
        sd = par_ref[rows, :][:, 4:5]
        for a in range(NA // 2):
            col = pl.ds(NB * a, NB)
            yc = y[a].astype(bf16).astype(f32)
            tok = yc + u_ref[rows, col] * sd
            y_ref[rows, col] = tok
        return tok

    def layernorm(tb):
        cols = pl.ds(tb * TB, TB)
        x = q_ref[:, cols].astype(f32)
        mean = jnp.mean(x, axis=0, keepdims=True)
        xc = x - mean
        var = jnp.mean(xc * xc, axis=0, keepdims=True)
        xn = xc * jax.lax.rsqrt(var + EPS)
        xn_ref[pl.ds(0, D), cols] = xn.astype(bf16)
        base_ref[:, cols] = x

    def ffn_up(n):
        tb, i = divmod(n, NCH)
        h = jnp.dot(w1t_ref[pl.ds(i * FC, FC), :],
                    xn_ref[:, pl.ds(tb * TB, TB)],
                    preferred_element_type=f32)
        hh = 0.5 * h
        hb_ref[n % 2] = (hh + hh * jnp.tanh(hh)).astype(bf16)

    def ffn_down(n):
        tb, i = divmod(n, NCH)
        part = jnp.dot(w2_ref[:, pl.ds(i * FC, FC)], hb_ref[n % 2],
                       preferred_element_type=f32)
        cols = pl.ds(tb * TB, TB)
        base_ref[:, cols] = base_ref[:, cols] + part

    def combine(rows, cols):
        out = (base_ref[rows, cols]
               + xn_ref[rows, cols].astype(f32) * y_ref[rows, cols])
        o_ref[rows, cols] = out.astype(o_ref.dtype)
        return out[0:8, 0:NB]

    def order_before(tok, g, n):
        if n < NTB * NCH:
            tb = n // NCH
            xn_ref[pl.ds(D + 8 * g, 8), pl.ds(tb * TB, NB)] = tok.astype(bf16)

    def out_copy(rows, cols, s):
        return pltpu.make_async_copy(o_ref.at[rows, cols],
                                     o_hbm.at[rows, cols], osem.at[s])

    def fwd_slot(i, n):
        kv_rows(i * CPI, CPI)
        for g in range(CPI // 8):
            r8 = i * CPI + g * 8
            order_before(s1_rows(u_ref, r8, r8), 2 * g, n)
            order_before(s1_rows(hk_ref, r8, D + r8), 2 * g + 1, n)

    N_S1 = NIT - PRE
    N_I1 = N_S1 + NCH
    N_C01 = (NTB - 1) * NCH + 1
    first2 = pl.ds(0, 2 * TB)
    third = pl.ds(2 * TB, TB)

    def row_part(j, parts):
        units = D // 16
        lo = (units * j // parts) * 16
        hi = (units * (j + 1) // parts) * 16
        return pl.ds(lo, hi - lo)

    def extra(n):
        if n < N_S1:
            fwd_slot(n + PRE, n + 1)
        elif n < N_I1:
            i = n - N_S1
            for g in range(RI // 8):
                order_before(i1_rows(i * RI + g * 8), g, n + 1)
        elif n < N_C01:
            rows = row_part(n - N_I1, N_C01 - N_I1)
            order_before(combine(rows, first2), 0, n + 1)
            out_copy(rows, first2, 0).start()
        else:
            rows = row_part(n - N_C01, NTB * NCH - N_C01)
            order_before(combine(rows, third), 0, n + 1)
            out_copy(rows, third, 1).start()

    with jax.named_scope("pro"):
        params()
        xn_ref[pl.ds(D, DP - D), :] = jnp.zeros((DP - D, S), bf16)
        w1t_ref[:, pl.ds(D, DP - D)] = jnp.zeros((F, DP - D), bf16)
        for i in range(PRE):
            for cp in kvh_copies(i):
                cp.wait()
            fwd_slot(i, NTB * NCH)
        cp_w1.wait()
        cp_w2.start()
        start_kvh(WAITS[0])
        w1t_ref[:, pl.ds(0, D)] = w1_ref[...].astype(f32).T.astype(bf16)
        q_copy(0).wait()
        layernorm(0)
        ffn_up(0)
        cp_w2.wait()

    for n in range(NTB * NCH):
        for i in WAITS.get(n, ()):
            for cp in kvh_copies(i):
                cp.wait()
        if n == 0:
            start_kvh(WAITS[4])
            q_copy(1).start()
        if n == 4:
            start_kvh(WAITS[8])
            q_copy(2).start()
            q_copy(1).wait()
            layernorm(1)
        if n == 8:
            cp_wf.start()
            cp_wi.start()
            q_copy(3).start()
            q_copy(2).wait()
            layernorm(2)
        if n == N_S1:
            cp_wf.wait()
            cp_wi.wait()
            q_copy(3).wait()
            spec_stage()
            layernorm(3)
        extra(n)
        if n + 1 < NTB * NCH:
            ffn_up(n + 1)
        ffn_down(n)

    with jax.named_scope("fin"):
        late = pl.ds((NTB - 1) * TB, TB)
        combine(pl.ds(0, D), late)
        cp_late = out_copy(pl.ds(0, D), late, 2)
        cp_late.start()
        out_copy(pl.ds(0, D), first2, 0).wait()
        out_copy(pl.ds(0, D), third, 1).wait()
        cp_late.wait()


@jax.jit
def pallas_parallel_sum__ssm_conv_h3__dense_activation_silu__prompt_kernel(
    A_q: jax.Array,
    A_k: jax.Array,
    A_v: jax.Array,
    A_shift_k: jax.Array,
    A_ssm_k: jax.Array,
    A_ssm_D: jax.Array,
    B_x: jax.Array,
    B_w1: jax.Array,
    B_w2: jax.Array,
):
    del B_x
    qt = A_q.reshape(S, D).T
    kt = A_k.reshape(S, D).T
    vt = A_v.reshape(S, D).T
    sk = A_shift_k.T
    sd = A_ssm_D.reshape(1, D)
    w2t = B_w2.T
    wf_np, wi_np = _dft_tables()
    wf = jnp.asarray(wf_np, dtype=jnp.bfloat16)
    wi = jnp.asarray(wi_np, dtype=jnp.bfloat16)

    hbm = pl.BlockSpec(memory_space=pl.ANY)
    vmem = pl.BlockSpec(memory_space=pltpu.VMEM)
    in_specs = [hbm, hbm, hbm, vmem, hbm, vmem, hbm, hbm, hbm, hbm]
    bf = jnp.bfloat16
    scratch = [
        pltpu.VMEM((D, S), bf),
        pltpu.VMEM((D, S), bf),
        pltpu.VMEM((D, S), bf),
        pltpu.VMEM((D, S), bf),
        pltpu.VMEM((D, F), bf),
        pltpu.VMEM((D, F), bf),
        pltpu.VMEM((D, S), bf),
        pltpu.VMEM((NF1, 2 * NB, 2 * NB), bf),
        pltpu.VMEM((NF1, 2 * NB, 2 * NB), bf),
        pltpu.VMEM((F, DP), bf),
        pltpu.VMEM((D, 8), jnp.float32),
        pltpu.VMEM((D, S), jnp.float32),
        pltpu.VMEM((NF1, 2 * D, 2 * NB), jnp.float32),
        pltpu.VMEM((NF1, D, 2 * NB), jnp.float32),
        pltpu.VMEM((D, S), jnp.float32),
        pltpu.VMEM((2, FC, TB), bf),
        pltpu.VMEM((D, S), jnp.float32),
        pltpu.VMEM((DP, S), bf),
        pltpu.SemaphoreType.DMA((3 * 2 * (F // FC) + NTB + 4,)),
        pltpu.SemaphoreType.DMA((3,)),
    ]
    out = pl.pallas_call(
        _kernel,
        in_specs=in_specs,
        out_specs=hbm,
        out_shape=jax.ShapeDtypeStruct((D, S), bf),
        scratch_shapes=scratch,
        compiler_params=pltpu.CompilerParams(
            vmem_limit_bytes=100 * 1024 * 1024,
        ),
    )(qt, kt, vt, sk, A_ssm_k, sd, B_w1, w2t, wf, wi)
    return out.T.reshape(1, S, D)
```

```python
import math

import numpy as np
import jax
import jax.numpy as jnp
import jax.experimental.pallas as pl
import jax.experimental.pallas.tpu as pltpu

S = 2048
D = 448
F = 1792
L = 2 * S
NB = 128
NA = L // NB
NF1 = NA // 2 + 1
CR = 224
NCB = D // CR
TB = 512
NTB = S // TB
DP = 512
FC = 256
EPS = 1e-5


def _add(a, b):
    if a is None:
        return b
    if b is None:
        return a
    return a + b


def _sub(a, b):
    if b is None:
        return a
    if a is None:
        return -b
    return a - b


def _mulc(a, c):
    if a is None or c == 0.0:
        return None
    if c == 1.0:
        return a
    if c == -1.0:
        return -a
    return a * c


def _cmul_const(z, wr, wi):
    zr, zi = z
    if abs(wr) < 1e-12:
        wr = 0.0
    if abs(wi) < 1e-12:
        wi = 0.0
    if abs(abs(wr) - 1) < 1e-12:
        wr = math.copysign(1.0, wr)
    if abs(abs(wi) - 1) < 1e-12:
        wi = math.copysign(1.0, wi)
    re = _sub(_mulc(zr, wr), _mulc(zi, wi))
    im = _add(_mulc(zr, wi), _mulc(zi, wr))
    return (re, im)


def _rdft(x):
    n = len(x)
    if n == 1:
        return [(x[0], None)]
    if n == 2:
        return [(_add(x[0], x[1]), None), (_sub(x[0], x[1]), None)]
    e = _rdft(x[0::2])
    o = _rdft(x[1::2])
    out = [None] * (n // 2 + 1)
    for k in range(n // 4 + 1):
        t = _cmul_const(o[k], math.cos(2 * math.pi * k / n),
                        -math.sin(2 * math.pi * k / n))
        out[k] = (_add(e[k][0], t[0]), _add(e[k][1], t[1]))
        if n // 2 - k != k:
            out[n // 2 - k] = (_sub(e[k][0], t[0]), _sub(t[1], e[k][1]))
    return out


def _irdft(x, n, need):
    if n == 1:
        return [x[0][0]]
    if n == 2:
        out = [_add(x[0][0], x[1][0])]
        if need > 1:
            out.append(_sub(x[0][0], x[1][0]))
        return out
    e = [None] * (n // 4 + 1)
    o = [None] * (n // 4 + 1)
    for k in range(n // 4 + 1):
        a = x[k]
        b = x[n // 2 - k]
        e[k] = (_add(a[0], b[0]), _sub(a[1], b[1]))
        d = (_sub(a[0], b[0]), _add(a[1], b[1]))
        o[k] = _cmul_const(d, math.cos(2 * math.pi * k / n),
                           math.sin(2 * math.pi * k / n))
    ne = (need + 1) // 2
    no = need // 2
    xe = _irdft(e, n // 2, ne)
    xo = _irdft(o, n // 2, no) if no > 0 else []
    return [xe[i // 2] if i % 2 == 0 else xo[i // 2] for i in range(need)]


def _dft_tables():
    b = np.arange(NB)
    fwd = np.zeros((NF1, 2 * NB, 2 * NB), np.float64)
    inv = np.zeros((NF1, 2 * NB, 2 * NB), np.float64)
    for f1 in range(NF1):
        f = f1 + NA * b
        th = 2.0 * np.pi * ((b[:, None] * f[None, :]) % L) / L
        c, s = np.cos(th), np.sin(th)
        fwd[f1] = np.block([[c, -s], [s, c]])
        inv[f1] = np.block([[c.T, s.T], [-s.T, c.T]]) / L
    return fwd.astype(np.float32), inv.astype(np.float32)


def _kernel(q_hbm, k_hbm, v_hbm, sk_ref, hk_hbm, sd_ref, w1_hbm, w2_hbm,
            wf_hbm, wi_hbm, o_hbm,
            q_ref, k_ref, v_ref, hk_ref, w1_ref, w2_ref, o_ref,
            wf_ref, wi_ref, w1t_ref, par_ref, u_ref, g_ref, p_ref, y_ref,
            hb_ref, base_ref, xn_ref, sem, osem):
    f32 = jnp.float32
    bf16 = jnp.bfloat16
    NCH = F // FC
    NIT = 2 * NCH
    CPI = D // NIT
    RI = D // NCH

    def kvh_copies(i):
        rows = pl.ds(i * CPI, CPI)
        return [pltpu.make_async_copy(src.at[rows, :], dst.at[rows, :],
                                      sem.at[3 * i + j])
                for j, (src, dst) in enumerate(
                    ((k_hbm, k_ref), (v_hbm, v_ref), (hk_hbm, hk_ref)))]

    def q_copy(tb):
        cols = pl.ds(tb * TB, TB)
        return pltpu.make_async_copy(q_hbm.at[:, cols], q_ref.at[:, cols],
                                     sem.at[3 * NIT + tb])

    cp_w1 = pltpu.make_async_copy(w1_hbm, w1_ref, sem.at[3 * NIT + NTB])
    cp_w2 = pltpu.make_async_copy(w2_hbm, w2_ref, sem.at[3 * NIT + NTB + 1])
    cp_wf = pltpu.make_async_copy(wf_hbm, wf_ref, sem.at[3 * NIT + NTB + 2])
    cp_wi = pltpu.make_async_copy(wi_hbm, wi_ref, sem.at[3 * NIT + NTB + 3])
    PRE = 5
    WAITS = {0: range(5, 9), 4: range(9, NIT)}

    def start_kvh(rng):
        for i in rng:
            for cp in kvh_copies(i):
                cp.start()

    start_kvh(range(PRE - 1))

    def params():
        par = jnp.concatenate(
            [sk_ref[...].astype(f32), sd_ref[...].astype(f32),
             jnp.zeros((3, D), f32)], axis=0)
        par_ref[...] = par.T

    def kv_rows(r0, n):
        rows = pl.ds(r0, n)
        par = par_ref[rows, :]
        k = k_ref[rows, :].astype(f32)
        lane = jax.lax.broadcasted_iota(jnp.int32, (n, S), 1)
        ks = k * par[:, 0:1]
        for j in range(1, 4):
            kj = jnp.where(lane >= j, pltpu.roll(k, j, 1), 0.0)
            ks = ks + kj * par[:, j:j + 1]
        u_ref[rows, :] = ks * v_ref[rows, :].astype(f32)

    def s1_rows(src, r8, g8):
        xs = [src[pl.ds(r8, 8), pl.ds(NB * a, NB)].astype(f32)
              for a in range(NA // 2)]
        xs = xs + [None] * (NA // 2)
        g = _rdft(xs)
        for f1 in range(NF1):
            gr, gi = g[f1]
            if gi is None:
                gi = jnp.zeros((8, NB), f32)
            g_ref[f1, pl.ds(g8, 8), pl.ds(0, NB)] = gr
            g_ref[f1, pl.ds(g8, 8), pl.ds(NB, NB)] = gi
        return g[NF1 // 2][1]

    def spec_stage():
        for f1 in range(NF1):
            x = jnp.dot(g_ref[f1].astype(bf16), wf_ref[f1],
                        preferred_element_type=f32)
            xr, xi = x[:D, :NB], x[:D, NB:]
            hr, hi = x[D:, :NB], x[D:, NB:]
            yr = xr * hr - xi * hi
            yi = xr * hi + xi * hr
            yy = jnp.concatenate([yr, yi], axis=1).astype(bf16)
            p_ref[f1] = jnp.dot(yy, wi_ref[f1], preferred_element_type=f32)

    def i1_rows(r8):
        rows = pl.ds(r8, 8)
        xs = [(p_ref[f1, rows, pl.ds(0, NB)], p_ref[f1, rows, pl.ds(NB, NB)])
              for f1 in range(NF1)]
        y = _irdft(xs, NA, NA // 2)
        sd = par_ref[rows, :][:, 4:5]
        for a in range(NA // 2):
            col = pl.ds(NB * a, NB)
            yc = y[a].astype(bf16).astype(f32)
            tok = yc + u_ref[rows, col] * sd
            y_ref[rows, col] = tok
        return tok

    def layernorm(tb):
        cols = pl.ds(tb * TB, TB)
        x = q_ref[:, cols].astype(f32)
        mean = jnp.mean(x, axis=0, keepdims=True)
        xc = x - mean
        var = jnp.mean(xc * xc, axis=0, keepdims=True)
        xn = xc * jax.lax.rsqrt(var + EPS)
        xn_ref[pl.ds(0, D), cols] = xn.astype(bf16)
        base_ref[:, cols] = x

    def ffn_up(n):
        tb, i = divmod(n, NCH)
        h = jnp.dot(w1t_ref[pl.ds(i * FC, FC), :],
                    xn_ref[:, pl.ds(tb * TB, TB)],
                    preferred_element_type=f32)
        hh = 0.5 * h
        hb_ref[n % 2] = (hh + hh * jnp.tanh(hh)).astype(bf16)

    def ffn_down(n):
        tb, i = divmod(n, NCH)
        part = jnp.dot(w2_ref[:, pl.ds(i * FC, FC)], hb_ref[n % 2],
                       preferred_element_type=f32)
        cols = pl.ds(tb * TB, TB)
        base_ref[:, cols] = base_ref[:, cols] + part

    def combine(rows, cols):
        out = (base_ref[rows, cols]
               + xn_ref[rows, cols].astype(f32) * y_ref[rows, cols])
        o_ref[rows, cols] = out.astype(o_ref.dtype)
        return out[0:8, 0:NB]

    def order_before(tok, g, n):
        if n < NTB * NCH:
            tb = n // NCH
            xn_ref[pl.ds(D + 8 * g, 8), pl.ds(tb * TB, NB)] = tok.astype(bf16)

    def out_copy(rows, cols, s):
        return pltpu.make_async_copy(o_ref.at[rows, cols],
                                     o_hbm.at[rows, cols], osem.at[s])

    def fwd_slot(i, n):
        kv_rows(i * CPI, CPI)
        for g in range(CPI // 8):
            r8 = i * CPI + g * 8
            order_before(s1_rows(u_ref, r8, r8), 2 * g, n)
            order_before(s1_rows(hk_ref, r8, D + r8), 2 * g + 1, n)

    N_S1 = NIT - PRE
    N_I1 = N_S1 + NCH
    N_C01 = (NTB - 1) * NCH + 1
    first2 = pl.ds(0, 2 * TB)
    third = pl.ds(2 * TB, TB)

    def row_part(j, parts):
        units = D // 16
        lo = (units * j // parts) * 16
        hi = (units * (j + 1) // parts) * 16
        return pl.ds(lo, hi - lo)

    def extra(n):
        if n < N_S1:
            fwd_slot(n + PRE, n + 1)
        elif n < N_I1:
            i = n - N_S1
            for g in range(RI // 8):
                order_before(i1_rows(i * RI + g * 8), g, n + 1)
        elif n < N_C01:
            rows = row_part(n - N_I1, N_C01 - N_I1)
            order_before(combine(rows, first2), 0, n + 1)
            out_copy(rows, first2, 0).start()
        else:
            rows = row_part(n - N_C01, NTB * NCH - N_C01)
            order_before(combine(rows, third), 0, n + 1)
            out_copy(rows, third, 1).start()

    with jax.named_scope("pro"):
        params()
        xn_ref[pl.ds(D, DP - D), :] = jnp.zeros((DP - D, S), bf16)
        w1t_ref[:, pl.ds(D, DP - D)] = jnp.zeros((F, DP - D), bf16)
        for i in range(PRE):
            for cp in kvh_copies(i):
                cp.wait()
            if i == 0:
                start_kvh(range(PRE - 1, PRE))
                cp_w1.start()
                q_copy(0).start()
            if i == 3:
                cp_w2.start()
            fwd_slot(i, NTB * NCH)
        cp_w1.wait()
        start_kvh(WAITS[0])
        w1t_ref[:, pl.ds(0, D)] = w1_ref[...].astype(f32).T.astype(bf16)
        q_copy(0).wait()
        layernorm(0)
        ffn_up(0)
        cp_w2.wait()

    for n in range(NTB * NCH):
        for i in WAITS.get(n, ()):
            for cp in kvh_copies(i):
                cp.wait()
        if n == 0:
            start_kvh(WAITS[4])
            q_copy(1).start()
        if n == 4:
            cp_wf.start()
            cp_wi.start()
            q_copy(2).start()
            q_copy(3).start()
            q_copy(1).wait()
            layernorm(1)
        if n == N_S1:
            cp_wf.wait()
            cp_wi.wait()
            q_copy(2).wait()
            q_copy(3).wait()
            spec_stage()
            layernorm(2)
            layernorm(3)
        extra(n)
        if n + 1 < NTB * NCH:
            ffn_up(n + 1)
        ffn_down(n)

    with jax.named_scope("fin"):
        late = pl.ds((NTB - 1) * TB, TB)
        combine(pl.ds(0, D), late)
        cp_late = out_copy(pl.ds(0, D), late, 2)
        cp_late.start()
        out_copy(pl.ds(0, D), first2, 0).wait()
        out_copy(pl.ds(0, D), third, 1).wait()
        cp_late.wait()


@jax.jit
def pallas_parallel_sum__ssm_conv_h3__dense_activation_silu__prompt_kernel(
    A_q: jax.Array,
    A_k: jax.Array,
    A_v: jax.Array,
    A_shift_k: jax.Array,
    A_ssm_k: jax.Array,
    A_ssm_D: jax.Array,
    B_x: jax.Array,
    B_w1: jax.Array,
    B_w2: jax.Array,
):
    del B_x
    qt = A_q.reshape(S, D).T
    kt = A_k.reshape(S, D).T
    vt = A_v.reshape(S, D).T
    sk = A_shift_k.T
    sd = A_ssm_D.reshape(1, D)
    w2t = B_w2.T
    wf_np, wi_np = _dft_tables()
    wf = jnp.asarray(wf_np, dtype=jnp.bfloat16)
    wi = jnp.asarray(wi_np, dtype=jnp.bfloat16)

    hbm = pl.BlockSpec(memory_space=pl.ANY)
    vmem = pl.BlockSpec(memory_space=pltpu.VMEM)
    in_specs = [hbm, hbm, hbm, vmem, hbm, vmem, hbm, hbm, hbm, hbm]
    bf = jnp.bfloat16
    scratch = [
        pltpu.VMEM((D, S), bf),
        pltpu.VMEM((D, S), bf),
        pltpu.VMEM((D, S), bf),
        pltpu.VMEM((D, S), bf),
        pltpu.VMEM((D, F), bf),
        pltpu.VMEM((D, F), bf),
        pltpu.VMEM((D, S), bf),
        pltpu.VMEM((NF1, 2 * NB, 2 * NB), bf),
        pltpu.VMEM((NF1, 2 * NB, 2 * NB), bf),
        pltpu.VMEM((F, DP), bf),
        pltpu.VMEM((D, 8), jnp.float32),
        pltpu.VMEM((D, S), jnp.float32),
        pltpu.VMEM((NF1, 2 * D, 2 * NB), jnp.float32),
        pltpu.VMEM((NF1, D, 2 * NB), jnp.float32),
        pltpu.VMEM((D, S), jnp.float32),
        pltpu.VMEM((2, FC, TB), bf),
        pltpu.VMEM((D, S), jnp.float32),
        pltpu.VMEM((DP, S), bf),
        pltpu.SemaphoreType.DMA((3 * 2 * (F // FC) + NTB + 4,)),
        pltpu.SemaphoreType.DMA((3,)),
    ]
    out = pl.pallas_call(
        _kernel,
        in_specs=in_specs,
        out_specs=hbm,
        out_shape=jax.ShapeDtypeStruct((D, S), bf),
        scratch_shapes=scratch,
        compiler_params=pltpu.CompilerParams(
            vmem_limit_bytes=100 * 1024 * 1024,
        ),
    )(qt, kt, vt, sk, A_ssm_k, sd, B_w1, w2t, wf, wi)
    return out.T.reshape(1, S, D)
```

```python
import math

import numpy as np
import jax
import jax.numpy as jnp
import jax.experimental.pallas as pl
import jax.experimental.pallas.tpu as pltpu

S = 2048
D = 448
F = 1792
L = 2 * S
NB = 128
NA = L // NB
NF1 = NA // 2 + 1
CR = 224
NCB = D // CR
TB = 512
NTB = S // TB
DP = 512
FC = 256
EPS = 1e-5


def _add(a, b):
    if a is None:
        return b
    if b is None:
        return a
    return a + b


def _sub(a, b):
    if b is None:
        return a
    if a is None:
        return -b
    return a - b


def _mulc(a, c):
    if a is None or c == 0.0:
        return None
    if c == 1.0:
        return a
    if c == -1.0:
        return -a
    return a * c


def _cmul_const(z, wr, wi):
    zr, zi = z
    if abs(wr) < 1e-12:
        wr = 0.0
    if abs(wi) < 1e-12:
        wi = 0.0
    if abs(abs(wr) - 1) < 1e-12:
        wr = math.copysign(1.0, wr)
    if abs(abs(wi) - 1) < 1e-12:
        wi = math.copysign(1.0, wi)
    re = _sub(_mulc(zr, wr), _mulc(zi, wi))
    im = _add(_mulc(zr, wi), _mulc(zi, wr))
    return (re, im)


def _rdft(x):
    n = len(x)
    if n == 1:
        return [(x[0], None)]
    if n == 2:
        return [(_add(x[0], x[1]), None), (_sub(x[0], x[1]), None)]
    e = _rdft(x[0::2])
    o = _rdft(x[1::2])
    out = [None] * (n // 2 + 1)
    for k in range(n // 4 + 1):
        t = _cmul_const(o[k], math.cos(2 * math.pi * k / n),
                        -math.sin(2 * math.pi * k / n))
        out[k] = (_add(e[k][0], t[0]), _add(e[k][1], t[1]))
        if n // 2 - k != k:
            out[n // 2 - k] = (_sub(e[k][0], t[0]), _sub(t[1], e[k][1]))
    return out


def _irdft(x, n, need):
    if n == 1:
        return [x[0][0]]
    if n == 2:
        out = [_add(x[0][0], x[1][0])]
        if need > 1:
            out.append(_sub(x[0][0], x[1][0]))
        return out
    e = [None] * (n // 4 + 1)
    o = [None] * (n // 4 + 1)
    for k in range(n // 4 + 1):
        a = x[k]
        b = x[n // 2 - k]
        e[k] = (_add(a[0], b[0]), _sub(a[1], b[1]))
        d = (_sub(a[0], b[0]), _add(a[1], b[1]))
        o[k] = _cmul_const(d, math.cos(2 * math.pi * k / n),
                           math.sin(2 * math.pi * k / n))
    ne = (need + 1) // 2
    no = need // 2
    xe = _irdft(e, n // 2, ne)
    xo = _irdft(o, n // 2, no) if no > 0 else []
    return [xe[i // 2] if i % 2 == 0 else xo[i // 2] for i in range(need)]


def _dft_tables():
    b = np.arange(NB)
    fwd = np.zeros((NF1, 2 * NB, 2 * NB), np.float64)
    inv = np.zeros((NF1, 2 * NB, 2 * NB), np.float64)
    for f1 in range(NF1):
        f = f1 + NA * b
        th = 2.0 * np.pi * ((b[:, None] * f[None, :]) % L) / L
        c, s = np.cos(th), np.sin(th)
        fwd[f1] = np.block([[c, -s], [s, c]])
        inv[f1] = np.block([[c.T, s.T], [-s.T, c.T]]) / L
    return fwd.astype(np.float32), inv.astype(np.float32)


def _kernel(q_hbm, k_hbm, v_hbm, sk_ref, hk_hbm, sd_ref, w1_hbm, w2_hbm,
            wf_hbm, wi_hbm, o_hbm,
            q_ref, k_ref, v_ref, hk_ref, w1_ref, w2_ref, o_ref,
            wf_ref, wi_ref, w1t_ref, par_ref, u_ref, g_ref, p_ref, y_ref,
            hb_ref, base_ref, xn_ref, sem, osem):
    f32 = jnp.float32
    bf16 = jnp.bfloat16
    NCH = F // FC
    NIT = 2 * NCH
    CPI = D // NIT
    RI = D // NCH

    def kvh_copies(i):
        rows = pl.ds(i * CPI, CPI)
        return [pltpu.make_async_copy(src.at[rows, :], dst.at[rows, :],
                                      sem.at[3 * i + j])
                for j, (src, dst) in enumerate(
                    ((k_hbm, k_ref), (v_hbm, v_ref), (hk_hbm, hk_ref)))]

    def q_copy(tb):
        cols = pl.ds(tb * TB, TB)
        return pltpu.make_async_copy(q_hbm.at[:, cols], q_ref.at[:, cols],
                                     sem.at[3 * NIT + tb])

    cp_w1 = pltpu.make_async_copy(w1_hbm, w1_ref, sem.at[3 * NIT + NTB])
    cp_w2 = pltpu.make_async_copy(w2_hbm, w2_ref, sem.at[3 * NIT + NTB + 1])
    cp_wf = pltpu.make_async_copy(wf_hbm, wf_ref, sem.at[3 * NIT + NTB + 2])
    cp_wi = pltpu.make_async_copy(wi_hbm, wi_ref, sem.at[3 * NIT + NTB + 3])
    PRE = 5
    LA = 3
    WAITS = {0: range(5, 9), 4: range(9, NIT)}

    def start_kvh(rng):
        for i in rng:
            for cp in kvh_copies(i):
                cp.start()

    start_kvh(range(PRE - 1))

    def params():
        par = jnp.concatenate(
            [sk_ref[...].astype(f32), sd_ref[...].astype(f32),
             jnp.zeros((3, D), f32)], axis=0)
        par_ref[...] = par.T

    def kv_rows(r0, n):
        rows = pl.ds(r0, n)
        par = par_ref[rows, :]
        k = k_ref[rows, :].astype(f32)
        lane = jax.lax.broadcasted_iota(jnp.int32, (n, S), 1)
        ks = k * par[:, 0:1]
        for j in range(1, 4):
            kj = jnp.where(lane >= j, pltpu.roll(k, j, 1), 0.0)
            ks = ks + kj * par[:, j:j + 1]
        u_ref[rows, :] = ks * v_ref[rows, :].astype(f32)

    def s1_rows(src, r8, g8):
        xs = [src[pl.ds(r8, 8), pl.ds(NB * a, NB)].astype(f32)
              for a in range(NA // 2)]
        xs = xs + [None] * (NA // 2)
        g = _rdft(xs)
        for f1 in range(NF1):
            gr, gi = g[f1]
            if gi is None:
                gi = jnp.zeros((8, NB), f32)
            g_ref[f1, pl.ds(g8, 8), pl.ds(0, NB)] = gr
            g_ref[f1, pl.ds(g8, 8), pl.ds(NB, NB)] = gi
        return g[NF1 // 2][1]

    def spec_stage():
        for f1 in range(NF1):
            x = jnp.dot(g_ref[f1].astype(bf16), wf_ref[f1],
                        preferred_element_type=f32)
            xr, xi = x[:D, :NB], x[:D, NB:]
            hr, hi = x[D:, :NB], x[D:, NB:]
            yr = xr * hr - xi * hi
            yi = xr * hi + xi * hr
            yy = jnp.concatenate([yr, yi], axis=1).astype(bf16)
            p_ref[f1] = jnp.dot(yy, wi_ref[f1], preferred_element_type=f32)

    def i1_rows(r8):
        rows = pl.ds(r8, 8)
        xs = [(p_ref[f1, rows, pl.ds(0, NB)], p_ref[f1, rows, pl.ds(NB, NB)])
              for f1 in range(NF1)]
        y = _irdft(xs, NA, NA // 2)
        sd = par_ref[rows, :][:, 4:5]
        for a in range(NA // 2):
            col = pl.ds(NB * a, NB)
            yc = y[a].astype(bf16).astype(f32)
            tok = yc + u_ref[rows, col] * sd
            y_ref[rows, col] = tok
        return tok

    def layernorm(tb):
        cols = pl.ds(tb * TB, TB)
        x = q_ref[:, cols].astype(f32)
        mean = jnp.mean(x, axis=0, keepdims=True)
        xc = x - mean
        var = jnp.mean(xc * xc, axis=0, keepdims=True)
        xn = xc * jax.lax.rsqrt(var + EPS)
        xn_ref[pl.ds(0, D), cols] = xn.astype(bf16)
        base_ref[:, cols] = x

    def ffn_up(n):
        tb, i = divmod(n, NCH)
        h = jnp.dot(w1t_ref[pl.ds(i * FC, FC), :],
                    xn_ref[:, pl.ds(tb * TB, TB)],
                    preferred_element_type=f32)
        hh = 0.5 * h
        hb_ref[n % 2] = (hh + hh * jnp.tanh(hh)).astype(bf16)

    def ffn_down(n):
        tb, i = divmod(n, NCH)
        part = jnp.dot(w2_ref[:, pl.ds(i * FC, FC)], hb_ref[n % 2],
                       preferred_element_type=f32)
        cols = pl.ds(tb * TB, TB)
        base_ref[:, cols] = base_ref[:, cols] + part

    def combine(rows, cols):
        out = (base_ref[rows, cols]
               + xn_ref[rows, cols].astype(f32) * y_ref[rows, cols])
        o_ref[rows, cols] = out.astype(o_ref.dtype)
        return out[0:8, 0:NB]

    def order_before(tok, g, n):
        if n < NTB * NCH:
            i = n % NCH
            w1t_ref[pl.ds(i * FC + 8 * g, 8), pl.ds(D, DP - D)] = (
                tok[:, :DP - D].astype(bf16))

    def out_copy(rows, cols, s):
        return pltpu.make_async_copy(o_ref.at[rows, cols],
                                     o_hbm.at[rows, cols], osem.at[s])

    def fwd_slot(i, n):
        kv_rows(i * CPI, CPI)
        for g in range(CPI // 8):
            r8 = i * CPI + g * 8
            order_before(s1_rows(u_ref, r8, r8), 2 * g, n)
            order_before(s1_rows(hk_ref, r8, D + r8), 2 * g + 1, n)

    N_S1 = NIT - PRE
    N_I1 = N_S1 + NCH
    N_C01 = (NTB - 1) * NCH + 1
    first2 = pl.ds(0, 2 * TB)
    third = pl.ds(2 * TB, TB)

    def row_part(j, parts):
        units = D // 16
        lo = (units * j // parts) * 16
        hi = (units * (j + 1) // parts) * 16
        return pl.ds(lo, hi - lo)

    def extra(n):
        if n < N_S1:
            fwd_slot(n + PRE, n + LA)
        elif n < N_I1:
            i = n - N_S1
            for g in range(RI // 8):
                order_before(i1_rows(i * RI + g * 8), g, n + LA)
        elif n < N_C01:
            rows = row_part(n - N_I1, N_C01 - N_I1)
            order_before(combine(rows, first2), 0, n + LA)
            out_copy(rows, first2, 0).start()
        else:
            rows = row_part(n - N_C01, NTB * NCH - N_C01)
            order_before(combine(rows, third), 0, n + LA)
            out_copy(rows, third, 1).start()

    with jax.named_scope("pro"):
        params()
        xn_ref[pl.ds(D, DP - D), :] = jnp.zeros((DP - D, S), bf16)
        w1t_ref[:, pl.ds(D, DP - D)] = jnp.zeros((F, DP - D), bf16)
        for i in range(PRE):
            for cp in kvh_copies(i):
                cp.wait()
            if i == 0:
                start_kvh(range(PRE - 1, PRE))
                cp_w1.start()
                q_copy(0).start()
            if i == 3:
                cp_w2.start()
            fwd_slot(i, NTB * NCH)
        cp_w1.wait()
        start_kvh(WAITS[0])
        w1t_ref[:, pl.ds(0, D)] = w1_ref[...].astype(f32).T.astype(bf16)
        q_copy(0).wait()
        layernorm(0)
        ffn_up(0)
        cp_w2.wait()

    for n in range(NTB * NCH):
        for i in WAITS.get(n, ()):
            for cp in kvh_copies(i):
                cp.wait()
        if n == 0:
            start_kvh(WAITS[4])
            q_copy(1).start()
        if n == 4:
            cp_wf.start()
            cp_wi.start()
            q_copy(2).start()
            q_copy(3).start()
            q_copy(1).wait()
            layernorm(1)
        if n == N_S1:
            cp_wf.wait()
            cp_wi.wait()
            q_copy(2).wait()
            q_copy(3).wait()
            spec_stage()
            layernorm(2)
            layernorm(3)
        extra(n)
        if n + 1 < NTB * NCH:
            ffn_up(n + 1)
        ffn_down(n)

    with jax.named_scope("fin"):
        late = pl.ds((NTB - 1) * TB, TB)
        combine(pl.ds(0, D), late)
        cp_late = out_copy(pl.ds(0, D), late, 2)
        cp_late.start()
        out_copy(pl.ds(0, D), first2, 0).wait()
        out_copy(pl.ds(0, D), third, 1).wait()
        cp_late.wait()


@jax.jit
def pallas_parallel_sum__ssm_conv_h3__dense_activation_silu__prompt_kernel(
    A_q: jax.Array,
    A_k: jax.Array,
    A_v: jax.Array,
    A_shift_k: jax.Array,
    A_ssm_k: jax.Array,
    A_ssm_D: jax.Array,
    B_x: jax.Array,
    B_w1: jax.Array,
    B_w2: jax.Array,
):
    del B_x
    qt = A_q.reshape(S, D).T
    kt = A_k.reshape(S, D).T
    vt = A_v.reshape(S, D).T
    sk = A_shift_k.T
    sd = A_ssm_D.reshape(1, D)
    w2t = B_w2.T
    wf_np, wi_np = _dft_tables()
    wf = jnp.asarray(wf_np, dtype=jnp.bfloat16)
    wi = jnp.asarray(wi_np, dtype=jnp.bfloat16)

    hbm = pl.BlockSpec(memory_space=pl.ANY)
    vmem = pl.BlockSpec(memory_space=pltpu.VMEM)
    in_specs = [hbm, hbm, hbm, vmem, hbm, vmem, hbm, hbm, hbm, hbm]
    bf = jnp.bfloat16
    scratch = [
        pltpu.VMEM((D, S), bf),
        pltpu.VMEM((D, S), bf),
        pltpu.VMEM((D, S), bf),
        pltpu.VMEM((D, S), bf),
        pltpu.VMEM((D, F), bf),
        pltpu.VMEM((D, F), bf),
        pltpu.VMEM((D, S), bf),
        pltpu.VMEM((NF1, 2 * NB, 2 * NB), bf),
        pltpu.VMEM((NF1, 2 * NB, 2 * NB), bf),
        pltpu.VMEM((F, DP), bf),
        pltpu.VMEM((D, 8), jnp.float32),
        pltpu.VMEM((D, S), jnp.float32),
        pltpu.VMEM((NF1, 2 * D, 2 * NB), jnp.float32),
        pltpu.VMEM((NF1, D, 2 * NB), jnp.float32),
        pltpu.VMEM((D, S), jnp.float32),
        pltpu.VMEM((2, FC, TB), bf),
        pltpu.VMEM((D, S), jnp.float32),
        pltpu.VMEM((DP, S), bf),
        pltpu.SemaphoreType.DMA((3 * 2 * (F // FC) + NTB + 4,)),
        pltpu.SemaphoreType.DMA((3,)),
    ]
    out = pl.pallas_call(
        _kernel,
        in_specs=in_specs,
        out_specs=hbm,
        out_shape=jax.ShapeDtypeStruct((D, S), bf),
        scratch_shapes=scratch,
        compiler_params=pltpu.CompilerParams(
            vmem_limit_bytes=100 * 1024 * 1024,
        ),
    )(qt, kt, vt, sk, A_ssm_k, sd, B_w1, w2t, wf, wi)
    return out.T.reshape(1, S, D)
```

```python
import math

import numpy as np
import jax
import jax.numpy as jnp
import jax.experimental.pallas as pl
import jax.experimental.pallas.tpu as pltpu

S = 2048
D = 448
F = 1792
L = 2 * S
NB = 128
NA = L // NB
NF1 = NA // 2 + 1
CR = 224
NCB = D // CR
TB = 512
NTB = S // TB
DP = 512
FC = 256
EPS = 1e-5


def _add(a, b):
    if a is None:
        return b
    if b is None:
        return a
    return a + b


def _sub(a, b):
    if b is None:
        return a
    if a is None:
        return -b
    return a - b


def _mulc(a, c):
    if a is None or c == 0.0:
        return None
    if c == 1.0:
        return a
    if c == -1.0:
        return -a
    return a * c


def _cmul_const(z, wr, wi):
    zr, zi = z
    if abs(wr) < 1e-12:
        wr = 0.0
    if abs(wi) < 1e-12:
        wi = 0.0
    if abs(abs(wr) - 1) < 1e-12:
        wr = math.copysign(1.0, wr)
    if abs(abs(wi) - 1) < 1e-12:
        wi = math.copysign(1.0, wi)
    re = _sub(_mulc(zr, wr), _mulc(zi, wi))
    im = _add(_mulc(zr, wi), _mulc(zi, wr))
    return (re, im)


def _rdft(x):
    n = len(x)
    if n == 1:
        return [(x[0], None)]
    if n == 2:
        return [(_add(x[0], x[1]), None), (_sub(x[0], x[1]), None)]
    e = _rdft(x[0::2])
    o = _rdft(x[1::2])
    out = [None] * (n // 2 + 1)
    for k in range(n // 4 + 1):
        t = _cmul_const(o[k], math.cos(2 * math.pi * k / n),
                        -math.sin(2 * math.pi * k / n))
        out[k] = (_add(e[k][0], t[0]), _add(e[k][1], t[1]))
        if n // 2 - k != k:
            out[n // 2 - k] = (_sub(e[k][0], t[0]), _sub(t[1], e[k][1]))
    return out


def _irdft(x, n, need):
    if n == 1:
        return [x[0][0]]
    if n == 2:
        out = [_add(x[0][0], x[1][0])]
        if need > 1:
            out.append(_sub(x[0][0], x[1][0]))
        return out
    e = [None] * (n // 4 + 1)
    o = [None] * (n // 4 + 1)
    for k in range(n // 4 + 1):
        a = x[k]
        b = x[n // 2 - k]
        e[k] = (_add(a[0], b[0]), _sub(a[1], b[1]))
        d = (_sub(a[0], b[0]), _add(a[1], b[1]))
        o[k] = _cmul_const(d, math.cos(2 * math.pi * k / n),
                           math.sin(2 * math.pi * k / n))
    ne = (need + 1) // 2
    no = need // 2
    xe = _irdft(e, n // 2, ne)
    xo = _irdft(o, n // 2, no) if no > 0 else []
    return [xe[i // 2] if i % 2 == 0 else xo[i // 2] for i in range(need)]


def _dft_tables():
    b = np.arange(NB)
    fwd = np.zeros((NF1, 2 * NB, 2 * NB), np.float64)
    inv = np.zeros((NF1, 2 * NB, 2 * NB), np.float64)
    for f1 in range(NF1):
        f = f1 + NA * b
        th = 2.0 * np.pi * ((b[:, None] * f[None, :]) % L) / L
        c, s = np.cos(th), np.sin(th)
        fwd[f1] = np.block([[c, -s], [s, c]])
        inv[f1] = np.block([[c.T, s.T], [-s.T, c.T]]) / L
    return fwd.astype(np.float32), inv.astype(np.float32)


def _kernel(q_hbm, k_hbm, v_hbm, sk_ref, hk_hbm, sd_ref, w1_hbm, w2_hbm,
            wf_hbm, wi_hbm, o_hbm,
            q_ref, k_ref, v_ref, hk_ref, w1_ref, w2_ref, o_ref,
            wf_ref, wi_ref, w1t_ref, par_ref, u_ref, g_ref, p_ref, y_ref,
            hb_ref, base_ref, xn_ref, sem, osem):
    f32 = jnp.float32
    bf16 = jnp.bfloat16
    NCH = F // FC
    NIT = 2 * NCH
    CPI = D // NIT
    RI = D // NCH

    def kvh_copies(i):
        rows = pl.ds(i * CPI, CPI)
        return [pltpu.make_async_copy(src.at[rows, :], dst.at[rows, :],
                                      sem.at[3 * i + j])
                for j, (src, dst) in enumerate(
                    ((k_hbm, k_ref), (v_hbm, v_ref), (hk_hbm, hk_ref)))]

    def q_copy(tb):
        cols = pl.ds(tb * TB, TB)
        return pltpu.make_async_copy(q_hbm.at[:, cols], q_ref.at[:, cols],
                                     sem.at[3 * NIT + tb])

    cp_w1 = pltpu.make_async_copy(w1_hbm, w1_ref, sem.at[3 * NIT + NTB])
    cp_w2 = pltpu.make_async_copy(w2_hbm, w2_ref, sem.at[3 * NIT + NTB + 1])
    cp_wf = pltpu.make_async_copy(wf_hbm, wf_ref, sem.at[3 * NIT + NTB + 2])
    cp_wi = pltpu.make_async_copy(wi_hbm, wi_ref, sem.at[3 * NIT + NTB + 3])
    PRE = 5
    LA = 3
    WAITS = {0: range(5, 7), 2: range(7, 10), 5: range(10, NIT)}

    def start_kvh(rng):
        for i in rng:
            for cp in kvh_copies(i):
                cp.start()

    start_kvh(range(PRE - 1))

    def params():
        par = jnp.concatenate(
            [sk_ref[...].astype(f32), sd_ref[...].astype(f32),
             jnp.zeros((3, D), f32)], axis=0)
        par_ref[...] = par.T

    def kv_rows(r0, n):
        rows = pl.ds(r0, n)
        par = par_ref[rows, :]
        k = k_ref[rows, :].astype(f32)
        lane = jax.lax.broadcasted_iota(jnp.int32, (n, S), 1)
        ks = k * par[:, 0:1]
        for j in range(1, 4):
            kj = jnp.where(lane >= j, pltpu.roll(k, j, 1), 0.0)
            ks = ks + kj * par[:, j:j + 1]
        u_ref[rows, :] = ks * v_ref[rows, :].astype(f32)

    def s1_rows(src, r8, g8):
        xs = [src[pl.ds(r8, 8), pl.ds(NB * a, NB)].astype(f32)
              for a in range(NA // 2)]
        xs = xs + [None] * (NA // 2)
        g = _rdft(xs)
        for f1 in range(NF1):
            gr, gi = g[f1]
            if gi is None:
                gi = jnp.zeros((8, NB), f32)
            g_ref[f1, pl.ds(g8, 8), pl.ds(0, NB)] = gr
            g_ref[f1, pl.ds(g8, 8), pl.ds(NB, NB)] = gi
        return g[NF1 // 2][1]

    def spec_stage():
        for f1 in range(NF1):
            x = jnp.dot(g_ref[f1].astype(bf16), wf_ref[f1],
                        preferred_element_type=f32)
            xr, xi = x[:D, :NB], x[:D, NB:]
            hr, hi = x[D:, :NB], x[D:, NB:]
            yr = xr * hr - xi * hi
            yi = xr * hi + xi * hr
            yy = jnp.concatenate([yr, yi], axis=1).astype(bf16)
            p_ref[f1] = jnp.dot(yy, wi_ref[f1], preferred_element_type=f32)

    def i1_rows(r8):
        rows = pl.ds(r8, 8)
        xs = [(p_ref[f1, rows, pl.ds(0, NB)], p_ref[f1, rows, pl.ds(NB, NB)])
              for f1 in range(NF1)]
        y = _irdft(xs, NA, NA // 2)
        sd = par_ref[rows, :][:, 4:5]
        for a in range(NA // 2):
            col = pl.ds(NB * a, NB)
            yc = y[a].astype(bf16).astype(f32)
            tok = yc + u_ref[rows, col] * sd
            y_ref[rows, col] = tok
        return tok

    def layernorm(tb):
        cols = pl.ds(tb * TB, TB)
        x = q_ref[:, cols].astype(f32)
        mean = jnp.mean(x, axis=0, keepdims=True)
        xc = x - mean
        var = jnp.mean(xc * xc, axis=0, keepdims=True)
        xn = xc * jax.lax.rsqrt(var + EPS)
        xn_ref[pl.ds(0, D), cols] = xn.astype(bf16)
        base_ref[:, cols] = x

    def ffn_up(n):
        tb, i = divmod(n, NCH)
        h = jnp.dot(w1t_ref[pl.ds(i * FC, FC), :],
                    xn_ref[:, pl.ds(tb * TB, TB)],
                    preferred_element_type=f32)
        hh = 0.5 * h
        hb_ref[n % 2] = (hh + hh * jnp.tanh(hh)).astype(bf16)

    def ffn_down(n):
        tb, i = divmod(n, NCH)
        part = jnp.dot(w2_ref[:, pl.ds(i * FC, FC)], hb_ref[n % 2],
                       preferred_element_type=f32)
        cols = pl.ds(tb * TB, TB)
        base_ref[:, cols] = base_ref[:, cols] + part

    def combine(rows, cols):
        out = (base_ref[rows, cols]
               + xn_ref[rows, cols].astype(f32) * y_ref[rows, cols])
        o_ref[rows, cols] = out.astype(o_ref.dtype)
        return out[0:8, 0:NB]

    def order_before(tok, g, n):
        if n < NTB * NCH:
            i = n % NCH
            w1t_ref[pl.ds(i * FC + 8 * g, 8), pl.ds(D, DP - D)] = (
                tok[:, :DP - D].astype(bf16))

    def out_copy(rows, cols, s):
        return pltpu.make_async_copy(o_ref.at[rows, cols],
                                     o_hbm.at[rows, cols], osem.at[s])

    def fwd_slot(i, n):
        kv_rows(i * CPI, CPI)
        for g in range(CPI // 8):
            r8 = i * CPI + g * 8
            order_before(s1_rows(u_ref, r8, r8), 2 * g, n)
            order_before(s1_rows(hk_ref, r8, D + r8), 2 * g + 1, n)

    N_S1 = NIT - PRE
    N_I1 = N_S1 + NCH
    N_C01 = (NTB - 1) * NCH + 1
    first2 = pl.ds(0, 2 * TB)
    third = pl.ds(2 * TB, TB)

    def row_part(j, parts):
        units = D // 16
        lo = (units * j // parts) * 16
        hi = (units * (j + 1) // parts) * 16
        return pl.ds(lo, hi - lo)

    def extra(n):
        if n < N_S1:
            fwd_slot(n + PRE, n + LA)
        elif n < N_I1:
            i = n - N_S1
            for g in range(RI // 8):
                order_before(i1_rows(i * RI + g * 8), g, n + LA)
        elif n < N_C01:
            rows = row_part(n - N_I1, N_C01 - N_I1)
            order_before(combine(rows, first2), 0, n + LA)
            out_copy(rows, first2, 0).start()
        else:
            rows = row_part(n - N_C01, NTB * NCH - N_C01)
            order_before(combine(rows, third), 0, n + LA)
            out_copy(rows, third, 1).start()

    with jax.named_scope("pro"):
        params()
        xn_ref[pl.ds(D, DP - D), :] = jnp.zeros((DP - D, S), bf16)
        w1t_ref[:, pl.ds(D, DP - D)] = jnp.zeros((F, DP - D), bf16)
        for i in range(PRE):
            for cp in kvh_copies(i):
                cp.wait()
            if i == 0:
                start_kvh(range(PRE - 1, PRE))
                cp_w1.start()
                q_copy(0).start()
            if i == 2:
                cp_w2.start()
            if i == 4:
                start_kvh(WAITS[0])
            fwd_slot(i, NTB * NCH)
        cp_w1.wait()
        start_kvh(WAITS[2])
        w1t_ref[:, pl.ds(0, D)] = w1_ref[...].astype(f32).T.astype(bf16)
        q_copy(0).wait()
        layernorm(0)
        ffn_up(0)
        cp_w2.wait()

    for n in range(NTB * NCH):
        for i in WAITS.get(n, ()):
            for cp in kvh_copies(i):
                cp.wait()
        if n == 0:
            start_kvh(WAITS[5])
            q_copy(1).start()
        if n == 5:
            cp_wf.start()
            cp_wi.start()
            q_copy(2).start()
            q_copy(3).start()
            q_copy(1).wait()
            layernorm(1)
        if n == N_S1:
            cp_wf.wait()
            cp_wi.wait()
            q_copy(2).wait()
            q_copy(3).wait()
            spec_stage()
            layernorm(2)
            layernorm(3)
        extra(n)
        if n + 1 < NTB * NCH:
            ffn_up(n + 1)
        ffn_down(n)

    with jax.named_scope("fin"):
        late = pl.ds((NTB - 1) * TB, TB)
        combine(pl.ds(0, D), late)
        cp_late = out_copy(pl.ds(0, D), late, 2)
        cp_late.start()
        out_copy(pl.ds(0, D), first2, 0).wait()
        out_copy(pl.ds(0, D), third, 1).wait()
        cp_late.wait()


@jax.jit
def pallas_parallel_sum__ssm_conv_h3__dense_activation_silu__prompt_kernel(
    A_q: jax.Array,
    A_k: jax.Array,
    A_v: jax.Array,
    A_shift_k: jax.Array,
    A_ssm_k: jax.Array,
    A_ssm_D: jax.Array,
    B_x: jax.Array,
    B_w1: jax.Array,
    B_w2: jax.Array,
):
    del B_x
    qt = A_q.reshape(S, D).T
    kt = A_k.reshape(S, D).T
    vt = A_v.reshape(S, D).T
    sk = A_shift_k.T
    sd = A_ssm_D.reshape(1, D)
    w2t = B_w2.T
    wf_np, wi_np = _dft_tables()
    wf = jnp.asarray(wf_np, dtype=jnp.bfloat16)
    wi = jnp.asarray(wi_np, dtype=jnp.bfloat16)

    hbm = pl.BlockSpec(memory_space=pl.ANY)
    vmem = pl.BlockSpec(memory_space=pltpu.VMEM)
    in_specs = [hbm, hbm, hbm, vmem, hbm, vmem, hbm, hbm, hbm, hbm]
    bf = jnp.bfloat16
    scratch = [
        pltpu.VMEM((D, S), bf),
        pltpu.VMEM((D, S), bf),
        pltpu.VMEM((D, S), bf),
        pltpu.VMEM((D, S), bf),
        pltpu.VMEM((D, F), bf),
        pltpu.VMEM((D, F), bf),
        pltpu.VMEM((D, S), bf),
        pltpu.VMEM((NF1, 2 * NB, 2 * NB), bf),
        pltpu.VMEM((NF1, 2 * NB, 2 * NB), bf),
        pltpu.VMEM((F, DP), bf),
        pltpu.VMEM((D, 8), jnp.float32),
        pltpu.VMEM((D, S), jnp.float32),
        pltpu.VMEM((NF1, 2 * D, 2 * NB), jnp.float32),
        pltpu.VMEM((NF1, D, 2 * NB), jnp.float32),
        pltpu.VMEM((D, S), jnp.float32),
        pltpu.VMEM((2, FC, TB), bf),
        pltpu.VMEM((D, S), jnp.float32),
        pltpu.VMEM((DP, S), bf),
        pltpu.SemaphoreType.DMA((3 * 2 * (F // FC) + NTB + 4,)),
        pltpu.SemaphoreType.DMA((3,)),
    ]
    out = pl.pallas_call(
        _kernel,
        in_specs=in_specs,
        out_specs=hbm,
        out_shape=jax.ShapeDtypeStruct((D, S), bf),
        scratch_shapes=scratch,
        compiler_params=pltpu.CompilerParams(
            vmem_limit_bytes=100 * 1024 * 1024,
        ),
    )(qt, kt, vt, sk, A_ssm_k, sd, B_w1, w2t, wf, wi)
    return out.T.reshape(1, S, D)
```

```python
import math

import numpy as np
import jax
import jax.numpy as jnp
import jax.experimental.pallas as pl
import jax.experimental.pallas.tpu as pltpu

S = 2048
D = 448
F = 1792
L = 2 * S
NB = 128
NA = L // NB
NF1 = NA // 2 + 1
CR = 224
NCB = D // CR
TB = 512
NTB = S // TB
DP = 512
FC = 256
EPS = 1e-5


def _add(a, b):
    if a is None:
        return b
    if b is None:
        return a
    return a + b


def _sub(a, b):
    if b is None:
        return a
    if a is None:
        return -b
    return a - b


def _mulc(a, c):
    if a is None or c == 0.0:
        return None
    if c == 1.0:
        return a
    if c == -1.0:
        return -a
    return a * c


def _cmul_const(z, wr, wi):
    zr, zi = z
    if abs(wr) < 1e-12:
        wr = 0.0
    if abs(wi) < 1e-12:
        wi = 0.0
    if abs(abs(wr) - 1) < 1e-12:
        wr = math.copysign(1.0, wr)
    if abs(abs(wi) - 1) < 1e-12:
        wi = math.copysign(1.0, wi)
    re = _sub(_mulc(zr, wr), _mulc(zi, wi))
    im = _add(_mulc(zr, wi), _mulc(zi, wr))
    return (re, im)


def _rdft(x):
    n = len(x)
    if n == 1:
        return [(x[0], None)]
    if n == 2:
        return [(_add(x[0], x[1]), None), (_sub(x[0], x[1]), None)]
    e = _rdft(x[0::2])
    o = _rdft(x[1::2])
    out = [None] * (n // 2 + 1)
    for k in range(n // 4 + 1):
        t = _cmul_const(o[k], math.cos(2 * math.pi * k / n),
                        -math.sin(2 * math.pi * k / n))
        out[k] = (_add(e[k][0], t[0]), _add(e[k][1], t[1]))
        if n // 2 - k != k:
            out[n // 2 - k] = (_sub(e[k][0], t[0]), _sub(t[1], e[k][1]))
    return out


def _irdft(x, n, need):
    if n == 1:
        return [x[0][0]]
    if n == 2:
        out = [_add(x[0][0], x[1][0])]
        if need > 1:
            out.append(_sub(x[0][0], x[1][0]))
        return out
    e = [None] * (n // 4 + 1)
    o = [None] * (n // 4 + 1)
    for k in range(n // 4 + 1):
        a = x[k]
        b = x[n // 2 - k]
        e[k] = (_add(a[0], b[0]), _sub(a[1], b[1]))
        d = (_sub(a[0], b[0]), _add(a[1], b[1]))
        o[k] = _cmul_const(d, math.cos(2 * math.pi * k / n),
                           math.sin(2 * math.pi * k / n))
    ne = (need + 1) // 2
    no = need // 2
    xe = _irdft(e, n // 2, ne)
    xo = _irdft(o, n // 2, no) if no > 0 else []
    return [xe[i // 2] if i % 2 == 0 else xo[i // 2] for i in range(need)]


def _dft_tables():
    b = np.arange(NB)
    fwd = np.zeros((NF1, 2 * NB, 2 * NB), np.float64)
    inv = np.zeros((NF1, 2 * NB, 2 * NB), np.float64)
    for f1 in range(NF1):
        f = f1 + NA * b
        th = 2.0 * np.pi * ((b[:, None] * f[None, :]) % L) / L
        c, s = np.cos(th), np.sin(th)
        fwd[f1] = np.block([[c, -s], [s, c]])
        inv[f1] = np.block([[c.T, s.T], [-s.T, c.T]]) / L
    return fwd.astype(np.float32), inv.astype(np.float32)


def _kernel(q_hbm, k_hbm, v_hbm, sk_ref, hk_hbm, sd_ref, w1_hbm, w2_hbm,
            wf_hbm, wi_hbm, o_hbm,
            q_ref, k_ref, v_ref, hk_ref, w1_ref, w2_ref, o_ref,
            wf_ref, wi_ref, w1t_ref, par_ref, u_ref, g_ref, p_ref, y_ref,
            hb_ref, base_ref, xn_ref, sem, osem):
    f32 = jnp.float32
    bf16 = jnp.bfloat16
    NCH = F // FC
    NIT = 2 * NCH
    CPI = D // NIT
    RI = D // NCH

    def kvh_copies(i):
        rows = pl.ds(i * CPI, CPI)
        return [pltpu.make_async_copy(src.at[rows, :], dst.at[rows, :],
                                      sem.at[3 * i + j])
                for j, (src, dst) in enumerate(
                    ((k_hbm, k_ref), (v_hbm, v_ref), (hk_hbm, hk_ref)))]

    def q_copy(tb):
        cols = pl.ds(tb * TB, TB)
        return pltpu.make_async_copy(q_hbm.at[:, cols], q_ref.at[:, cols],
                                     sem.at[3 * NIT + tb])

    cp_w1 = pltpu.make_async_copy(w1_hbm, w1_ref, sem.at[3 * NIT + NTB])
    cp_w2 = pltpu.make_async_copy(w2_hbm, w2_ref, sem.at[3 * NIT + NTB + 1])
    cp_wf = pltpu.make_async_copy(wf_hbm, wf_ref, sem.at[3 * NIT + NTB + 2])
    cp_wi = pltpu.make_async_copy(wi_hbm, wi_ref, sem.at[3 * NIT + NTB + 3])
    PRE = 5
    LA = 3
    WAITS = {0: range(5, 9), 4: range(9, NIT)}

    def start_kvh(rng):
        for i in rng:
            for cp in kvh_copies(i):
                cp.start()

    start_kvh(range(PRE - 1))

    def params():
        par = jnp.concatenate(
            [sk_ref[...].astype(f32), sd_ref[...].astype(f32),
             jnp.zeros((3, D), f32)], axis=0)
        par_ref[...] = par.T

    def kv_rows(r0, n):
        rows = pl.ds(r0, n)
        par = par_ref[rows, :]
        k = k_ref[rows, :].astype(f32)
        lane = jax.lax.broadcasted_iota(jnp.int32, (n, S), 1)
        ks = k * par[:, 0:1]
        for j in range(1, 4):
            kj = jnp.where(lane >= j, pltpu.roll(k, j, 1), 0.0)
            ks = ks + kj * par[:, j:j + 1]
        u_ref[rows, :] = ks * v_ref[rows, :].astype(f32)

    def s1_rows(src, r8, g8):
        xs = [src[pl.ds(r8, 8), pl.ds(NB * a, NB)].astype(f32)
              for a in range(NA // 2)]
        xs = xs + [None] * (NA // 2)
        g = _rdft(xs)
        for f1 in range(NF1):
            gr, gi = g[f1]
            if gi is None:
                gi = jnp.zeros((8, NB), f32)
            g_ref[f1, pl.ds(g8, 8), pl.ds(0, NB)] = gr
            g_ref[f1, pl.ds(g8, 8), pl.ds(NB, NB)] = gi
        return g[NF1 // 2][1]

    def spec_stage():
        for f1 in range(NF1):
            x = jnp.dot(g_ref[f1].astype(bf16), wf_ref[f1],
                        preferred_element_type=f32)
            xr, xi = x[:D, :NB], x[:D, NB:]
            hr, hi = x[D:, :NB], x[D:, NB:]
            yr = xr * hr - xi * hi
            yi = xr * hi + xi * hr
            yy = jnp.concatenate([yr, yi], axis=1).astype(bf16)
            p_ref[f1] = jnp.dot(yy, wi_ref[f1], preferred_element_type=f32)

    def i1_rows(r8):
        rows = pl.ds(r8, 8)
        xs = [(p_ref[f1, rows, pl.ds(0, NB)], p_ref[f1, rows, pl.ds(NB, NB)])
              for f1 in range(NF1)]
        y = _irdft(xs, NA, NA // 2)
        sd = par_ref[rows, :][:, 4:5]
        for a in range(NA // 2):
            col = pl.ds(NB * a, NB)
            yc = y[a].astype(bf16).astype(f32)
            tok = yc + u_ref[rows, col] * sd
            y_ref[rows, col] = tok
        return tok

    def layernorm(tb):
        cols = pl.ds(tb * TB, TB)
        x = q_ref[:, cols].astype(f32)
        mean = jnp.mean(x, axis=0, keepdims=True)
        xc = x - mean
        var = jnp.mean(xc * xc, axis=0, keepdims=True)
        xn = xc * jax.lax.rsqrt(var + EPS)
        xn_ref[pl.ds(0, D), cols] = xn.astype(bf16)
        base_ref[:, cols] = x

    def ffn_up(n):
        tb, i = divmod(n, NCH)
        h = jnp.dot(w1t_ref[pl.ds(i * FC, FC), :],
                    xn_ref[:, pl.ds(tb * TB, TB)],
                    preferred_element_type=f32)
        hh = 0.5 * h
        hb_ref[n % 2] = (hh + hh * jnp.tanh(hh)).astype(bf16)

    def ffn_down(n):
        tb, i = divmod(n, NCH)
        part = jnp.dot(w2_ref[:, pl.ds(i * FC, FC)], hb_ref[n % 2],
                       preferred_element_type=f32)
        cols = pl.ds(tb * TB, TB)
        base_ref[:, cols] = base_ref[:, cols] + part

    def combine(rows, cols):
        out = (base_ref[rows, cols]
               + xn_ref[rows, cols].astype(f32) * y_ref[rows, cols])
        o_ref[rows, cols] = out.astype(o_ref.dtype)
        return out[0:8, 0:NB]

    def order_before(tok, g, n):
        if n < NTB * NCH:
            i = n % NCH
            t = jnp.clip(tok[:, :DP - D], -1.0, 1.0)
            t = jnp.where(t == t, t, 0.0)
            w1t_ref[pl.ds(i * FC + 8 * g, 8), pl.ds(D, DP - D)] = (
                t.astype(bf16))

    def out_copy(rows, cols, s):
        return pltpu.make_async_copy(o_ref.at[rows, cols],
                                     o_hbm.at[rows, cols], osem.at[s])

    def fwd_slot(i, n):
        kv_rows(i * CPI, CPI)
        for g in range(CPI // 8):
            r8 = i * CPI + g * 8
            order_before(s1_rows(u_ref, r8, r8), 2 * g, n)
            order_before(s1_rows(hk_ref, r8, D + r8), 2 * g + 1, n)

    N_S1 = NIT - PRE
    N_I1 = N_S1 + NCH
    N_C01 = (NTB - 1) * NCH + 1
    first2 = pl.ds(0, 2 * TB)
    third = pl.ds(2 * TB, TB)

    def row_part(j, parts):
        units = D // 16
        lo = (units * j // parts) * 16
        hi = (units * (j + 1) // parts) * 16
        return pl.ds(lo, hi - lo)

    def extra(n):
        if n < N_S1:
            fwd_slot(n + PRE, n + LA)
        elif n < N_I1:
            i = n - N_S1
            for g in range(RI // 8):
                order_before(i1_rows(i * RI + g * 8), g, n + LA)
        elif n < N_C01:
            rows = row_part(n - N_I1, N_C01 - N_I1)
            order_before(combine(rows, first2), 0, n + LA)
            out_copy(rows, first2, 0).start()
        else:
            rows = row_part(n - N_C01, NTB * NCH - N_C01)
            order_before(combine(rows, third), 0, n + LA)
            out_copy(rows, third, 1).start()

    with jax.named_scope("pro"):
        params()
        xn_ref[pl.ds(D, DP - D), :] = jnp.zeros((DP - D, S), bf16)
        w1t_ref[:, pl.ds(D, DP - D)] = jnp.zeros((F, DP - D), bf16)
        for i in range(PRE):
            for cp in kvh_copies(i):
                cp.wait()
            if i == 0:
                start_kvh(range(PRE - 1, PRE))
                cp_w1.start()
                q_copy(0).start()
            if i == 3:
                cp_w2.start()
            fwd_slot(i, NTB * NCH)
        cp_w1.wait()
        start_kvh(WAITS[0])
        w1t_ref[:, pl.ds(0, D)] = w1_ref[...].astype(f32).T.astype(bf16)
        q_copy(0).wait()
        layernorm(0)
        ffn_up(0)
        cp_w2.wait()

    for n in range(NTB * NCH):
        for i in WAITS.get(n, ()):
            for cp in kvh_copies(i):
                cp.wait()
        if n == 0:
            start_kvh(WAITS[4])
            q_copy(1).start()
        if n == 4:
            cp_wf.start()
            cp_wi.start()
            q_copy(2).start()
            q_copy(3).start()
            q_copy(1).wait()
            layernorm(1)
        if n == N_S1:
            cp_wf.wait()
            cp_wi.wait()
            q_copy(2).wait()
            q_copy(3).wait()
            spec_stage()
            layernorm(2)
            layernorm(3)
        extra(n)
        if n + 1 < NTB * NCH:
            ffn_up(n + 1)
        ffn_down(n)

    with jax.named_scope("fin"):
        late = pl.ds((NTB - 1) * TB, TB)
        combine(pl.ds(0, D), late)
        cp_late = out_copy(pl.ds(0, D), late, 2)
        cp_late.start()
        out_copy(pl.ds(0, D), first2, 0).wait()
        out_copy(pl.ds(0, D), third, 1).wait()
        cp_late.wait()


@jax.jit
def pallas_parallel_sum__ssm_conv_h3__dense_activation_silu__prompt_kernel(
    A_q: jax.Array,
    A_k: jax.Array,
    A_v: jax.Array,
    A_shift_k: jax.Array,
    A_ssm_k: jax.Array,
    A_ssm_D: jax.Array,
    B_x: jax.Array,
    B_w1: jax.Array,
    B_w2: jax.Array,
):
    del B_x
    qt = A_q.reshape(S, D).T
    kt = A_k.reshape(S, D).T
    vt = A_v.reshape(S, D).T
    sk = A_shift_k.T
    sd = A_ssm_D.reshape(1, D)
    w2t = B_w2.T
    wf_np, wi_np = _dft_tables()
    wf = jnp.asarray(wf_np, dtype=jnp.bfloat16)
    wi = jnp.asarray(wi_np, dtype=jnp.bfloat16)

    hbm = pl.BlockSpec(memory_space=pl.ANY)
    vmem = pl.BlockSpec(memory_space=pltpu.VMEM)
    in_specs = [hbm, hbm, hbm, vmem, hbm, vmem, hbm, hbm, hbm, hbm]
    bf = jnp.bfloat16
    scratch = [
        pltpu.VMEM((D, S), bf),
        pltpu.VMEM((D, S), bf),
        pltpu.VMEM((D, S), bf),
        pltpu.VMEM((D, S), bf),
        pltpu.VMEM((D, F), bf),
        pltpu.VMEM((D, F), bf),
        pltpu.VMEM((D, S), bf),
        pltpu.VMEM((NF1, 2 * NB, 2 * NB), bf),
        pltpu.VMEM((NF1, 2 * NB, 2 * NB), bf),
        pltpu.VMEM((F, DP), bf),
        pltpu.VMEM((D, 8), jnp.float32),
        pltpu.VMEM((D, S), jnp.float32),
        pltpu.VMEM((NF1, 2 * D, 2 * NB), jnp.float32),
        pltpu.VMEM((NF1, D, 2 * NB), jnp.float32),
        pltpu.VMEM((D, S), jnp.float32),
        pltpu.VMEM((2, FC, TB), bf),
        pltpu.VMEM((D, S), jnp.float32),
        pltpu.VMEM((DP, S), bf),
        pltpu.SemaphoreType.DMA((3 * 2 * (F // FC) + NTB + 4,)),
        pltpu.SemaphoreType.DMA((3,)),
    ]
    out = pl.pallas_call(
        _kernel,
        in_specs=in_specs,
        out_specs=hbm,
        out_shape=jax.ShapeDtypeStruct((D, S), bf),
        scratch_shapes=scratch,
        compiler_params=pltpu.CompilerParams(
            vmem_limit_bytes=100 * 1024 * 1024,
        ),
    )(qt, kt, vt, sk, A_ssm_k, sd, B_w1, w2t, wf, wi)
    return out.T.reshape(1, S, D)
```

```python
import math

import numpy as np
import jax
import jax.numpy as jnp
import jax.experimental.pallas as pl
import jax.experimental.pallas.tpu as pltpu

S = 2048
D = 448
F = 1792
L = 2 * S
NB = 128
NA = L // NB
NF1 = NA // 2 + 1
NFF = NA + 1
CR = 224
NCB = D // CR
TB = 512
NTB = S // TB
DP = 512
FC = 256
EPS = 1e-5


def _add(a, b):
    if a is None:
        return b
    if b is None:
        return a
    return a + b


def _sub(a, b):
    if b is None:
        return a
    if a is None:
        return -b
    return a - b


def _mulc(a, c):
    if a is None or c == 0.0:
        return None
    if c == 1.0:
        return a
    if c == -1.0:
        return -a
    return a * c


def _cmul_const(z, wr, wi):
    zr, zi = z
    if abs(wr) < 1e-12:
        wr = 0.0
    if abs(wi) < 1e-12:
        wi = 0.0
    if abs(abs(wr) - 1) < 1e-12:
        wr = math.copysign(1.0, wr)
    if abs(abs(wi) - 1) < 1e-12:
        wi = math.copysign(1.0, wi)
    re = _sub(_mulc(zr, wr), _mulc(zi, wi))
    im = _add(_mulc(zr, wi), _mulc(zi, wr))
    return (re, im)


def _rdft(x):
    n = len(x)
    if n == 1:
        return [(x[0], None)]
    if n == 2:
        return [(_add(x[0], x[1]), None), (_sub(x[0], x[1]), None)]
    e = _rdft(x[0::2])
    o = _rdft(x[1::2])
    out = [None] * (n // 2 + 1)
    for k in range(n // 4 + 1):
        t = _cmul_const(o[k], math.cos(2 * math.pi * k / n),
                        -math.sin(2 * math.pi * k / n))
        out[k] = (_add(e[k][0], t[0]), _add(e[k][1], t[1]))
        if n // 2 - k != k:
            out[n // 2 - k] = (_sub(e[k][0], t[0]), _sub(t[1], e[k][1]))
    return out


def _irdft(x, n, need):
    if n == 1:
        return [x[0][0]]
    if n == 2:
        out = [_add(x[0][0], x[1][0])]
        if need > 1:
            out.append(_sub(x[0][0], x[1][0]))
        return out
    e = [None] * (n // 4 + 1)
    o = [None] * (n // 4 + 1)
    for k in range(n // 4 + 1):
        a = x[k]
        b = x[n // 2 - k]
        e[k] = (_add(a[0], b[0]), _sub(a[1], b[1]))
        d = (_sub(a[0], b[0]), _add(a[1], b[1]))
        o[k] = _cmul_const(d, math.cos(2 * math.pi * k / n),
                           math.sin(2 * math.pi * k / n))
    ne = (need + 1) // 2
    no = need // 2
    xe = _irdft(e, n // 2, ne)
    xo = _irdft(o, n // 2, no) if no > 0 else []
    return [xe[i // 2] if i % 2 == 0 else xo[i // 2] for i in range(need)]


def _dft_tables():
    hb = NB // 2
    b = np.arange(hb)
    fwd = np.zeros((NFF, NB, NB), np.float64)
    inv = np.zeros((NFF, NB, NB), np.float64)
    for f1 in range(NFF):
        f = f1 + 2 * NA * b
        th = 2.0 * np.pi * ((b[:, None] * f[None, :]) % L) / L
        c, s = np.cos(th), np.sin(th)
        fwd[f1] = np.block([[c, -s], [s, c]])
        inv[f1] = np.block([[c.T, s.T], [-s.T, c.T]]) / L
        if f1 > NA // 2:
            fwd[f1, hb:, :] *= -1.0
            inv[f1, :, hb:] *= -1.0
    return fwd.astype(np.float32), inv.astype(np.float32)


def _kernel(q_hbm, k_hbm, v_hbm, sk_ref, hk_hbm, sd_ref, w1_hbm, w2_hbm,
            wf_hbm, wi_hbm, o_hbm,
            q_ref, k_ref, v_ref, hk_ref, w1_ref, w2_ref, o_ref,
            wf_ref, wi_ref, w1t_ref, par_ref, u_ref, g_ref, p_ref, y_ref,
            hb_ref, base_ref, xn_ref, sem, osem):
    f32 = jnp.float32
    bf16 = jnp.bfloat16
    NCH = F // FC
    NIT = 2 * NCH
    CPI = D // NIT
    RI = D // NCH

    def kvh_copies(i):
        rows = pl.ds(i * CPI, CPI)
        return [pltpu.make_async_copy(src.at[rows, :], dst.at[rows, :],
                                      sem.at[3 * i + j])
                for j, (src, dst) in enumerate(
                    ((k_hbm, k_ref), (v_hbm, v_ref), (hk_hbm, hk_ref)))]

    def q_copy(tb):
        cols = pl.ds(tb * TB, TB)
        return pltpu.make_async_copy(q_hbm.at[:, cols], q_ref.at[:, cols],
                                     sem.at[3 * NIT + tb])

    cp_w1 = pltpu.make_async_copy(w1_hbm, w1_ref, sem.at[3 * NIT + NTB])
    cp_w2 = pltpu.make_async_copy(w2_hbm, w2_ref, sem.at[3 * NIT + NTB + 1])
    cp_wf = pltpu.make_async_copy(wf_hbm, wf_ref, sem.at[3 * NIT + NTB + 2])
    cp_wi = pltpu.make_async_copy(wi_hbm, wi_ref, sem.at[3 * NIT + NTB + 3])
    PRE = 5
    LA = 3
    WAITS = {0: range(5, 9), 4: range(9, NIT)}

    def start_kvh(rng):
        for i in rng:
            for cp in kvh_copies(i):
                cp.start()

    start_kvh(range(PRE - 1))

    def params():
        par = jnp.concatenate(
            [sk_ref[...].astype(f32), sd_ref[...].astype(f32),
             jnp.zeros((3, D), f32)], axis=0)
        par_ref[...] = par.T

    def kv_rows(r0, n):
        rows = pl.ds(r0, n)
        par = par_ref[rows, :]
        k = k_ref[rows, :].astype(f32)
        lane = jax.lax.broadcasted_iota(jnp.int32, (n, S), 1)
        ks = k * par[:, 0:1]
        for j in range(1, 4):
            kj = jnp.where(lane >= j, pltpu.roll(k, j, 1), 0.0)
            ks = ks + kj * par[:, j:j + 1]
        u_ref[rows, :] = ks * v_ref[rows, :].astype(f32)

    def s1_rows(src, r8, g8):
        xs = [src[pl.ds(r8, 8), pl.ds(NB * a, NB)].astype(f32)
              for a in range(NA // 2)]
        xs = xs + [None] * (NA // 2)
        g = _rdft(xs)
        for f1 in range(NF1):
            gr, gi = g[f1]
            if gi is None:
                gi = jnp.zeros((8, NB), f32)
            g_ref[f1, pl.ds(g8, 8), pl.ds(0, NB)] = gr
            g_ref[f1, pl.ds(g8, 8), pl.ds(NB, NB)] = gi
        return g[NF1 // 2][1]

    def spec_stage():
        hb = NB // 2

        def lane_consts(rows):
            low = jax.lax.broadcasted_iota(jnp.int32, (rows, NB), 1) < hb
            return low, jnp.where(low, 1.0, -1.0).astype(f32)

        low2, sgn2 = lane_consts(2 * D)
        low1, sgn1 = lane_consts(D)
        swap = lambda x: pltpu.roll(x, hb, 1)

        def through(z, f1):
            x = jnp.dot(z.astype(bf16), wf_ref[f1],
                        preferred_element_type=f32)
            xu, xh = x[:D], x[D:]
            xs, hs = swap(xu), swap(xh)
            y = (jnp.where(low1, xu, xs) * xh
                 - jnp.where(low1, xs, -xu) * hs)
            return jnp.dot(y.astype(bf16), wi_ref[f1],
                           preferred_element_type=f32)

        for m in range(NF1):
            c = math.cos(2 * math.pi * m / (2 * NA))
            s = math.sin(2 * math.pi * m / (2 * NA))
            vr = g_ref[m, :, pl.ds(0, NB)]
            vi = g_ref[m, :, pl.ds(NB, NB)]
            rvr, rvi = swap(vr), swap(vi)
            p1 = jnp.where(low2, vr, rvi)
            p2 = jnp.where(low2, rvr, vi)
            if m == 0:
                t = p2
            else:
                p3 = jnp.where(low2, rvi, -vr)
                t = p3 if m == NF1 - 1 else c * p2 + s * p3
            pa = through(p1 + t, m)
            if m < NF1 - 1:
                pb = through(p1 - t, NA - m)
            else:
                pb = pa * sgn1
            e = pa + pb
            dif = pa - pb
            if m == 0:
                o = dif
            else:
                sd_ = swap(dif)
                sd_ = jnp.where(low1, -sd_, sd_)
                o = sd_ if m == NF1 - 1 else c * dif + s * sd_
            p_ref[m, :, pl.ds(0, NB)] = jnp.where(low1, e, swap(o))
            p_ref[m, :, pl.ds(NB, NB)] = jnp.where(low1, swap(e), o)

    def i1_rows(r8):
        rows = pl.ds(r8, 8)
        xs = [(p_ref[f1, rows, pl.ds(0, NB)], p_ref[f1, rows, pl.ds(NB, NB)])
              for f1 in range(NF1)]
        y = _irdft(xs, NA, NA // 2)
        sd = par_ref[rows, :][:, 4:5]
        for a in range(NA // 2):
            col = pl.ds(NB * a, NB)
            yc = y[a].astype(bf16).astype(f32)
            tok = yc + u_ref[rows, col] * sd
            y_ref[rows, col] = tok
        return tok

    def layernorm(tb):
        cols = pl.ds(tb * TB, TB)
        x = q_ref[:, cols].astype(f32)
        mean = jnp.mean(x, axis=0, keepdims=True)
        xc = x - mean
        var = jnp.mean(xc * xc, axis=0, keepdims=True)
        xn = xc * jax.lax.rsqrt(var + EPS)
        xn_ref[pl.ds(0, D), cols] = xn.astype(bf16)
        base_ref[:, cols] = x

    def ffn_up(n):
        tb, i = divmod(n, NCH)
        h = jnp.dot(w1t_ref[pl.ds(i * FC, FC), :],
                    xn_ref[:, pl.ds(tb * TB, TB)],
                    preferred_element_type=f32)
        hh = 0.5 * h
        hb_ref[n % 2] = (hh + hh * jnp.tanh(hh)).astype(bf16)

    def ffn_down(n):
        tb, i = divmod(n, NCH)
        part = jnp.dot(w2_ref[:, pl.ds(i * FC, FC)], hb_ref[n % 2],
                       preferred_element_type=f32)
        cols = pl.ds(tb * TB, TB)
        base_ref[:, cols] = base_ref[:, cols] + part

    def combine(rows, cols):
        out = (base_ref[rows, cols]
               + xn_ref[rows, cols].astype(f32) * y_ref[rows, cols])
        o_ref[rows, cols] = out.astype(o_ref.dtype)
        return out[0:8, 0:NB]

    def order_before(tok, g, n):
        if n < NTB * NCH:
            i = n % NCH
            t = jnp.clip(tok[:, :DP - D], -1.0, 1.0)
            t = jnp.where(t == t, t, 0.0)
            w1t_ref[pl.ds(i * FC + 8 * g, 8), pl.ds(D, DP - D)] = (
                t.astype(bf16))

    def out_copy(rows, cols, s):
        return pltpu.make_async_copy(o_ref.at[rows, cols],
                                     o_hbm.at[rows, cols], osem.at[s])

    def fwd_slot(i, n):
        kv_rows(i * CPI, CPI)
        for g in range(CPI // 8):
            r8 = i * CPI + g * 8
            order_before(s1_rows(u_ref, r8, r8), 2 * g, n)
            order_before(s1_rows(hk_ref, r8, D + r8), 2 * g + 1, n)

    N_S1 = NIT - PRE
    N_I1 = N_S1 + NCH
    N_C01 = (NTB - 1) * NCH + 1
    first2 = pl.ds(0, 2 * TB)
    third = pl.ds(2 * TB, TB)

    def row_part(j, parts):
        units = D // 16
        lo = (units * j // parts) * 16
        hi = (units * (j + 1) // parts) * 16
        return pl.ds(lo, hi - lo)

    def extra(n):
        if n < N_S1:
            fwd_slot(n + PRE, n + LA)
        elif n < N_I1:
            i = n - N_S1
            for g in range(RI // 8):
                order_before(i1_rows(i * RI + g * 8), g, n + LA)
        elif n < N_C01:
            rows = row_part(n - N_I1, N_C01 - N_I1)
            order_before(combine(rows, first2), 0, n + LA)
            out_copy(rows, first2, 0).start()
        else:
            rows = row_part(n - N_C01, NTB * NCH - N_C01)
            order_before(combine(rows, third), 0, n + LA)
            out_copy(rows, third, 1).start()

    with jax.named_scope("pro"):
        params()
        xn_ref[pl.ds(D, DP - D), :] = jnp.zeros((DP - D, S), bf16)
        w1t_ref[:, pl.ds(D, DP - D)] = jnp.zeros((F, DP - D), bf16)
        for i in range(PRE):
            for cp in kvh_copies(i):
                cp.wait()
            if i == 0:
                start_kvh(range(PRE - 1, PRE))
                cp_w1.start()
                q_copy(0).start()
            if i == 3:
                cp_w2.start()
            fwd_slot(i, NTB * NCH)
        cp_w1.wait()
        start_kvh(WAITS[0])
        w1t_ref[:, pl.ds(0, D)] = w1_ref[...].astype(f32).T.astype(bf16)
        q_copy(0).wait()
        layernorm(0)
        ffn_up(0)
        cp_w2.wait()

    for n in range(NTB * NCH):
        for i in WAITS.get(n, ()):
            for cp in kvh_copies(i):
                cp.wait()
        if n == 0:
            start_kvh(WAITS[4])
            q_copy(1).start()
        if n == 4:
            cp_wf.start()
            cp_wi.start()
            q_copy(2).start()
            q_copy(3).start()
            q_copy(1).wait()
            layernorm(1)
        if n == N_S1:
            cp_wf.wait()
            cp_wi.wait()
            q_copy(2).wait()
            q_copy(3).wait()
            spec_stage()
            layernorm(2)
            layernorm(3)
        extra(n)
        if n + 1 < NTB * NCH:
            ffn_up(n + 1)
        ffn_down(n)

    with jax.named_scope("fin"):
        late = pl.ds((NTB - 1) * TB, TB)
        combine(pl.ds(0, D), late)
        cp_late = out_copy(pl.ds(0, D), late, 2)
        cp_late.start()
        out_copy(pl.ds(0, D), first2, 0).wait()
        out_copy(pl.ds(0, D), third, 1).wait()
        cp_late.wait()


@jax.jit
def pallas_parallel_sum__ssm_conv_h3__dense_activation_silu__prompt_kernel(
    A_q: jax.Array,
    A_k: jax.Array,
    A_v: jax.Array,
    A_shift_k: jax.Array,
    A_ssm_k: jax.Array,
    A_ssm_D: jax.Array,
    B_x: jax.Array,
    B_w1: jax.Array,
    B_w2: jax.Array,
):
    del B_x
    qt = A_q.reshape(S, D).T
    kt = A_k.reshape(S, D).T
    vt = A_v.reshape(S, D).T
    sk = A_shift_k.T
    sd = A_ssm_D.reshape(1, D)
    w2t = B_w2.T
    wf_np, wi_np = _dft_tables()
    wf = jnp.asarray(wf_np, dtype=jnp.bfloat16)
    wi = jnp.asarray(wi_np, dtype=jnp.bfloat16)

    hbm = pl.BlockSpec(memory_space=pl.ANY)
    vmem = pl.BlockSpec(memory_space=pltpu.VMEM)
    in_specs = [hbm, hbm, hbm, vmem, hbm, vmem, hbm, hbm, hbm, hbm]
    bf = jnp.bfloat16
    scratch = [
        pltpu.VMEM((D, S), bf),
        pltpu.VMEM((D, S), bf),
        pltpu.VMEM((D, S), bf),
        pltpu.VMEM((D, S), bf),
        pltpu.VMEM((D, F), bf),
        pltpu.VMEM((D, F), bf),
        pltpu.VMEM((D, S), bf),
        pltpu.VMEM((NFF, NB, NB), bf),
        pltpu.VMEM((NFF, NB, NB), bf),
        pltpu.VMEM((F, DP), bf),
        pltpu.VMEM((D, 8), jnp.float32),
        pltpu.VMEM((D, S), jnp.float32),
        pltpu.VMEM((NF1, 2 * D, 2 * NB), jnp.float32),
        pltpu.VMEM((NF1, D, 2 * NB), jnp.float32),
        pltpu.VMEM((D, S), jnp.float32),
        pltpu.VMEM((2, FC, TB), bf),
        pltpu.VMEM((D, S), jnp.float32),
        pltpu.VMEM((DP, S), bf),
        pltpu.SemaphoreType.DMA((3 * 2 * (F // FC) + NTB + 4,)),
        pltpu.SemaphoreType.DMA((3,)),
    ]
    out = pl.pallas_call(
        _kernel,
        in_specs=in_specs,
        out_specs=hbm,
        out_shape=jax.ShapeDtypeStruct((D, S), bf),
        scratch_shapes=scratch,
        compiler_params=pltpu.CompilerParams(
            vmem_limit_bytes=100 * 1024 * 1024,
        ),
    )(qt, kt, vt, sk, A_ssm_k, sd, B_w1, w2t, wf, wi)
    return out.T.reshape(1, S, D)
```

```python
import math

import numpy as np
import jax
import jax.numpy as jnp
import jax.experimental.pallas as pl
import jax.experimental.pallas.tpu as pltpu

S = 2048
D = 448
F = 1792
L = 2 * S
NB = 128
NA = L // NB
NF1 = NA // 2 + 1
NFF = NA + 1
CR = 224
NCB = D // CR
TB = 512
NTB = S // TB
DP = 512
FC = 256
EPS = 1e-5


def _add(a, b):
    if a is None:
        return b
    if b is None:
        return a
    return a + b


def _sub(a, b):
    if b is None:
        return a
    if a is None:
        return -b
    return a - b


def _mulc(a, c):
    if a is None or c == 0.0:
        return None
    if c == 1.0:
        return a
    if c == -1.0:
        return -a
    return a * c


def _cmul_const(z, wr, wi):
    zr, zi = z
    if abs(wr) < 1e-12:
        wr = 0.0
    if abs(wi) < 1e-12:
        wi = 0.0
    if abs(abs(wr) - 1) < 1e-12:
        wr = math.copysign(1.0, wr)
    if abs(abs(wi) - 1) < 1e-12:
        wi = math.copysign(1.0, wi)
    re = _sub(_mulc(zr, wr), _mulc(zi, wi))
    im = _add(_mulc(zr, wi), _mulc(zi, wr))
    return (re, im)


def _rdft(x):
    n = len(x)
    if n == 1:
        return [(x[0], None)]
    if n == 2:
        return [(_add(x[0], x[1]), None), (_sub(x[0], x[1]), None)]
    e = _rdft(x[0::2])
    o = _rdft(x[1::2])
    out = [None] * (n // 2 + 1)
    for k in range(n // 4 + 1):
        t = _cmul_const(o[k], math.cos(2 * math.pi * k / n),
                        -math.sin(2 * math.pi * k / n))
        out[k] = (_add(e[k][0], t[0]), _add(e[k][1], t[1]))
        if n // 2 - k != k:
            out[n // 2 - k] = (_sub(e[k][0], t[0]), _sub(t[1], e[k][1]))
    return out


def _irdft(x, n, need):
    if n == 1:
        return [x[0][0]]
    if n == 2:
        out = [_add(x[0][0], x[1][0])]
        if need > 1:
            out.append(_sub(x[0][0], x[1][0]))
        return out
    e = [None] * (n // 4 + 1)
    o = [None] * (n // 4 + 1)
    for k in range(n // 4 + 1):
        a = x[k]
        b = x[n // 2 - k]
        e[k] = (_add(a[0], b[0]), _sub(a[1], b[1]))
        d = (_sub(a[0], b[0]), _add(a[1], b[1]))
        o[k] = _cmul_const(d, math.cos(2 * math.pi * k / n),
                           math.sin(2 * math.pi * k / n))
    ne = (need + 1) // 2
    no = need // 2
    xe = _irdft(e, n // 2, ne)
    xo = _irdft(o, n // 2, no) if no > 0 else []
    return [xe[i // 2] if i % 2 == 0 else xo[i // 2] for i in range(need)]


def _dft_tables():
    hb = NB // 2
    b = np.arange(hb)
    fwd = np.zeros((NFF, NB, NB), np.float64)
    inv = np.zeros((NFF, NB, NB), np.float64)
    for f1 in range(NFF):
        f = f1 + 2 * NA * b
        th = 2.0 * np.pi * ((b[:, None] * f[None, :]) % L) / L
        c, s = np.cos(th), np.sin(th)
        fwd[f1] = np.block([[c, -s], [s, c]])
        inv[f1] = np.block([[c.T, s.T], [-s.T, c.T]]) / L
        if f1 > NA // 2:
            fwd[f1, hb:, :] *= -1.0
            inv[f1, :, hb:] *= -1.0
    return fwd.astype(np.float32), inv.astype(np.float32)


def _kernel(q_hbm, k_hbm, v_hbm, sk_ref, hk_hbm, sd_ref, w1_hbm, w2_hbm,
            wf_hbm, wi_hbm, o_hbm,
            q_ref, k_ref, v_ref, hk_ref, w1_ref, w2_ref, o_ref,
            wf_ref, wi_ref, w1t_ref, par_ref, u_ref, g_ref, p_ref, y_ref,
            hb_ref, base_ref, xn_ref, sem, osem):
    f32 = jnp.float32
    bf16 = jnp.bfloat16
    NCH = F // FC
    NIT = 2 * NCH
    CPI = D // NIT
    RI = D // NCH

    def kvh_copies(i):
        rows = pl.ds(i * CPI, CPI)
        return [pltpu.make_async_copy(src.at[rows, :], dst.at[rows, :],
                                      sem.at[3 * i + j])
                for j, (src, dst) in enumerate(
                    ((k_hbm, k_ref), (v_hbm, v_ref), (hk_hbm, hk_ref)))]

    def q_copy(tb):
        cols = pl.ds(tb * TB, TB)
        return pltpu.make_async_copy(q_hbm.at[:, cols], q_ref.at[:, cols],
                                     sem.at[3 * NIT + tb])

    cp_w1 = pltpu.make_async_copy(w1_hbm, w1_ref, sem.at[3 * NIT + NTB])
    cp_w2 = pltpu.make_async_copy(w2_hbm, w2_ref, sem.at[3 * NIT + NTB + 1])
    cp_wf = pltpu.make_async_copy(wf_hbm, wf_ref, sem.at[3 * NIT + NTB + 2])
    cp_wi = pltpu.make_async_copy(wi_hbm, wi_ref, sem.at[3 * NIT + NTB + 3])
    PRE = 5
    LA = 3
    WAITS = {0: range(5, 9), 4: range(9, NIT)}

    def start_kvh(rng):
        for i in rng:
            for cp in kvh_copies(i):
                cp.start()

    start_kvh(range(PRE - 1))

    def params():
        par = jnp.concatenate(
            [sk_ref[...].astype(f32), sd_ref[...].astype(f32),
             jnp.zeros((3, D), f32)], axis=0)
        par_ref[...] = par.T

    def kv_rows(r0, n):
        rows = pl.ds(r0, n)
        par = par_ref[rows, :]
        k = k_ref[rows, :].astype(f32)
        lane = jax.lax.broadcasted_iota(jnp.int32, (n, S), 1)
        ks = k * par[:, 0:1]
        for j in range(1, 4):
            kj = jnp.where(lane >= j, pltpu.roll(k, j, 1), 0.0)
            ks = ks + kj * par[:, j:j + 1]
        u_ref[rows, :] = ks * v_ref[rows, :].astype(f32)

    hb = NB // 2
    low8 = jax.lax.broadcasted_iota(jnp.int32, (8, NB), 1) < hb
    swap = lambda x: pltpu.roll(x, hb, 1)

    def tw64(m):
        return (math.cos(2 * math.pi * m / (2 * NA)),
                math.sin(2 * math.pi * m / (2 * NA)))

    def s1_rows(src, r8, g8):
        xs = [src[pl.ds(r8, 8), pl.ds(NB * a, NB)].astype(f32)
              for a in range(NA // 2)]
        xs = xs + [None] * (NA // 2)
        g = _rdft(xs)
        rows = pl.ds(g8, 8)
        for m in range(NF1):
            c, s = tw64(m)
            vr, vi = g[m]
            rvr = swap(vr)
            if vi is None:
                p1 = jnp.where(low8, vr, 0.0)
                p2 = jnp.where(low8, rvr, 0.0)
                p3 = jnp.where(low8, 0.0, -vr)
            else:
                rvi = swap(vi)
                p1 = jnp.where(low8, vr, rvi)
                p2 = jnp.where(low8, rvr, vi)
                p3 = jnp.where(low8, rvi, -vr)
            if m == 0:
                t = p2
            elif m == NF1 - 1:
                t = p3
            else:
                t = c * p2 + s * p3
            g_ref[m, rows, :] = p1 + t
            if m < NF1 - 1:
                g_ref[NA - m, rows, :] = p1 - t
        return t

    def spec_stage():
        low1 = jax.lax.broadcasted_iota(jnp.int32, (D, NB), 1) < hb

        def fwd(f1):
            g_ref[f1] = jnp.dot(g_ref[f1].astype(bf16), wf_ref[f1],
                                preferred_element_type=f32)

        def inv(f1):
            xu = g_ref[f1, pl.ds(0, D), :]
            xh = g_ref[f1, pl.ds(D, D), :]
            xs, hs = swap(xu), swap(xh)
            y = (jnp.where(low1, xu, xs) * xh
                 - jnp.where(low1, xs, -xu) * hs)
            p_ref[f1] = jnp.dot(y.astype(bf16), wi_ref[f1],
                                preferred_element_type=f32)

        fwd(0)
        fwd(1)
        for f1 in range(NFF):
            if f1 + 2 < NFF:
                fwd(f1 + 2)
            inv(f1)

    def i1_rows(r8):
        rows = pl.ds(r8, 8)
        xs = []
        for m in range(NF1):
            c, s = tw64(m)
            pa = p_ref[m, rows, :]
            if m < NF1 - 1:
                pb = p_ref[NA - m, rows, :]
            else:
                pb = jnp.where(low8, pa, -pa)
            e = pa + pb
            dif = pa - pb
            if m == 0:
                o = dif
            else:
                sd_ = swap(dif)
                sd_ = jnp.where(low8, -sd_, sd_)
                o = sd_ if m == NF1 - 1 else c * dif + s * sd_
            xs.append((jnp.where(low8, e, swap(o)),
                       jnp.where(low8, swap(e), o)))
        y = _irdft(xs, NA, NA // 2)
        sd = par_ref[rows, :][:, 4:5]
        for a in range(NA // 2):
            col = pl.ds(NB * a, NB)
            yc = y[a].astype(bf16).astype(f32)
            tok = yc + u_ref[rows, col] * sd
            y_ref[rows, col] = tok
        return tok

    def layernorm(tb):
        cols = pl.ds(tb * TB, TB)
        x = q_ref[:, cols].astype(f32)
        mean = jnp.mean(x, axis=0, keepdims=True)
        xc = x - mean
        var = jnp.mean(xc * xc, axis=0, keepdims=True)
        xn = xc * jax.lax.rsqrt(var + EPS)
        xn_ref[pl.ds(0, D), cols] = xn.astype(bf16)
        base_ref[:, cols] = x

    def ffn_up(n):
        tb, i = divmod(n, NCH)
        h = jnp.dot(w1t_ref[pl.ds(i * FC, FC), :],
                    xn_ref[:, pl.ds(tb * TB, TB)],
                    preferred_element_type=f32)
        hh = 0.5 * h
        hb_ref[n % 2] = (hh + hh * jnp.tanh(hh)).astype(bf16)

    def ffn_down(n):
        tb, i = divmod(n, NCH)
        part = jnp.dot(w2_ref[:, pl.ds(i * FC, FC)], hb_ref[n % 2],
                       preferred_element_type=f32)
        cols = pl.ds(tb * TB, TB)
        base_ref[:, cols] = base_ref[:, cols] + part

    def combine(rows, cols):
        out = (base_ref[rows, cols]
               + xn_ref[rows, cols].astype(f32) * y_ref[rows, cols])
        o_ref[rows, cols] = out.astype(o_ref.dtype)
        return out[0:8, 0:NB]

    def order_before(tok, g, n):
        if n < NTB * NCH:
            i = n % NCH
            t = jnp.clip(tok[:, :DP - D], -1.0, 1.0)
            t = jnp.where(t == t, t, 0.0)
            w1t_ref[pl.ds(i * FC + 8 * g, 8), pl.ds(D, DP - D)] = (
                t.astype(bf16))

    def out_copy(rows, cols, s):
        return pltpu.make_async_copy(o_ref.at[rows, cols],
                                     o_hbm.at[rows, cols], osem.at[s])

    def fwd_slot(i, n):
        kv_rows(i * CPI, CPI)
        for g in range(CPI // 8):
            r8 = i * CPI + g * 8
            order_before(s1_rows(u_ref, r8, r8), 2 * g, n)
            order_before(s1_rows(hk_ref, r8, D + r8), 2 * g + 1, n)

    N_S1 = NIT - PRE
    N_I1 = N_S1 + NCH
    N_C01 = (NTB - 1) * NCH + 1
    first2 = pl.ds(0, 2 * TB)
    third = pl.ds(2 * TB, TB)

    def row_part(j, parts):
        units = D // 16
        lo = (units * j // parts) * 16
        hi = (units * (j + 1) // parts) * 16
        return pl.ds(lo, hi - lo)

    def extra(n):
        if n < N_S1:
            fwd_slot(n + PRE, n + LA)
        elif n < N_I1:
            i = n - N_S1
            for g in range(RI // 8):
                order_before(i1_rows(i * RI + g * 8), g, n + LA)
        elif n < N_C01:
            rows = row_part(n - N_I1, N_C01 - N_I1)
            order_before(combine(rows, first2), 0, n + LA)
            out_copy(rows, first2, 0).start()
        else:
            rows = row_part(n - N_C01, NTB * NCH - N_C01)
            order_before(combine(rows, third), 0, n + LA)
            out_copy(rows, third, 1).start()

    with jax.named_scope("pro"):
        params()
        xn_ref[pl.ds(D, DP - D), :] = jnp.zeros((DP - D, S), bf16)
        w1t_ref[:, pl.ds(D, DP - D)] = jnp.zeros((F, DP - D), bf16)
        for i in range(PRE):
            for cp in kvh_copies(i):
                cp.wait()
            if i == 0:
                start_kvh(range(PRE - 1, PRE))
                cp_w1.start()
                q_copy(0).start()
            if i == 3:
                cp_w2.start()
            fwd_slot(i, NTB * NCH)
        cp_w1.wait()
        start_kvh(WAITS[0])
        w1t_ref[:, pl.ds(0, D)] = w1_ref[...].astype(f32).T.astype(bf16)
        q_copy(0).wait()
        layernorm(0)
        ffn_up(0)
        cp_w2.wait()

    for n in range(NTB * NCH):
        for i in WAITS.get(n, ()):
            for cp in kvh_copies(i):
                cp.wait()
        if n == 0:
            start_kvh(WAITS[4])
            q_copy(1).start()
        if n == 4:
            cp_wf.start()
            cp_wi.start()
            q_copy(2).start()
            q_copy(3).start()
            q_copy(1).wait()
            layernorm(1)
        if n == N_S1:
            cp_wf.wait()
            cp_wi.wait()
            q_copy(2).wait()
            q_copy(3).wait()
            spec_stage()
            layernorm(2)
            layernorm(3)
        extra(n)
        if n + 1 < NTB * NCH:
            ffn_up(n + 1)
        ffn_down(n)

    with jax.named_scope("fin"):
        late = pl.ds((NTB - 1) * TB, TB)
        combine(pl.ds(0, D), late)
        cp_late = out_copy(pl.ds(0, D), late, 2)
        cp_late.start()
        out_copy(pl.ds(0, D), first2, 0).wait()
        out_copy(pl.ds(0, D), third, 1).wait()
        cp_late.wait()


@jax.jit
def pallas_parallel_sum__ssm_conv_h3__dense_activation_silu__prompt_kernel(
    A_q: jax.Array,
    A_k: jax.Array,
    A_v: jax.Array,
    A_shift_k: jax.Array,
    A_ssm_k: jax.Array,
    A_ssm_D: jax.Array,
    B_x: jax.Array,
    B_w1: jax.Array,
    B_w2: jax.Array,
):
    del B_x
    qt = A_q.reshape(S, D).T
    kt = A_k.reshape(S, D).T
    vt = A_v.reshape(S, D).T
    sk = A_shift_k.T
    sd = A_ssm_D.reshape(1, D)
    w2t = B_w2.T
    wf_np, wi_np = _dft_tables()
    wf = jnp.asarray(wf_np, dtype=jnp.bfloat16)
    wi = jnp.asarray(wi_np, dtype=jnp.bfloat16)

    hbm = pl.BlockSpec(memory_space=pl.ANY)
    vmem = pl.BlockSpec(memory_space=pltpu.VMEM)
    in_specs = [hbm, hbm, hbm, vmem, hbm, vmem, hbm, hbm, hbm, hbm]
    bf = jnp.bfloat16
    scratch = [
        pltpu.VMEM((D, S), bf),
        pltpu.VMEM((D, S), bf),
        pltpu.VMEM((D, S), bf),
        pltpu.VMEM((D, S), bf),
        pltpu.VMEM((D, F), bf),
        pltpu.VMEM((D, F), bf),
        pltpu.VMEM((D, S), bf),
        pltpu.VMEM((NFF, NB, NB), bf),
        pltpu.VMEM((NFF, NB, NB), bf),
        pltpu.VMEM((F, DP), bf),
        pltpu.VMEM((D, 8), jnp.float32),
        pltpu.VMEM((D, S), jnp.float32),
        pltpu.VMEM((NFF, 2 * D, NB), jnp.float32),
        pltpu.VMEM((NFF, D, NB), jnp.float32),
        pltpu.VMEM((D, S), jnp.float32),
        pltpu.VMEM((2, FC, TB), bf),
        pltpu.VMEM((D, S), jnp.float32),
        pltpu.VMEM((DP, S), bf),
        pltpu.SemaphoreType.DMA((3 * 2 * (F // FC) + NTB + 4,)),
        pltpu.SemaphoreType.DMA((3,)),
    ]
    out = pl.pallas_call(
        _kernel,
        in_specs=in_specs,
        out_specs=hbm,
        out_shape=jax.ShapeDtypeStruct((D, S), bf),
        scratch_shapes=scratch,
        compiler_params=pltpu.CompilerParams(
            vmem_limit_bytes=100 * 1024 * 1024,
        ),
    )(qt, kt, vt, sk, A_ssm_k, sd, B_w1, w2t, wf, wi)
    return out.T.reshape(1, S, D)
```

```python
import math

import numpy as np
import jax
import jax.numpy as jnp
import jax.experimental.pallas as pl
import jax.experimental.pallas.tpu as pltpu

S = 2048
D = 448
F = 1792
L = 2 * S
NB = 128
NA = L // NB
NF1 = NA // 2 + 1
NFF = NA + 1
CR = 224
NCB = D // CR
TB = 512
NTB = S // TB
DP = 512
FC = 256
EPS = 1e-5


def _add(a, b):
    if a is None:
        return b
    if b is None:
        return a
    return a + b


def _sub(a, b):
    if b is None:
        return a
    if a is None:
        return -b
    return a - b


def _mulc(a, c):
    if a is None or c == 0.0:
        return None
    if c == 1.0:
        return a
    if c == -1.0:
        return -a
    return a * c


def _cmul_const(z, wr, wi):
    zr, zi = z
    if abs(wr) < 1e-12:
        wr = 0.0
    if abs(wi) < 1e-12:
        wi = 0.0
    if abs(abs(wr) - 1) < 1e-12:
        wr = math.copysign(1.0, wr)
    if abs(abs(wi) - 1) < 1e-12:
        wi = math.copysign(1.0, wi)
    re = _sub(_mulc(zr, wr), _mulc(zi, wi))
    im = _add(_mulc(zr, wi), _mulc(zi, wr))
    return (re, im)


def _rdft(x):
    n = len(x)
    if n == 1:
        return [(x[0], None)]
    if n == 2:
        return [(_add(x[0], x[1]), None), (_sub(x[0], x[1]), None)]
    e = _rdft(x[0::2])
    o = _rdft(x[1::2])
    out = [None] * (n // 2 + 1)
    for k in range(n // 4 + 1):
        t = _cmul_const(o[k], math.cos(2 * math.pi * k / n),
                        -math.sin(2 * math.pi * k / n))
        out[k] = (_add(e[k][0], t[0]), _add(e[k][1], t[1]))
        if n // 2 - k != k:
            out[n // 2 - k] = (_sub(e[k][0], t[0]), _sub(t[1], e[k][1]))
    return out


def _irdft(x, n, need):
    if n == 1:
        return [x[0][0]]
    if n == 2:
        out = [_add(x[0][0], x[1][0])]
        if need > 1:
            out.append(_sub(x[0][0], x[1][0]))
        return out
    e = [None] * (n // 4 + 1)
    o = [None] * (n // 4 + 1)
    for k in range(n // 4 + 1):
        a = x[k]
        b = x[n // 2 - k]
        e[k] = (_add(a[0], b[0]), _sub(a[1], b[1]))
        d = (_sub(a[0], b[0]), _add(a[1], b[1]))
        o[k] = _cmul_const(d, math.cos(2 * math.pi * k / n),
                           math.sin(2 * math.pi * k / n))
    ne = (need + 1) // 2
    no = need // 2
    xe = _irdft(e, n // 2, ne)
    xo = _irdft(o, n // 2, no) if no > 0 else []
    return [xe[i // 2] if i % 2 == 0 else xo[i // 2] for i in range(need)]


def _dft_tables():
    hb = NB // 2
    b = np.arange(hb)
    fwd = np.zeros((NFF, NB, NB), np.float64)
    inv = np.zeros((NFF, NB, NB), np.float64)
    for f1 in range(NFF):
        f = f1 + 2 * NA * b
        th = 2.0 * np.pi * ((b[:, None] * f[None, :]) % L) / L
        c, s = np.cos(th), np.sin(th)
        fwd[f1] = np.block([[c, -s], [s, c]])
        inv[f1] = np.block([[c.T, s.T], [-s.T, c.T]]) / L
        if f1 > NA // 2:
            fwd[f1, hb:, :] *= -1.0
            inv[f1, :, hb:] *= -1.0
    return fwd.astype(np.float32), inv.astype(np.float32)


def _kernel(q_hbm, k_hbm, v_hbm, sk_ref, hk_hbm, sd_ref, w1_hbm, w2_hbm,
            wf_hbm, wi_hbm, o_hbm,
            q_ref, k_ref, v_ref, hk_ref, w1_ref, w2_ref, o_ref,
            wf_ref, wi_ref, w1t_ref, par_ref, u_ref, g_ref, p_ref, y_ref,
            hb_ref, base_ref, xn_ref, sem, osem):
    f32 = jnp.float32
    bf16 = jnp.bfloat16
    NCH = F // FC
    NIT = 2 * NCH
    CPI = D // NIT
    RI = D // NCH

    def kvh_copies(i):
        rows = pl.ds(i * CPI, CPI)
        return [pltpu.make_async_copy(src.at[rows, :], dst.at[rows, :],
                                      sem.at[3 * i + j])
                for j, (src, dst) in enumerate(
                    ((k_hbm, k_ref), (v_hbm, v_ref), (hk_hbm, hk_ref)))]

    def q_copy(tb):
        cols = pl.ds(tb * TB, TB)
        return pltpu.make_async_copy(q_hbm.at[:, cols], q_ref.at[:, cols],
                                     sem.at[3 * NIT + tb])

    cp_w1 = pltpu.make_async_copy(w1_hbm, w1_ref, sem.at[3 * NIT + NTB])
    cp_w2 = pltpu.make_async_copy(w2_hbm, w2_ref, sem.at[3 * NIT + NTB + 1])
    cp_wf = pltpu.make_async_copy(wf_hbm, wf_ref, sem.at[3 * NIT + NTB + 2])
    cp_wi = pltpu.make_async_copy(wi_hbm, wi_ref, sem.at[3 * NIT + NTB + 3])
    PRE = 5
    LA = 3

    def start_kvh(rng):
        for i in rng:
            for cp in kvh_copies(i):
                cp.start()

    start_kvh(range(PRE - 1))

    def params():
        par = jnp.concatenate(
            [sk_ref[...].astype(f32), sd_ref[...].astype(f32),
             jnp.zeros((3, D), f32)], axis=0)
        par_ref[...] = par.T

    def kv_rows(r0, n):
        rows = pl.ds(r0, n)
        par = par_ref[rows, :]
        k = k_ref[rows, :].astype(f32)
        lane = jax.lax.broadcasted_iota(jnp.int32, (n, S), 1)
        ks = k * par[:, 0:1]
        for j in range(1, 4):
            kj = jnp.where(lane >= j, pltpu.roll(k, j, 1), 0.0)
            ks = ks + kj * par[:, j:j + 1]
        u_ref[rows, :] = ks * v_ref[rows, :].astype(f32)

    hb = NB // 2
    low8 = jax.lax.broadcasted_iota(jnp.int32, (8, NB), 1) < hb
    swap = lambda x: pltpu.roll(x, hb, 1)

    def tw64(m):
        return (math.cos(2 * math.pi * m / (2 * NA)),
                math.sin(2 * math.pi * m / (2 * NA)))

    def s1_rows(src, r8, g8):
        xs = [src[pl.ds(r8, 8), pl.ds(NB * a, NB)].astype(f32)
              for a in range(NA // 2)]
        xs = xs + [None] * (NA // 2)
        g = _rdft(xs)
        rows = pl.ds(g8, 8)
        for m in range(NF1):
            c, s = tw64(m)
            vr, vi = g[m]
            rvr = swap(vr)
            if vi is None:
                p1 = jnp.where(low8, vr, 0.0)
                p2 = jnp.where(low8, rvr, 0.0)
                p3 = jnp.where(low8, 0.0, -vr)
            else:
                rvi = swap(vi)
                p1 = jnp.where(low8, vr, rvi)
                p2 = jnp.where(low8, rvr, vi)
                p3 = jnp.where(low8, rvi, -vr)
            if m == 0:
                t = p2
            elif m == NF1 - 1:
                t = p3
            else:
                t = c * p2 + s * p3
            g_ref[m, rows, :] = p1 + t
            if m < NF1 - 1:
                g_ref[NA - m, rows, :] = p1 - t
        return t

    def spec_stage():
        low1 = jax.lax.broadcasted_iota(jnp.int32, (D, NB), 1) < hb

        def fwd(f1):
            g_ref[f1] = jnp.dot(g_ref[f1].astype(bf16), wf_ref[f1],
                                preferred_element_type=f32)

        def inv(f1):
            xu = g_ref[f1, pl.ds(0, D), :]
            xh = g_ref[f1, pl.ds(D, D), :]
            xs, hs = swap(xu), swap(xh)
            y = (jnp.where(low1, xu, xs) * xh
                 - jnp.where(low1, xs, -xu) * hs)
            p_ref[f1] = jnp.dot(y.astype(bf16), wi_ref[f1],
                                preferred_element_type=f32)

        fwd(0)
        fwd(1)
        for f1 in range(NFF):
            if f1 + 2 < NFF:
                fwd(f1 + 2)
            inv(f1)

    def i1_rows(r8):
        rows = pl.ds(r8, 8)
        xs = []
        for m in range(NF1):
            c, s = tw64(m)
            pa = p_ref[m, rows, :]
            if m < NF1 - 1:
                pb = p_ref[NA - m, rows, :]
            else:
                pb = jnp.where(low8, pa, -pa)
            e = pa + pb
            dif = pa - pb
            if m == 0:
                o = dif
            else:
                sd_ = swap(dif)
                sd_ = jnp.where(low8, -sd_, sd_)
                o = sd_ if m == NF1 - 1 else c * dif + s * sd_
            xs.append((jnp.where(low8, e, swap(o)),
                       jnp.where(low8, swap(e), o)))
        y = _irdft(xs, NA, NA // 2)
        sd = par_ref[rows, :][:, 4:5]
        for a in range(NA // 2):
            col = pl.ds(NB * a, NB)
            yc = y[a].astype(bf16).astype(f32)
            tok = yc + u_ref[rows, col] * sd
            y_ref[rows, col] = tok
        return tok

    def layernorm(tb):
        cols = pl.ds(tb * TB, TB)
        x = q_ref[:, cols].astype(f32)
        mean = jnp.mean(x, axis=0, keepdims=True)
        xc = x - mean
        var = jnp.mean(xc * xc, axis=0, keepdims=True)
        xn = xc * jax.lax.rsqrt(var + EPS)
        xn_ref[pl.ds(0, D), cols] = xn.astype(bf16)
        base_ref[:, cols] = x

    def ffn_up(n):
        tb, i = divmod(n, NCH)
        h = jnp.dot(w1t_ref[pl.ds(i * FC, FC), :],
                    xn_ref[:, pl.ds(tb * TB, TB)],
                    preferred_element_type=f32)
        hh = 0.5 * h
        hb_ref[n % 2] = (hh + hh * jnp.tanh(hh)).astype(bf16)

    def ffn_down(n):
        tb, i = divmod(n, NCH)
        part = jnp.dot(w2_ref[:, pl.ds(i * FC, FC)], hb_ref[n % 2],
                       preferred_element_type=f32)
        cols = pl.ds(tb * TB, TB)
        base_ref[:, cols] = base_ref[:, cols] + part

    def combine(rows, cols):
        out = (base_ref[rows, cols]
               + xn_ref[rows, cols].astype(f32) * y_ref[rows, cols])
        o_ref[rows, cols] = out.astype(o_ref.dtype)
        return out[0:8, 0:NB]

    def order_before(tok, g, n):
        if n < NTB * NCH:
            i = n % NCH
            t = jnp.clip(tok[:, :DP - D], -1.0, 1.0)
            t = jnp.where(t == t, t, 0.0)
            w1t_ref[pl.ds(i * FC + 8 * g, 8), pl.ds(D, DP - D)] = (
                t.astype(bf16))

    def out_copy(rows, cols, s):
        return pltpu.make_async_copy(o_ref.at[rows, cols],
                                     o_hbm.at[rows, cols], osem.at[s])

    def fwd_slot(i, n):
        kv_rows(i * CPI, CPI)
        for g in range(CPI // 8):
            r8 = i * CPI + g * 8
            order_before(s1_rows(u_ref, r8, r8), 2 * g, n)
            order_before(s1_rows(hk_ref, r8, D + r8), 2 * g + 1, n)

    NSL = NTB * NCH
    N_S1 = 12
    N_I1 = 22
    early = pl.ds(0, (NTB - 1) * TB)

    def split(items, j, parts):
        return items[len(items) * j // parts:len(items) * (j + 1) // parts]

    def row_part(j, parts):
        units = D // 16
        lo = (units * j // parts) * 16
        hi = (units * (j + 1) // parts) * 16
        return pl.ds(lo, hi - lo)

    s1_units = list(range(PRE * CPI, D, 16))
    i1_units = list(range(0, D, 8))
    need = {}
    for n in range(N_S1):
        last = (split(s1_units, n, N_S1)[-1] + 15) // CPI
        need[n] = last
    WAITS = {}
    done = PRE - 1
    for n in (0, 5):
        hi = need[min(n + 4, N_S1 - 1)] if n == 0 else NIT - 1
        WAITS[n] = range(done + 1, hi + 1)
        done = hi

    def extra(n):
        if n < N_S1:
            g = 0
            for r16 in split(s1_units, n, N_S1):
                kv_rows(r16, 16)
                for r8 in (r16, r16 + 8):
                    order_before(s1_rows(u_ref, r8, r8), g, n + LA)
                    order_before(s1_rows(hk_ref, r8, D + r8), g + 1, n + LA)
                    g += 2
        elif n < N_I1:
            for g, r8 in enumerate(split(i1_units, n - N_S1, N_I1 - N_S1)):
                order_before(i1_rows(r8), g, n + LA)
        else:
            rows = row_part(n - N_I1, NSL - N_I1)
            order_before(combine(rows, early), 0, n + LA)
            out_copy(rows, early, 0).start()

    with jax.named_scope("pro"):
        params()
        xn_ref[pl.ds(D, DP - D), :] = jnp.zeros((DP - D, S), bf16)
        w1t_ref[:, pl.ds(D, DP - D)] = jnp.zeros((F, DP - D), bf16)
        for i in range(PRE):
            for cp in kvh_copies(i):
                cp.wait()
            if i == 0:
                start_kvh(range(PRE - 1, PRE))
                cp_w1.start()
                q_copy(0).start()
            if i == 3:
                cp_w2.start()
            fwd_slot(i, NSL)
        cp_w1.wait()
        start_kvh(WAITS[0])
        w1t_ref[:, pl.ds(0, D)] = w1_ref[...].astype(f32).T.astype(bf16)
        q_copy(0).wait()
        layernorm(0)
        ffn_up(0)
        cp_w2.wait()

    for n in range(NSL):
        for i in WAITS.get(n, ()):
            for cp in kvh_copies(i):
                cp.wait()
        if n == 0:
            start_kvh(WAITS[5])
            q_copy(1).start()
        if n == 5:
            cp_wf.start()
            cp_wi.start()
            q_copy(2).start()
            q_copy(3).start()
            q_copy(1).wait()
            layernorm(1)
        if n == N_S1:
            cp_wf.wait()
            cp_wi.wait()
            q_copy(2).wait()
            q_copy(3).wait()
            layernorm(2)
            spec_stage()
            layernorm(3)
        extra(n)
        if n + 1 < NSL:
            ffn_up(n + 1)
        ffn_down(n)

    with jax.named_scope("fin"):
        late = pl.ds((NTB - 1) * TB, TB)
        combine(pl.ds(0, D), late)
        cp_late = out_copy(pl.ds(0, D), late, 1)
        cp_late.start()
        out_copy(pl.ds(0, D), early, 0).wait()
        cp_late.wait()


@jax.jit
def pallas_parallel_sum__ssm_conv_h3__dense_activation_silu__prompt_kernel(
    A_q: jax.Array,
    A_k: jax.Array,
    A_v: jax.Array,
    A_shift_k: jax.Array,
    A_ssm_k: jax.Array,
    A_ssm_D: jax.Array,
    B_x: jax.Array,
    B_w1: jax.Array,
    B_w2: jax.Array,
):
    del B_x
    qt = A_q.reshape(S, D).T
    kt = A_k.reshape(S, D).T
    vt = A_v.reshape(S, D).T
    sk = A_shift_k.T
    sd = A_ssm_D.reshape(1, D)
    w2t = B_w2.T
    wf_np, wi_np = _dft_tables()
    wf = jnp.asarray(wf_np, dtype=jnp.bfloat16)
    wi = jnp.asarray(wi_np, dtype=jnp.bfloat16)

    hbm = pl.BlockSpec(memory_space=pl.ANY)
    vmem = pl.BlockSpec(memory_space=pltpu.VMEM)
    in_specs = [hbm, hbm, hbm, vmem, hbm, vmem, hbm, hbm, hbm, hbm]
    bf = jnp.bfloat16
    scratch = [
        pltpu.VMEM((D, S), bf),
        pltpu.VMEM((D, S), bf),
        pltpu.VMEM((D, S), bf),
        pltpu.VMEM((D, S), bf),
        pltpu.VMEM((D, F), bf),
        pltpu.VMEM((D, F), bf),
        pltpu.VMEM((D, S), bf),
        pltpu.VMEM((NFF, NB, NB), bf),
        pltpu.VMEM((NFF, NB, NB), bf),
        pltpu.VMEM((F, DP), bf),
        pltpu.VMEM((D, 8), jnp.float32),
        pltpu.VMEM((D, S), jnp.float32),
        pltpu.VMEM((NFF, 2 * D, NB), jnp.float32),
        pltpu.VMEM((NFF, D, NB), jnp.float32),
        pltpu.VMEM((D, S), jnp.float32),
        pltpu.VMEM((2, FC, TB), bf),
        pltpu.VMEM((D, S), jnp.float32),
        pltpu.VMEM((DP, S), bf),
        pltpu.SemaphoreType.DMA((3 * 2 * (F // FC) + NTB + 4,)),
        pltpu.SemaphoreType.DMA((2,)),
    ]
    out = pl.pallas_call(
        _kernel,
        in_specs=in_specs,
        out_specs=hbm,
        out_shape=jax.ShapeDtypeStruct((D, S), bf),
        scratch_shapes=scratch,
        compiler_params=pltpu.CompilerParams(
            vmem_limit_bytes=100 * 1024 * 1024,
        ),
    )(qt, kt, vt, sk, A_ssm_k, sd, B_w1, w2t, wf, wi)
    return out.T.reshape(1, S, D)
```

```python
import math

import numpy as np
import jax
import jax.numpy as jnp
import jax.experimental.pallas as pl
import jax.experimental.pallas.tpu as pltpu

S = 2048
D = 448
F = 1792
L = 2 * S
NB = 128
NA = L // NB
NF1 = NA // 2 + 1
NFF = NA + 1
TB = 512
NTB = S // TB
DP = 512
FC = 256
EPS = 1e-5


def _add(a, b):
    if a is None:
        return b
    if b is None:
        return a
    return a + b


def _sub(a, b):
    if b is None:
        return a
    if a is None:
        return -b
    return a - b


def _mulc(a, c):
    if a is None or c == 0.0:
        return None
    if c == 1.0:
        return a
    if c == -1.0:
        return -a
    return a * c


def _cmul_const(z, wr, wi):
    zr, zi = z
    if abs(wr) < 1e-12:
        wr = 0.0
    if abs(wi) < 1e-12:
        wi = 0.0
    if abs(abs(wr) - 1) < 1e-12:
        wr = math.copysign(1.0, wr)
    if abs(abs(wi) - 1) < 1e-12:
        wi = math.copysign(1.0, wi)
    re = _sub(_mulc(zr, wr), _mulc(zi, wi))
    im = _add(_mulc(zr, wi), _mulc(zi, wr))
    return (re, im)


def _rdft(x):
    n = len(x)
    if n == 1:
        return [(x[0], None)]
    if n == 2:
        return [(_add(x[0], x[1]), None), (_sub(x[0], x[1]), None)]
    e = _rdft(x[0::2])
    o = _rdft(x[1::2])
    out = [None] * (n // 2 + 1)
    for k in range(n // 4 + 1):
        t = _cmul_const(o[k], math.cos(2 * math.pi * k / n),
                        -math.sin(2 * math.pi * k / n))
        out[k] = (_add(e[k][0], t[0]), _add(e[k][1], t[1]))
        if n // 2 - k != k:
            out[n // 2 - k] = (_sub(e[k][0], t[0]), _sub(t[1], e[k][1]))
    return out


def _irdft(x, n, need):
    if n == 1:
        return [x[0][0]]
    if n == 2:
        out = [_add(x[0][0], x[1][0])]
        if need > 1:
            out.append(_sub(x[0][0], x[1][0]))
        return out
    e = [None] * (n // 4 + 1)
    o = [None] * (n // 4 + 1)
    for k in range(n // 4 + 1):
        a = x[k]
        b = x[n // 2 - k]
        e[k] = (_add(a[0], b[0]), _sub(a[1], b[1]))
        d = (_sub(a[0], b[0]), _add(a[1], b[1]))
        o[k] = _cmul_const(d, math.cos(2 * math.pi * k / n),
                           math.sin(2 * math.pi * k / n))
    ne = (need + 1) // 2
    no = need // 2
    xe = _irdft(e, n // 2, ne)
    xo = _irdft(o, n // 2, no) if no > 0 else []
    return [xe[i // 2] if i % 2 == 0 else xo[i // 2] for i in range(need)]


def _dft_tables():
    hb = NB // 2
    b = np.arange(hb)
    fwd = np.zeros((NFF, NB, NB), np.float64)
    inv = np.zeros((NFF, NB, NB), np.float64)
    for f1 in range(NFF):
        f = f1 + 2 * NA * b
        th = 2.0 * np.pi * ((b[:, None] * f[None, :]) % L) / L
        c, s = np.cos(th), np.sin(th)
        fwd[f1] = np.block([[c, -s], [s, c]])
        inv[f1] = np.block([[c.T, s.T], [-s.T, c.T]]) / L
        if f1 > NA // 2:
            fwd[f1, hb:, :] *= -1.0
            inv[f1, :, hb:] *= -1.0
    return fwd.astype(np.float32), inv.astype(np.float32)


def _kernel(q_hbm, k_hbm, v_hbm, sk_ref, hk_hbm, sd_ref, w1_hbm, w2_hbm,
            wf_hbm, wi_hbm, o_hbm,
            q_ref, k_ref, v_ref, hk_ref, w1_ref, w2_ref, o_ref,
            wf_ref, wi_ref, w1t_ref, par_ref, u_ref, g_ref, p_ref, y_ref,
            hb_ref, base_ref, xn_ref, sem, osem):
    f32 = jnp.float32
    bf16 = jnp.bfloat16
    NCH = F // FC
    NIT = 2 * NCH
    CPI = D // NIT

    def kvh_copies(i):
        rows = pl.ds(i * CPI, CPI)
        return [pltpu.make_async_copy(src.at[rows, :], dst.at[rows, :],
                                      sem.at[3 * i + j])
                for j, (src, dst) in enumerate(
                    ((k_hbm, k_ref), (v_hbm, v_ref), (hk_hbm, hk_ref)))]

    def q_copy(tb):
        cols = pl.ds(tb * TB, TB)
        return pltpu.make_async_copy(q_hbm.at[:, cols], q_ref.at[:, cols],
                                     sem.at[3 * NIT + tb])

    cp_w1 = pltpu.make_async_copy(w1_hbm, w1_ref, sem.at[3 * NIT + NTB])
    cp_w2 = pltpu.make_async_copy(w2_hbm, w2_ref, sem.at[3 * NIT + NTB + 1])
    cp_wf = pltpu.make_async_copy(wf_hbm, wf_ref, sem.at[3 * NIT + NTB + 2])
    cp_wi = pltpu.make_async_copy(wi_hbm, wi_ref, sem.at[3 * NIT + NTB + 3])
    PRE = 6
    LA = 3

    def start_kvh(rng):
        for i in rng:
            for cp in kvh_copies(i):
                cp.start()

    start_kvh(range(PRE - 1))

    def params():
        par = jnp.concatenate(
            [sk_ref[...].astype(f32), sd_ref[...].astype(f32),
             jnp.zeros((3, D), f32)], axis=0)
        par_ref[...] = par.T

    def kv_rows(r0, n):
        rows = pl.ds(r0, n)
        par = par_ref[rows, :]
        k = k_ref[rows, :].astype(f32)
        lane = jax.lax.broadcasted_iota(jnp.int32, (n, S), 1)
        ks = k * par[:, 0:1]
        for j in range(1, 4):
            kj = jnp.where(lane >= j, pltpu.roll(k, j, 1), 0.0)
            ks = ks + kj * par[:, j:j + 1]
        u_ref[rows, :] = ks * v_ref[rows, :].astype(f32)

    hb = NB // 2
    low8 = jax.lax.broadcasted_iota(jnp.int32, (8, NB), 1) < hb
    swap = lambda x: pltpu.roll(x, hb, 1)

    def tw64(m):
        return (math.cos(2 * math.pi * m / (2 * NA)),
                math.sin(2 * math.pi * m / (2 * NA)))

    def s1_rows(src, r8, g8):
        xs = [src[pl.ds(r8, 8), pl.ds(NB * a, NB)].astype(f32)
              for a in range(NA // 2)]
        xs = xs + [None] * (NA // 2)
        g = _rdft(xs)
        rows = pl.ds(g8, 8)
        for m in range(NF1):
            c, s = tw64(m)
            vr, vi = g[m]
            rvr = swap(vr)
            if vi is None:
                p1 = jnp.where(low8, vr, 0.0)
                p2 = jnp.where(low8, rvr, 0.0)
                p3 = jnp.where(low8, 0.0, -vr)
            else:
                rvi = swap(vi)
                p1 = jnp.where(low8, vr, rvi)
                p2 = jnp.where(low8, rvr, vi)
                p3 = jnp.where(low8, rvi, -vr)
            if m == 0:
                t = p2
            elif m == NF1 - 1:
                t = p3
            else:
                t = c * p2 + s * p3
            g_ref[m, rows, :] = p1 + t
            if m < NF1 - 1:
                g_ref[NA - m, rows, :] = p1 - t
        return t

    def spec_stage():
        low1 = jax.lax.broadcasted_iota(jnp.int32, (D, NB), 1) < hb

        def fwd(f1):
            g_ref[f1] = jnp.dot(g_ref[f1].astype(bf16), wf_ref[f1],
                                preferred_element_type=f32)

        def inv(f1):
            xu = g_ref[f1, pl.ds(0, D), :]
            xh = g_ref[f1, pl.ds(D, D), :]
            xs, hs = swap(xu), swap(xh)
            y = (jnp.where(low1, xu, xs) * xh
                 - jnp.where(low1, xs, -xu) * hs)
            p_ref[f1] = jnp.dot(y.astype(bf16), wi_ref[f1],
                                preferred_element_type=f32)

        fwd(0)
        fwd(1)
        for f1 in range(NFF):
            if f1 + 2 < NFF:
                fwd(f1 + 2)
            inv(f1)

    def i1_rows(r8):
        rows = pl.ds(r8, 8)
        xs = []
        for m in range(NF1):
            c, s = tw64(m)
            pa = p_ref[m, rows, :]
            if m < NF1 - 1:
                pb = p_ref[NA - m, rows, :]
            else:
                pb = jnp.where(low8, pa, -pa)
            e = pa + pb
            dif = pa - pb
            if m == 0:
                o = dif
            else:
                sd_ = swap(dif)
                sd_ = jnp.where(low8, -sd_, sd_)
                o = sd_ if m == NF1 - 1 else c * dif + s * sd_
            xs.append((jnp.where(low8, e, swap(o)),
                       jnp.where(low8, swap(e), o)))
        y = _irdft(xs, NA, NA // 2)
        sd = par_ref[rows, :][:, 4:5]
        for a in range(NA // 2):
            col = pl.ds(NB * a, NB)
            yc = y[a].astype(bf16).astype(f32)
            tok = yc + u_ref[rows, col] * sd
            y_ref[rows, col] = tok
        return tok

    def layernorm(tb):
        cols = pl.ds(tb * TB, TB)
        x = q_ref[:, cols].astype(f32)
        mean = jnp.mean(x, axis=0, keepdims=True)
        xc = x - mean
        var = jnp.mean(xc * xc, axis=0, keepdims=True)
        xn = xc * jax.lax.rsqrt(var + EPS)
        xn_ref[pl.ds(0, D), cols] = xn.astype(bf16)
        base_ref[:, cols] = x

    def ffn_up(n):
        tb, i = divmod(n, NCH)
        h = jnp.dot(w1t_ref[pl.ds(i * FC, FC), :],
                    xn_ref[:, pl.ds(tb * TB, TB)],
                    preferred_element_type=f32)
        hh = 0.5 * h
        hb_ref[n % 2] = (hh + hh * jnp.tanh(hh)).astype(bf16)

    def ffn_down(n):
        tb, i = divmod(n, NCH)
        part = jnp.dot(w2_ref[:, pl.ds(i * FC, FC)], hb_ref[n % 2],
                       preferred_element_type=f32)
        cols = pl.ds(tb * TB, TB)
        base_ref[:, cols] = base_ref[:, cols] + part

    def combine(rows, cols):
        out = (base_ref[rows, cols]
               + xn_ref[rows, cols].astype(f32) * y_ref[rows, cols])
        o_ref[rows, cols] = out.astype(o_ref.dtype)
        return out[0:8, 0:NB]

    def order_before(tok, g, n):
        if n < NTB * NCH:
            i = n % NCH
            t = jnp.clip(tok[:, :DP - D], -1.0, 1.0)
            t = jnp.where(t == t, t, 0.0)
            w1t_ref[pl.ds(i * FC + 8 * g, 8), pl.ds(D, DP - D)] = (
                t.astype(bf16))

    def out_copy(rows, cols, s):
        return pltpu.make_async_copy(o_ref.at[rows, cols],
                                     o_hbm.at[rows, cols], osem.at[s])

    def fwd_slot(i, n):
        kv_rows(i * CPI, CPI)
        for g in range(CPI // 8):
            r8 = i * CPI + g * 8
            order_before(s1_rows(u_ref, r8, r8), 2 * g, n)
            order_before(s1_rows(hk_ref, r8, D + r8), 2 * g + 1, n)

    NSL = NTB * NCH
    N_S1 = 10
    N_I1 = 21
    early = pl.ds(0, (NTB - 1) * TB)

    def split(items, j, parts):
        return items[len(items) * j // parts:len(items) * (j + 1) // parts]

    def row_part(j, parts):
        units = D // 16
        lo = (units * j // parts) * 16
        hi = (units * (j + 1) // parts) * 16
        return pl.ds(lo, hi - lo)

    s1_units = list(range(PRE * CPI, D, 16))
    i1_units = list(range(0, D, 8))
    need = {}
    for n in range(N_S1):
        last = (split(s1_units, n, N_S1)[-1] + 15) // CPI
        need[n] = last
    WAITS = {}
    done = PRE - 1
    for n in (0, 5):
        hi = need[min(n + 4, N_S1 - 1)] if n == 0 else NIT - 1
        WAITS[n] = range(done + 1, hi + 1)
        done = hi

    def extra(n):
        if n < N_S1:
            g = 0
            for r16 in split(s1_units, n, N_S1):
                kv_rows(r16, 16)
                for r8 in (r16, r16 + 8):
                    order_before(s1_rows(u_ref, r8, r8), g, n + LA)
                    order_before(s1_rows(hk_ref, r8, D + r8), g + 1, n + LA)
                    g += 2
        elif n < N_I1:
            for g, r8 in enumerate(split(i1_units, n - N_S1, N_I1 - N_S1)):
                order_before(i1_rows(r8), g, n + LA)
        else:
            rows = row_part(n - N_I1, NSL - N_I1)
            order_before(combine(rows, early), 0, n + LA)
            out_copy(rows, early, 0).start()

    with jax.named_scope("pro"):
        params()
        xn_ref[pl.ds(D, DP - D), :] = jnp.zeros((DP - D, S), bf16)
        w1t_ref[:, pl.ds(D, DP - D)] = jnp.zeros((F, DP - D), bf16)
        for i in range(PRE):
            for cp in kvh_copies(i):
                cp.wait()
            if i == 0:
                start_kvh(range(PRE - 1, PRE))
                cp_w1.start()
                q_copy(0).start()
            if i == min(3, PRE - 1):
                cp_w2.start()
            fwd_slot(i, NSL)
        cp_w1.wait()
        start_kvh(WAITS[0])
        w1t_ref[:, pl.ds(0, D)] = w1_ref[...].astype(f32).T.astype(bf16)
        q_copy(0).wait()
        layernorm(0)
        ffn_up(0)
        cp_w2.wait()

    for n in range(NSL):
        for i in WAITS.get(n, ()):
            for cp in kvh_copies(i):
                cp.wait()
        if n == 0:
            start_kvh(WAITS[5])
            q_copy(1).start()
        if n == 5:
            cp_wf.start()
            cp_wi.start()
            q_copy(2).start()
            q_copy(3).start()
            q_copy(1).wait()
            layernorm(1)
        if n == N_S1:
            cp_wf.wait()
            cp_wi.wait()
            q_copy(2).wait()
            q_copy(3).wait()
            layernorm(2)
            spec_stage()
            layernorm(3)
        extra(n)
        if n + 1 < NSL:
            ffn_up(n + 1)
        ffn_down(n)

    with jax.named_scope("fin"):
        late = pl.ds((NTB - 1) * TB, TB)
        combine(pl.ds(0, D), late)
        cp_late = out_copy(pl.ds(0, D), late, 1)
        cp_late.start()
        out_copy(pl.ds(0, D), early, 0).wait()
        cp_late.wait()


@jax.jit
def pallas_parallel_sum__ssm_conv_h3__dense_activation_silu__prompt_kernel(
    A_q: jax.Array,
    A_k: jax.Array,
    A_v: jax.Array,
    A_shift_k: jax.Array,
    A_ssm_k: jax.Array,
    A_ssm_D: jax.Array,
    B_x: jax.Array,
    B_w1: jax.Array,
    B_w2: jax.Array,
):
    del B_x
    qt = A_q.reshape(S, D).T
    kt = A_k.reshape(S, D).T
    vt = A_v.reshape(S, D).T
    sk = A_shift_k.T
    sd = A_ssm_D.reshape(1, D)
    w2t = B_w2.T
    wf_np, wi_np = _dft_tables()
    wf = jnp.asarray(wf_np, dtype=jnp.bfloat16)
    wi = jnp.asarray(wi_np, dtype=jnp.bfloat16)

    hbm = pl.BlockSpec(memory_space=pl.ANY)
    vmem = pl.BlockSpec(memory_space=pltpu.VMEM)
    in_specs = [hbm, hbm, hbm, vmem, hbm, vmem, hbm, hbm, hbm, hbm]
    bf = jnp.bfloat16
    scratch = [
        pltpu.VMEM((D, S), bf),
        pltpu.VMEM((D, S), bf),
        pltpu.VMEM((D, S), bf),
        pltpu.VMEM((D, S), bf),
        pltpu.VMEM((D, F), bf),
        pltpu.VMEM((D, F), bf),
        pltpu.VMEM((D, S), bf),
        pltpu.VMEM((NFF, NB, NB), bf),
        pltpu.VMEM((NFF, NB, NB), bf),
        pltpu.VMEM((F, DP), bf),
        pltpu.VMEM((D, 8), jnp.float32),
        pltpu.VMEM((D, S), jnp.float32),
        pltpu.VMEM((NFF, 2 * D, NB), jnp.float32),
        pltpu.VMEM((NFF, D, NB), jnp.float32),
        pltpu.VMEM((D, S), jnp.float32),
        pltpu.VMEM((2, FC, TB), bf),
        pltpu.VMEM((D, S), jnp.float32),
        pltpu.VMEM((DP, S), bf),
        pltpu.SemaphoreType.DMA((3 * 2 * (F // FC) + NTB + 4,)),
        pltpu.SemaphoreType.DMA((2,)),
    ]
    out = pl.pallas_call(
        _kernel,
        in_specs=in_specs,
        out_specs=hbm,
        out_shape=jax.ShapeDtypeStruct((D, S), bf),
        scratch_shapes=scratch,
        compiler_params=pltpu.CompilerParams(
            vmem_limit_bytes=100 * 1024 * 1024,
        ),
    )(qt, kt, vt, sk, A_ssm_k, sd, B_w1, w2t, wf, wi)
    return out.T.reshape(1, S, D)
```
